```python
import jax
import jax.numpy as jnp

def _softmax(x, axis=-1):
    return jax.nn.softmax(x, axis=axis)
def _gelu(x):
    return jax.nn.gelu(x, approximate=True)
def _silu(x):
    return jax.nn.silu(x)
def _sigmoid(x):
    return jax.nn.sigmoid(x)
def _layernorm(x, axis=-1, eps=1e-5):
    m = jnp.mean(x, axis=axis, keepdims=True)
    v = jnp.var(x, axis=axis, keepdims=True)
    return (x - m) / jnp.sqrt(v + eps)
def _scatter_add(tgt, idx, src, axis=0):
    return tgt.at[idx].add(src)
def _segment_sum(src, seg, n):
    return jax.ops.segment_sum(src, seg, n)
class _Rng:
    def __init__(self, key):
        self._k = key
    def _next(self):
        self._k, sub = jax.random.split(self._k)
        return sub
    def normal(self, shape):
        return jax.random.normal(self._next(), shape, dtype=jnp.bfloat16)
    def randint(self, lo, hi, shape):
        return jax.random.randint(self._next(), shape, lo, hi, dtype=jnp.int32)
    def uniform(self, shape, lo=0.0, hi=1.0):
        return jax.random.uniform(self._next(), shape, jnp.bfloat16, lo, hi)
    def permutation(self, n):
        return jax.random.permutation(self._next(), n)


kernel_name = 'concat_heads__sliding_local_dilated__compressed_kv_cla__prompt'

def setup_inputs():
    _rng = _Rng(jax.random.key(int.from_bytes(__import__("os").urandom(4), "little")))
    _w = (lambda a: (lambda t: t.astype(jnp.bfloat16) if jnp.issubdtype(t.dtype, jnp.floating) else t)(jnp.asarray(a)))
    def _A_setup():
        B, S, D = 1, 2048, 1024
        return {
            "x": _w((lambda *s: _rng.normal(s) * 0.05)(B, S, D)),
            "wqkv": _w((lambda *s: _rng.normal(s) * 0.05)(D, 3 * D)),
            "wo": _w((lambda *s: _rng.normal(s) * 0.05)(D, D)),
        }
    _A_in = _A_setup()

    def _B_setup():
        B, H, Sq, Sk, D, M = 1, 32, 2048, 2048, 128, 1024
        Dc = 4 * D
        return {
            "x": _w((lambda *s: _rng.normal(s) * 0.05)(B, Sq, M)),
            "c_kv": _w((lambda *s: _rng.normal(s) * 0.05)(B, Sk, Dc)),
            "w_q": _w((lambda *s: _rng.normal(s) * 0.05)(M, H, D) * (M ** -0.5)),
            "w_uk": _w((lambda *s: _rng.normal(s) * 0.05)(Dc, H, D) * (Dc ** -0.5)),
            "w_uv": _w((lambda *s: _rng.normal(s) * 0.05)(Dc, H, D) * (Dc ** -0.5)),
            "w_o": _w((lambda *s: _rng.normal(s) * 0.05)(H, D, M) * ((H * D) ** -0.5)),
        }
    _B_in = _B_setup()

    return {
        "A_x": _A_in["x"],
        "A_wqkv": _A_in["wqkv"],
        "A_wo": _A_in["wo"],
        "B_x": _B_in["x"],
        "B_c_kv": _B_in["c_kv"],
        "B_w_q": _B_in["w_q"],
        "B_w_uk": _B_in["w_uk"],
        "B_w_uv": _B_in["w_uv"],
        "B_w_o": _B_in["w_o"],
    }

def reference(A_x, A_wqkv, A_wo, B_x, B_c_kv, B_w_q, B_w_uk, B_w_uv, B_w_o):
    def _A_ref(x, wqkv, wo):
        B, S, D = x.shape
        H = 32; Dh = D // H
        W, dil = 8, 2
        qkv = (lambda x, *d: x.transpose(*d))((x @ wqkv).reshape(B, S, 3, H, Dh), 2, 0, 3, 1, 4)
        q, k, v = qkv[0], qkv[1], qkv[2]
        scale = Dh ** -0.5
        pos = jnp.arange(S)
        off = jnp.arange(W) * dil
        idx = pos[:, None] - off[None, :]
        mask = idx >= 0
        idx_c = jnp.where(mask, idx, 0).reshape(-1)
        kg = k[:, :, idx_c, :].reshape(B, H, S, W, Dh)
        vg = v[:, :, idx_c, :].reshape(B, H, S, W, Dh)
        logits = jnp.einsum("bhsd,bhswd->bhsw", q, kg) * scale
        logits = jnp.where(mask[None, None, :, :], logits, -1e9)
        attn = _softmax(logits, axis=-1)
        o = jnp.einsum("bhsw,bhswd->bhsd", attn, vg)
        return (lambda x, *d: x.transpose(*d))(o, 0, 2, 1, 3).reshape(B, S, D) @ wo

    def _B_ref(x, c_kv, w_q, w_uk, w_uv, w_o):
        B, Sq, M = x.shape[0], x.shape[1], x.shape[2]
        Sk = c_kv.shape[1]
        H, D = w_q.shape[1], w_q.shape[2]
        q = jnp.einsum("bqm,mhd->bhqd", x, w_q)
        k = jnp.einsum("bkc,chd->bhkd", c_kv, w_uk)
        v = jnp.einsum("bkc,chd->bhkd", c_kv, w_uv)
        scores = jnp.einsum("bhqd,bhkd->bhqk", q, k) * (D ** -0.5)
        off = Sk - Sq
        qi = jnp.arange(Sq)[:, None]
        kj = jnp.arange(Sk)[None, :]
        cmask = kj <= (qi + off)
        scores = jnp.where(cmask[None, None], scores, -1e9)
        p = _softmax(scores, axis=-1)
        ctx = jnp.einsum("bhqk,bhkd->bhqd", p, v)
        return jnp.einsum("bhqd,hdm->bqm", ctx, w_o)

    a = _A_ref(A_x, A_wqkv, A_wo)
    b = _B_ref(B_x, B_c_kv, B_w_q, B_w_uk, B_w_uv, B_w_o)
    return jnp.concatenate([a, b], axis=-1)
```

```python
import math

import jax
import jax.numpy as jnp
import jax.experimental.pallas as pl
import jax.experimental.pallas.tpu as pltpu

bf16 = jnp.bfloat16
f32 = jnp.float32
u32 = jnp.uint32

S = 2048
DA = 1024
HA = 32
DH = 32
WIN = 8
DIL = 2
M = 1024
C = 512
H = 32
D = 128
LOG2E = math.log2(math.e)
NEG = -1e30
PADR = 16
DP = HA + 1
TA = 256
TQ = 256
TP = 256
TO = 256
NT = (((1,), (1,)), ((), ()))


def _unpack(x):
    return pltpu.bitcast(x, bf16)


def _pack(x):
    return pltpu.bitcast(x, u32)


def _dot(a, b):
    return jnp.dot(a, b, preferred_element_type=f32)


def _dot_nt(a, b):
    return jax.lax.dot_general(a, b, NT, preferred_element_type=f32)


def _prep_wqkv(wqkv_v, stage, wtp):
    def body(rb, carry):
        r0 = pl.multiple_of(rb * 128, 128)
        for t in range(3):
            for cb in range(8):
                c0 = t * DA + cb * 128
                tile = wqkv_v[pl.ds(r0, 128), c0:c0 + 128].astype(f32).T
                for hl in range(4):
                    stage[pl.ds(t * HA * DP + 4 * cb + hl, DH, stride=DP), :] = (
                        tile[hl * DH:(hl + 1) * DH, :])
        for t in range(3):
            for d in range(DH):
                rows = stage[pl.ds(t * HA * DP + d * DP, HA), :]
                o0 = (t * DA + d * HA) // 2
                wtp[rb, o0:o0 + HA // 2, :] = _pack(rows.astype(bf16))
        return carry

    jax.lax.fori_loop(0, 8, body, 0)


def _prep_wo(wo_v, stage, wop):
    for nb in range(8):
        for h in range(HA):
            rows = wo_v[h * DH:(h + 1) * DH, nb * 128:(nb + 1) * 128].astype(f32)
            stage[pl.ds(h, DH, stride=DP), :] = rows
        for d in range(DH):
            rows = stage[pl.ds(d * DP, HA), :]
            wop[nb, d * (HA // 2):(d + 1) * (HA // 2), :] = _pack(rows.astype(bf16))


def _a_proj(r, ax_v, wtp, qp, kp, vp):
    r0 = pl.multiple_of(r * TA, TA)
    x = ax_v[pl.ds(r0, TA), :]
    NB = 512
    for t, dst, off in ((0, qp, None), (1, kp, PADR), (2, vp, PADR)):
        for n in range(DA // NB):
            f0 = (t * DA + n * NB) // 2
            w = jnp.concatenate(
                [_unpack(wtp[rb, f0:f0 + NB // 2, :]) for rb in range(8)], axis=1)
            y = _dot_nt(x, w)
            if off is None:
                dst[:, n * NB:(n + 1) * NB] = y
            else:
                for cc in range(NB // 128):
                    dst[n * (NB // 128) + cc, pl.ds(r0 + off, TA), :] = (
                        y[:, cc * 128:(cc + 1) * 128])


def _a_attn(r, qp, kp, vp, op):
    G = 16
    scale = (DH ** -0.5) * LOG2E
    for g in range(TA // G):
        row0 = r * TA + g * G
        q = qp[g * G:(g + 1) * G, :]
        pos = row0 + jax.lax.broadcasted_iota(jnp.int32, (G, 128), 0)
        logits = []
        for w in range(WIN):
            z = None
            for c in range(8):
                p = q[:, c * 128:(c + 1) * 128] * kp[c, pl.ds(row0 + PADR - DIL * w, G), :]
                z = p if z is None else z + p
            z = z + pltpu.roll(z, 64, 1)
            z = z + pltpu.roll(z, 32, 1)
            z = z * scale
            if w > 0:
                z = jnp.where(pos >= DIL * w, z, NEG)
            logits.append(z)
        m = logits[0]
        for w in range(1, WIN):
            m = jnp.maximum(m, logits[w])
        es = [jnp.exp2(z - m) for z in logits]
        l = es[0]
        for w in range(1, WIN):
            l = l + es[w]
        inv = 1.0 / l
        attn = [e * inv for e in es]
        o0 = pl.multiple_of(row0 // 2, G // 2)
        for c in range(8):
            acc = None
            for w in range(WIN):
                v = vp[c, pl.ds(row0 + PADR - DIL * w, G), :]
                acc = attn[w] * v if acc is None else acc + attn[w] * v
            op[pl.ds(o0, G // 2), c * 128:(c + 1) * 128] = _pack(acc.astype(bf16))


def _deinterleave(raw, dst, rows):
    pitch = rows + 1

    def body(mb, carry):
        base = pl.multiple_of(mb * 8, 8)
        blk = _pack(raw[pl.ds(pl.multiple_of(base * H, 8 * H), 8 * H), :])
        for mm in range(8):
            dst[pl.ds(base + mm, H // 2, stride=pitch), :] = (
                blk[mm * (H // 2):(mm + 1) * (H // 2), :])
        return carry

    jax.lax.fori_loop(0, rows // 8, body, 0)


def _pair_weights(wt, j, rows):
    w = wt[pl.ds(j * (rows + 1), rows), :]
    lo = pltpu.bitcast(w << 16, f32).astype(bf16)
    hi = pltpu.bitcast(w & jnp.uint32(0xFFFF0000), f32).astype(bf16)
    return jnp.concatenate([lo, hi], axis=1)


def _b_proj(r, ws, bxp, cp, qb, kb, vb, b):
    wq, wk, wv = ws
    rows = slice(r * TP // 2, (r + 1) * TP // 2)
    xs = _unpack(bxp[rows, :])
    cs = _unpack(cp[rows, :])
    q = _dot(xs, wq) * ((D ** -0.5) * LOG2E)
    k = _dot(cs, wk)
    v = _dot(cs, wv)
    for e in range(2):
        qb[b, e, rows, :] = _pack(q[:, e * D:(e + 1) * D].astype(bf16))
        kb[b, e, rows, :] = _pack(k[:, e * D:(e + 1) * D].astype(bf16))
        vb[b, e, rows, :] = _pack(v[:, e * D:(e + 1) * D].astype(bf16))


def _b_qk(i, qb, kb, b, e):
    HQ = TQ // 2
    k0 = i * TQ
    n = k0 + HQ
    q = _unpack(qb[b, e, k0 // 2:(k0 + TQ) // 2, :])
    s = _dot_nt(q, _unpack(kb[b, e, 0:n // 2, :]))
    s2 = _dot_nt(q[HQ:], _unpack(kb[b, e, n // 2:(n + HQ) // 2, :]))
    row = jax.lax.broadcasted_iota(jnp.int32, (HQ, 128), 0)
    col = jax.lax.broadcasted_iota(jnp.int32, (HQ, 128), 1)
    tri = col <= row
    nb = n // 128
    top = [s[:HQ, j * 128:(j + 1) * 128] for j in range(nb)]
    top[-1] = jnp.where(tri, top[-1], NEG)
    bot = [s[HQ:, j * 128:(j + 1) * 128] for j in range(nb)]
    bot.append(jnp.where(tri, s2, NEG))
    mps = []
    for blocks in (top, bot):
        mp = blocks[0]
        for c in blocks[1:]:
            mp = jnp.maximum(mp, c)
        mps.append(mp)
    return (top, bot), mps


def _b_softmax_pv(i, blocks, mps, prev, vb, ctx, b, e, h):
    HQ = TQ // 2
    k0 = i * TQ
    n = k0 + HQ
    ps, ls = [], []
    for half in range(2):
        mp = mps[half]
        if prev is not None:
            mp = jnp.maximum(mp, jnp.minimum(prev[half], NEG))
        m = jnp.max(mp, axis=1, keepdims=True)
        lp = None
        pl_ = []
        for jj, c in enumerate(blocks[half]):
            p = jnp.exp2(c - m)
            lp = p if lp is None else lp + p
            if jj == len(blocks[half]) - 1:
                p = p + jnp.minimum(lp, 0.0)
            pl_.append(p.astype(bf16))
        ps.append(pl_)
        ls.append(jnp.sum(lp, axis=1, keepdims=True))
    nb = n // 128
    pc = jnp.concatenate(
        [jnp.concatenate(ps[0], axis=1), jnp.concatenate(ps[1][:nb], axis=1)], axis=0)
    o = _dot(pc, _unpack(vb[b, e, 0:n // 2, :]))
    o2 = _dot(ps[1][nb], _unpack(vb[b, e, n // 2:(n + HQ) // 2, :]))
    o_top = o[:HQ] * (1.0 / ls[0])
    o_bot = (o[HQ:] + o2) * (1.0 / ls[1])
    ctx[h, k0 // 2:(k0 + HQ) // 2, :] = _pack(o_top.astype(bf16))
    ctx[h, (k0 + HQ) // 2:(k0 + TQ) // 2, :] = _pack(o_bot.astype(bf16))
    return (o_top, o_bot)


def _b_pair(j, b, qb, kb, vb, ctx, fillers):
    nT = S // TQ
    order = list(range(nT))[::-1]
    fillers = list(fillers)
    per_head = len(fillers) // 2
    for e in range(2):
        mine = fillers[e * per_head:(e + 1) * per_head]
        cur = _b_qk(order[0], qb, kb, b, e)
        prev = None
        for t, i in enumerate(order):
            nxt = _b_qk(order[t + 1], qb, kb, b, e) if t + 1 < nT else None
            prev = _b_softmax_pv(i, cur[0], cur[1], prev, vb, ctx, b, e, 2 * j + e)
            cur = nxt
            if t >= nT - len(mine):
                mine[t - (nT - len(mine))]()


def _kernel(ax_h, wqkv_h, wo_h, bx_h, c_h, wq_h, wuk_h, wuv_h, wob_h, out_h,
            bx_v, c_v, wq_raw, wuk_raw, wuv_raw, wob_v, wop, op,
            wq_t, wk_t, wv_t, bxp, cp, out_s, sem_in, sem_out):

    def copy_in(src, dst, i):
        return pltpu.make_async_copy(src, dst, sem_in.at[i])

    late = [copy_in(bx_h, bx_v, 3), copy_in(c_h, c_v, 4), copy_in(wq_h, wq_raw, 5),
            copy_in(wuk_h, wuk_raw, 6), copy_in(wuv_h, wuv_raw, 7),
            copy_in(wob_h, wob_v, 8)]

    def phase_a(ax_v, wqkv_v, wo_v, stage, wtp, qp, kp, vp):
        early = [copy_in(wqkv_h, wqkv_v, 0), copy_in(ax_h, ax_v, 1),
                 copy_in(wo_h, wo_v, 2)]
        for cpy in early:
            cpy.start()
        for cpy in late:
            cpy.start()
        kp[:, 0:PADR, :] = jnp.zeros((8, PADR, 128), f32)
        vp[:, 0:PADR, :] = jnp.zeros((8, PADR, 128), f32)
        early[0].wait()
        _prep_wqkv(wqkv_v, stage, wtp)
        early[2].wait()
        _prep_wo(wo_v, stage, wop)
        early[1].wait()

        def body(r, carry):
            _a_proj(r, ax_v, wtp, qp, kp, vp)
            _a_attn(r, qp, kp, vp, op)
            return carry

        jax.lax.fori_loop(0, S // TA, body, 0)

    pl.run_scoped(
        phase_a,
        pltpu.VMEM((S, DA), bf16), pltpu.VMEM((DA, 3 * DA), bf16),
        pltpu.VMEM((DA, DA), bf16), pltpu.VMEM((3 * HA * DP, 128), f32),
        pltpu.VMEM((8, 3 * DA // 2, 128), u32), pltpu.VMEM((TA, DA), f32),
        pltpu.VMEM((8, S + PADR, 128), f32), pltpu.VMEM((8, S + PADR, 128), f32))

    for cpy in late[:5]:
        cpy.wait()
    bxp[...] = _pack(bx_v[...])
    cp[...] = _pack(c_v[...])
    _deinterleave(wq_raw, wq_t, M)
    _deinterleave(wuk_raw, wk_t, C)
    _deinterleave(wuv_raw, wv_t, C)

    def phase_b(qb, kb, vb, ctx):
        def weights(j):
            return (_pair_weights(wq_t, j, M), _pair_weights(wk_t, j, C),
                    _pair_weights(wv_t, j, C))

        ws0 = weights(0)
        for r in range(S // TP):
            _b_proj(r, ws0, bxp, cp, qb, kb, vb, 0)

        def body(j, carry):
            b = j % 2
            ws = weights(j + 1)
            fillers = [
                (lambda r=r: _b_proj(r, ws, bxp, cp, qb, kb, vb, 1 - b))
                for r in range(S // TP)]
            _b_pair(j, b, qb, kb, vb, ctx, fillers)
            return carry

        jax.lax.fori_loop(0, H // 2 - 1, body, 0)
        _b_pair(H // 2 - 1, (H // 2 - 1) % 2, qb, kb, vb, ctx, [])

        late[5].wait()

        def out_copy(r):
            r0 = pl.multiple_of(r * TO, TO)
            return pltpu.make_async_copy(
                out_s.at[pl.ds(r0, TO), :], out_h.at[pl.ds(r0, TO), :], sem_out)

        def obody(r, carry):
            r0 = pl.multiple_of(r * TO, TO)
            p0 = pl.multiple_of(r * (TO // 2), TO // 2)
            oa = _unpack(op[pl.ds(p0, TO // 2), :])
            woa = jnp.concatenate([_unpack(wop[nb]) for nb in range(8)], axis=1)
            out_s[pl.ds(r0, TO), 0:DA] = _dot(oa, woa).astype(bf16)
            cb = jnp.concatenate(
                [_unpack(ctx[h, pl.ds(p0, TO // 2), :]) for h in range(H)], axis=1)
            out_s[pl.ds(r0, TO), DA:DA + M] = _dot(cb, wob_v[...]).astype(bf16)
            out_copy(r).start()
            return carry

        jax.lax.fori_loop(0, S // TO, obody, 0)
        for r in range(S // TO):
            out_copy(r).wait()

    pl.run_scoped(
        phase_b,
        pltpu.VMEM((2, 2, S // 2, D), u32), pltpu.VMEM((2, 2, S // 2, D), u32),
        pltpu.VMEM((2, 2, S // 2, D), u32), pltpu.VMEM((H, S // 2, D), u32))


@jax.jit
def pallas_concat_heads__sliding_local_dilated__compressed_kv_cla__prompt_kernel(
    A_x: jax.Array,
    A_wqkv: jax.Array,
    A_wo: jax.Array,
    B_x: jax.Array,
    B_c_kv: jax.Array,
    B_w_q: jax.Array,
    B_w_uk: jax.Array,
    B_w_uv: jax.Array,
    B_w_o: jax.Array,
):
    any_spec = pl.BlockSpec(memory_space=pl.ANY)
    out = pl.pallas_call(
        _kernel,
        out_shape=jax.ShapeDtypeStruct((S, DA + M), bf16),
        in_specs=[any_spec] * 9,
        out_specs=any_spec,
        scratch_shapes=[
            pltpu.VMEM((S, M), bf16),
            pltpu.VMEM((S, C), bf16),
            pltpu.VMEM((M * H, D), bf16),
            pltpu.VMEM((C * H, D), bf16),
            pltpu.VMEM((C * H, D), bf16),
            pltpu.VMEM((H * D, M), bf16),
            pltpu.VMEM((8, DA // 2, 128), u32),
            pltpu.VMEM((S // 2, DA), u32),
            pltpu.VMEM((H // 2 * (M + 1), D), u32),
            pltpu.VMEM((H // 2 * (C + 1), D), u32),
            pltpu.VMEM((H // 2 * (C + 1), D), u32),
            pltpu.VMEM((S // 2, M), u32),
            pltpu.VMEM((S // 2, C), u32),
            pltpu.VMEM((S, DA + M), bf16),
            pltpu.SemaphoreType.DMA((9,)),
            pltpu.SemaphoreType.DMA(()),
        ],
        compiler_params=pltpu.CompilerParams(vmem_limit_bytes=120 * 1024 * 1024),
    )(
        A_x.reshape(S, DA), A_wqkv, A_wo,
        B_x.reshape(S, M), B_c_kv.reshape(S, C),
        B_w_q.reshape(M * H, D), B_w_uk.reshape(C * H, D), B_w_uv.reshape(C * H, D),
        B_w_o.reshape(H * D, M),
    )
    return out.reshape(1, S, DA + M)
```

```python
import math

import jax
import jax.numpy as jnp
import jax.experimental.pallas as pl
import jax.experimental.pallas.tpu as pltpu

bf16 = jnp.bfloat16
f32 = jnp.float32
u32 = jnp.uint32

S = 2048
DA = 1024
HA = 32
DH = 32
WIN = 8
DIL = 2
M = 1024
C = 512
H = 32
D = 128
LOG2E = math.log2(math.e)
NEG = -1e30
PADR = 16
DP = HA + 1
TA = 256
TQ = 256
TP = 256
TO = 256
NT = (((1,), (1,)), ((), ()))


def _unpack(x):
    return pltpu.bitcast(x, bf16)


def _pack(x):
    return pltpu.bitcast(x, u32)


def _dot(a, b):
    return jnp.dot(a, b, preferred_element_type=f32)


def _dot_nt(a, b):
    return jax.lax.dot_general(a, b, NT, preferred_element_type=f32)


def _prep_wqkv(wqkv_v, stage, wtp, wait_chunk):
    def body(rb, carry):
        r0 = pl.multiple_of(rb * 128, 128)
        wait_chunk(rb)
        for t in range(3):
            for cb in range(8):
                c0 = t * DA + cb * 128
                tile = wqkv_v[pl.ds(r0, 128), c0:c0 + 128].astype(f32).T
                for hl in range(4):
                    stage[pl.ds(t * HA * DP + 4 * cb + hl, DH, stride=DP), :] = (
                        tile[hl * DH:(hl + 1) * DH, :])
        for t in range(3):
            for d in range(DH):
                rows = stage[pl.ds(t * HA * DP + d * DP, HA), :]
                o0 = (t * DA + d * HA) // 2
                wtp[rb, o0:o0 + HA // 2, :] = _pack(rows.astype(bf16))
        return carry

    jax.lax.fori_loop(0, 8, body, 0)


def _prep_wo_block(nb, wo_v, stage, wop):
    for h in range(HA):
        rows = wo_v[nb, h * DH:(h + 1) * DH, :].astype(f32)
        stage[pl.ds(h, DH, stride=DP), :] = rows
    for d in range(DH):
        rows = stage[pl.ds(d * DP, HA), :]
        wop[nb, d * (HA // 2):(d + 1) * (HA // 2), :] = _pack(rows.astype(bf16))


NB = 512


def _a_proj_piece(r, piece, ax_v, wtp, qp, kp, vp):
    t, n = divmod(piece, DA // NB)
    r0 = pl.multiple_of(r * TA, TA)
    x = ax_v[pl.ds(r0, TA), :]
    f0 = (t * DA + n * NB) // 2
    w = jnp.concatenate(
        [_unpack(wtp[rb, f0:f0 + NB // 2, :]) for rb in range(8)], axis=1)
    y = _dot_nt(x, w)
    dst = (qp, kp, vp)[t]
    for cc in range(NB // 128):
        dst[n * (NB // 128) + cc, pl.ds(r0 + PADR, TA), :] = (
            y[:, cc * 128:(cc + 1) * 128])


GA = 16


def _a_attn_group(row0, qp, kp, vp, op):
    G = GA
    scale = (DH ** -0.5) * LOG2E
    pos = row0 + jax.lax.broadcasted_iota(jnp.int32, (G, 128), 0)
    q = [qp[c, pl.ds(row0 + PADR, G), :] for c in range(8)]
    logits = []
    for w in range(WIN):
        z = None
        for c in range(8):
            p = q[c] * kp[c, pl.ds(row0 + PADR - DIL * w, G), :]
            z = p if z is None else z + p
        z = z + pltpu.roll(z, 64, 1)
        z = z + pltpu.roll(z, 32, 1)
        z = z * scale
        if w > 0:
            z = jnp.where(pos >= DIL * w, z, NEG)
        logits.append(z)
    m = logits[0]
    for w in range(1, WIN):
        m = jnp.maximum(m, logits[w])
    es = [jnp.exp2(z - m) for z in logits]
    l = es[0]
    for w in range(1, WIN):
        l = l + es[w]
    inv = 1.0 / l
    attn = [e * inv for e in es]
    o0 = pl.multiple_of(row0 // 2, G // 2)
    for c in range(8):
        acc = None
        for w in range(WIN):
            v = vp[c, pl.ds(row0 + PADR - DIL * w, G), :]
            acc = attn[w] * v if acc is None else acc + attn[w] * v
        op[pl.ds(o0, G // 2), c * 128:(c + 1) * 128] = _pack(acc.astype(bf16))


def _deinterleave_block(mb, raw, dst, rows):
    pitch = rows + 1
    base = pl.multiple_of(mb * 8, 8)
    blk = _pack(raw[pl.ds(pl.multiple_of(base * H, 8 * H), 8 * H), :])
    for mm in range(8):
        dst[pl.ds(base + mm, H // 2, stride=pitch), :] = (
            blk[mm * (H // 2):(mm + 1) * (H // 2), :])


def _pair_weights(wt, j, rows):
    w = wt[pl.ds(j * (rows + 1), rows), :]
    lo = pltpu.bitcast(w << 16, f32).astype(bf16)
    hi = pltpu.bitcast(w & jnp.uint32(0xFFFF0000), f32).astype(bf16)
    return jnp.concatenate([lo, hi], axis=1)


def _b_proj_parts(p0, ws, bxp, cp, qb, kb, vb, slot0):
    wq, wk, wv = ws
    rows = pl.ds(p0, TP // 2)

    def put(dst, y):
        for e in range(2):
            dst[slot0 + e, rows, :] = _pack(y[:, e * D:(e + 1) * D].astype(bf16))

    return [
        lambda: put(qb, _dot(_unpack(bxp[rows, :]), wq) * ((D ** -0.5) * LOG2E)),
        lambda: put(kb, _dot(_unpack(cp[rows, :]), wk)),
        lambda: put(vb, _dot(_unpack(cp[rows, :]), wv)),
    ]


HQ = TQ // 2


def _b_qk(i, qa, ka):
    k0 = i * TQ
    n = k0 + HQ
    q = qa[k0:k0 + TQ]
    s = _dot_nt(q, ka[0:n])
    s2 = _dot_nt(q[HQ:], ka[n:n + HQ])
    row = jax.lax.broadcasted_iota(jnp.int32, (HQ, 128), 0)
    col = jax.lax.broadcasted_iota(jnp.int32, (HQ, 128), 1)
    tri = col <= row
    nb = n // 128
    top = [s[:HQ, j * 128:(j + 1) * 128] for j in range(nb)]
    top[-1] = jnp.where(tri, top[-1], NEG)
    bot = [s[HQ:, j * 128:(j + 1) * 128] for j in range(nb)]
    bot.append(jnp.where(tri, s2, NEG))
    mps = []
    for blocks in (top, bot):
        mp = blocks[0]
        for c in blocks[1:]:
            mp = jnp.maximum(mp, c)
        mps.append(mp)
    return (top, bot), mps


def _b_softmax(blocks, mps, prev):
    ps, lps = [], []
    for half in range(2):
        mp = mps[half]
        if prev is not None:
            mp = jnp.maximum(mp, jnp.minimum(prev[half], NEG))
        m = jnp.max(mp, axis=1, keepdims=True)
        lp = None
        pl_ = []
        for jj, c in enumerate(blocks[half]):
            p = jnp.exp2(c - m)
            lp = p if lp is None else lp + p
            if jj == len(blocks[half]) - 1:
                p = p + jnp.minimum(lp, 0.0)
            pl_.append(p.astype(bf16))
        ps.append(pl_)
        lps.append(lp)
    return ps, lps


def _b_pv(i, ps, lps, va, ctx, h):
    k0 = i * TQ
    n = k0 + HQ
    nb = n // 128
    ls = [jnp.sum(lp, axis=1, keepdims=True) for lp in lps]
    pc = jnp.concatenate(
        [jnp.concatenate(ps[0], axis=1), jnp.concatenate(ps[1][:nb], axis=1)], axis=0)
    o = _dot(pc, va[0:n])
    o2 = _dot(ps[1][nb], va[n:n + HQ])
    o_top = o[:HQ] * (1.0 / ls[0])
    o_bot = (o[HQ:] + o2) * (1.0 / ls[1])
    ctx[h, k0 // 2:(k0 + HQ) // 2, :] = _pack(o_top.astype(bf16))
    ctx[h, (k0 + HQ) // 2:(k0 + TQ) // 2, :] = _pack(o_bot.astype(bf16))
    return (o_top, o_bot)


def _b_head(h, slot, qb, kb, vb, ctx, fillers):
    nT = S // TQ
    order = list(range(nT))[::-1]
    qa, ka, va = _unpack(qb[slot]), _unpack(kb[slot]), _unpack(vb[slot])
    cur = _b_qk(order[0], qa, ka)
    prev = None
    for t, i in enumerate(order):
        nxt = _b_qk(order[t + 1], qa, ka) if t + 1 < nT else None
        ps, lps = _b_softmax(cur[0], cur[1], prev)
        for f in fillers.get(t, ()):
            f()
        prev = _b_pv(i, ps, lps, va, ctx, h)
        cur = nxt


def _kernel(ax_h, wqkv_h, wo_h, bx_h, c_h, wq_h, wuk_h, wuv_h, wob_h, out_h,
            wob_v, wop, op, qp, kp, vp,
            wq_t, wk_t, wv_t, bxp, cp, out_s,
            sem_w, sem_ax, sem_f, sem_wob, sem_out):
    NR = S // TA

    def rows(ref, r, n):
        return ref.at[pl.ds(pl.multiple_of(r * n, n), n), :]

    wob_copy = pltpu.make_async_copy(wob_h, wob_v, sem_wob)

    def phase_a(ax_v, wqkv_v, wo_v, stage, wtp, bx_v, c_v, wq_raw, wuk_raw, wuv_raw):
        def w_copy(r):
            return pltpu.make_async_copy(rows(wqkv_h, r, 128), rows(wqkv_v, r, 128),
                                         sem_w.at[r])

        def ax_copy(r):
            return pltpu.make_async_copy(rows(ax_h, r, TA), rows(ax_v, r, TA),
                                         sem_ax.at[r])

        def f_copies(r):
            return [
                pltpu.make_async_copy(rows(wq_h, r, M * H // NR),
                                      rows(wq_raw, r, M * H // NR), sem_f.at[6 * r]),
                pltpu.make_async_copy(rows(wuk_h, r, C * H // NR),
                                      rows(wuk_raw, r, C * H // NR), sem_f.at[6 * r + 1]),
                pltpu.make_async_copy(rows(wuv_h, r, C * H // NR),
                                      rows(wuv_raw, r, C * H // NR), sem_f.at[6 * r + 2]),
                pltpu.make_async_copy(rows(bx_h, r, TA), rows(bx_v, r, TA),
                                      sem_f.at[6 * r + 3]),
                pltpu.make_async_copy(rows(c_h, r, TA), rows(c_v, r, TA),
                                      sem_f.at[6 * r + 4]),
            ]

        def wo_copy(r):
            c0 = pl.multiple_of(r * 128, 128)
            return pltpu.make_async_copy(wo_h.at[:, pl.ds(c0, 128)], wo_v.at[r],
                                         sem_f.at[6 * r + 5])

        for r in range(NR):
            w_copy(r).start()
        ax_copy(0).start()
        for ref in (kp, vp):
            ref[:, 0:PADR, :] = jnp.zeros((8, PADR, 128), f32)
        _prep_wqkv(wqkv_v, stage, wtp, lambda rb: w_copy(rb).wait())
        ax_copy(1).start()

        def body(r, carry):
            ax_copy(r).wait()

            @pl.when(r + 2 < NR)
            def _():
                ax_copy(r + 2).start()

            for cpy in f_copies(r):
                cpy.start()
            wo_copy(r).start()
            for piece in range(3 * DA // NB):
                _a_proj_piece(r, piece, ax_v, wtp, qp, kp, vp)
            for g in range(TA // GA):
                _a_attn_group(r * TA + g * GA, qp, kp, vp, op)
            return carry

        jax.lax.fori_loop(0, NR, body, 0)
        wob_copy.start()

        for r in range(NR):
            for cpy in f_copies(r):
                cpy.wait()
            wo_copy(r).wait()

        def prep(r, carry):
            for i in range(16):
                _deinterleave_block(r * 16 + i, wq_raw, wq_t, M)
            for i in range(8):
                _deinterleave_block(r * 8 + i, wuk_raw, wk_t, C)
                _deinterleave_block(r * 8 + i, wuv_raw, wv_t, C)
            src = pl.ds(pl.multiple_of(r * TA, TA), TA)
            dst = pl.ds(pl.multiple_of(r * (TA // 2), TA // 2), TA // 2)
            bxp[dst, :] = _pack(bx_v[src, :])
            cp[dst, :] = _pack(c_v[src, :])
            _prep_wo_block(r, wo_v, stage, wop)
            return carry

        jax.lax.fori_loop(0, NR, prep, 0)

    pl.run_scoped(
        phase_a,
        pltpu.VMEM((S, DA), bf16), pltpu.VMEM((DA, 3 * DA), bf16),
        pltpu.VMEM((8, DA, 128), bf16), pltpu.VMEM((3 * HA * DP, 128), f32),
        pltpu.VMEM((8, 3 * DA // 2, 128), u32),
        pltpu.VMEM((S, M), bf16), pltpu.VMEM((S, C), bf16),
        pltpu.VMEM((M * H, D), bf16), pltpu.VMEM((C * H, D), bf16),
        pltpu.VMEM((C * H, D), bf16))

    def phase_b(qb, kb, vb, ctx):
        def weights(j):
            return (_pair_weights(wq_t, j, M), _pair_weights(wk_t, j, C),
                    _pair_weights(wv_t, j, C))

        ws0 = weights(0)
        for r in range(S // TP):
            for f in _b_proj_parts(r * (TP // 2), ws0, bxp, cp, qb, kb, vb, 0):
                f()

        def body(h, carry):
            e = h % 2
            ws = weights(h // 2 + 1)
            wslot = 2 * ((h // 2 + 1) % 2)
            half = S // 4
            nf = S // TP // 2
            fillers = {
                S // TQ - nf + r: _b_proj_parts(
                    pl.multiple_of(e * half + r * (TP // 2), TP // 2),
                    ws, bxp, cp, qb, kb, vb, wslot)
                for r in range(nf)}
            _b_head(h, h % 4, qb, kb, vb, ctx, fillers)
            return carry

        jax.lax.fori_loop(0, H - 2, body, 0)

        def tail(h, carry):
            _b_head(h, h % 4, qb, kb, vb, ctx, {})
            return carry

        jax.lax.fori_loop(H - 2, H, tail, 0)

        wob_copy.wait()

        def out_copy(r):
            r0 = pl.multiple_of(r * TO, TO)
            return pltpu.make_async_copy(
                out_s.at[pl.ds(r0, TO), :], out_h.at[pl.ds(r0, TO), :], sem_out)

        def obody(r, carry):
            r0 = pl.multiple_of(r * TO, TO)
            p0 = pl.multiple_of(r * (TO // 2), TO // 2)
            oa = _unpack(op[pl.ds(p0, TO // 2), :])
            woa = jnp.concatenate([_unpack(wop[nb]) for nb in range(8)], axis=1)
            out_s[pl.ds(r0, TO), 0:DA] = _dot(oa, woa).astype(bf16)
            cb = jnp.concatenate(
                [_unpack(ctx[h, pl.ds(p0, TO // 2), :]) for h in range(H)], axis=1)
            out_s[pl.ds(r0, TO), DA:DA + M] = _dot(cb, wob_v[...]).astype(bf16)
            out_copy(r).start()
            return carry

        jax.lax.fori_loop(0, S // TO, obody, 0)
        for r in range(S // TO):
            out_copy(r).wait()

    pl.run_scoped(
        phase_b,
        pltpu.VMEM((4, S // 2, D), u32), pltpu.VMEM((4, S // 2, D), u32),
        pltpu.VMEM((4, S // 2, D), u32), pltpu.VMEM((H, S // 2, D), u32))


@jax.jit
def pallas_concat_heads__sliding_local_dilated__compressed_kv_cla__prompt_kernel(
    A_x: jax.Array,
    A_wqkv: jax.Array,
    A_wo: jax.Array,
    B_x: jax.Array,
    B_c_kv: jax.Array,
    B_w_q: jax.Array,
    B_w_uk: jax.Array,
    B_w_uv: jax.Array,
    B_w_o: jax.Array,
):
    any_spec = pl.BlockSpec(memory_space=pl.ANY)
    out = pl.pallas_call(
        _kernel,
        out_shape=jax.ShapeDtypeStruct((S, DA + M), bf16),
        in_specs=[any_spec] * 9,
        out_specs=any_spec,
        scratch_shapes=[
            pltpu.VMEM((H * D, M), bf16),
            pltpu.VMEM((8, DA // 2, 128), u32),
            pltpu.VMEM((S // 2, DA), u32),
            pltpu.VMEM((8, S + PADR, 128), f32),
            pltpu.VMEM((8, S + PADR, 128), f32),
            pltpu.VMEM((8, S + PADR, 128), f32),
            pltpu.VMEM((H // 2 * (M + 1), D), u32),
            pltpu.VMEM((H // 2 * (C + 1), D), u32),
            pltpu.VMEM((H // 2 * (C + 1), D), u32),
            pltpu.VMEM((S // 2, M), u32),
            pltpu.VMEM((S // 2, C), u32),
            pltpu.VMEM((S, DA + M), bf16),
            pltpu.SemaphoreType.DMA((8,)),
            pltpu.SemaphoreType.DMA((8,)),
            pltpu.SemaphoreType.DMA((48,)),
            pltpu.SemaphoreType.DMA(()),
            pltpu.SemaphoreType.DMA(()),
        ],
        compiler_params=pltpu.CompilerParams(vmem_limit_bytes=120 * 1024 * 1024),
    )(
        A_x.reshape(S, DA), A_wqkv, A_wo,
        B_x.reshape(S, M), B_c_kv.reshape(S, C),
        B_w_q.reshape(M * H, D), B_w_uk.reshape(C * H, D), B_w_uv.reshape(C * H, D),
        B_w_o.reshape(H * D, M),
    )
    return out.reshape(1, S, DA + M)
```

```python
import math

import jax
import jax.numpy as jnp
import jax.experimental.pallas as pl
import jax.experimental.pallas.tpu as pltpu

bf16 = jnp.bfloat16
f32 = jnp.float32
u32 = jnp.uint32

S = 2048
DA = 1024
HA = 32
DH = 32
WIN = 8
DIL = 2
M = 1024
C = 512
H = 32
D = 128
LOG2E = math.log2(math.e)
NEG = -1e30
PADR = 16
DP = HA + 1
TA = 256
TQ = 256
TP = 256
TO = 256
NT = (((1,), (1,)), ((), ()))


def _unpack(x):
    return pltpu.bitcast(x, bf16)


def _pack(x):
    return pltpu.bitcast(x, u32)


def _dot(a, b):
    return jnp.dot(a, b, preferred_element_type=f32)


def _dot_nt(a, b):
    return jax.lax.dot_general(a, b, NT, preferred_element_type=f32)


def _prep_wqkv(wqkv_v, stage, wtp, wait_chunk):
    def body(rb, carry):
        r0 = pl.multiple_of(rb * 128, 128)
        wait_chunk(rb)
        for t in range(3):
            for cb in range(8):
                c0 = t * DA + cb * 128
                tile = wqkv_v[pl.ds(r0, 128), c0:c0 + 128].astype(f32).T
                for hl in range(4):
                    stage[pl.ds(t * HA * DP + 4 * cb + hl, DH, stride=DP), :] = (
                        tile[hl * DH:(hl + 1) * DH, :])
        for t in range(3):
            for d in range(DH):
                rows = stage[pl.ds(t * HA * DP + d * DP, HA), :]
                o0 = (t * DA + d * HA) // 2
                wtp[rb, o0:o0 + HA // 2, :] = _pack(rows.astype(bf16))
        return carry

    jax.lax.fori_loop(0, 8, body, 0)


def _prep_wo_block(nb, wo_v, stage, wop):
    for h in range(HA):
        rows = wo_v[nb, h * DH:(h + 1) * DH, :].astype(f32)
        stage[pl.ds(h, DH, stride=DP), :] = rows
    for d in range(DH):
        rows = stage[pl.ds(d * DP, HA), :]
        wop[nb, d * (HA // 2):(d + 1) * (HA // 2), :] = _pack(rows.astype(bf16))


NB = 512


def _a_proj_piece(r, piece, ax_v, wtp, qp, kp, vp):
    t, n = divmod(piece, DA // NB)
    r0 = pl.multiple_of(r * TA, TA)
    x = ax_v[pl.ds(r0, TA), :]
    f0 = (t * DA + n * NB) // 2
    w = jnp.concatenate(
        [_unpack(wtp[rb, f0:f0 + NB // 2, :]) for rb in range(8)], axis=1)
    y = _dot_nt(x, w)
    dst = (qp, kp, vp)[t]
    for cc in range(NB // 128):
        dst[n * (NB // 128) + cc, pl.ds(r0 + PADR, TA), :] = (
            y[:, cc * 128:(cc + 1) * 128])


GA = 16


def _a_attn_group(row0, qp, kp, vp, op):
    G = GA
    scale = (DH ** -0.5) * LOG2E
    pos = row0 + jax.lax.broadcasted_iota(jnp.int32, (G, 128), 0)
    q = [qp[c, pl.ds(row0 + PADR, G), :] for c in range(8)]
    logits = []
    for w in range(WIN):
        z = None
        for c in range(8):
            p = q[c] * kp[c, pl.ds(row0 + PADR - DIL * w, G), :]
            z = p if z is None else z + p
        z = z + pltpu.roll(z, 64, 1)
        z = z + pltpu.roll(z, 32, 1)
        z = z * scale
        if w > 0:
            z = jnp.where(pos >= DIL * w, z, NEG)
        logits.append(z)
    m = logits[0]
    for w in range(1, WIN):
        m = jnp.maximum(m, logits[w])
    es = [jnp.exp2(z - m) for z in logits]
    l = es[0]
    for w in range(1, WIN):
        l = l + es[w]
    inv = 1.0 / l
    attn = [e * inv for e in es]
    o0 = pl.multiple_of(row0 // 2, G // 2)
    for c in range(8):
        acc = None
        for w in range(WIN):
            v = vp[c, pl.ds(row0 + PADR - DIL * w, G), :]
            acc = attn[w] * v if acc is None else acc + attn[w] * v
        op[pl.ds(o0, G // 2), c * 128:(c + 1) * 128] = _pack(acc.astype(bf16))


def _deinterleave_block(mb, raw, dst, rows):
    pitch = rows + 1
    base = pl.multiple_of(mb * 8, 8)
    blk = _pack(raw[pl.ds(pl.multiple_of(base * H, 8 * H), 8 * H), :])
    for mm in range(8):
        dst[pl.ds(base + mm, H // 2, stride=pitch), :] = (
            blk[mm * (H // 2):(mm + 1) * (H // 2), :])


def _pair_weights(wt, j, rows):
    w = wt[pl.ds(j * (rows + 1), rows), :]
    lo = pltpu.bitcast(w << 16, f32).astype(bf16)
    hi = pltpu.bitcast(w & jnp.uint32(0xFFFF0000), f32).astype(bf16)
    return jnp.concatenate([lo, hi], axis=1)


def _b_proj_parts(p0, ws, bxp, cp, qb, kb, vb, slot0):
    wq, wk, wv = ws
    rows = pl.ds(p0, TP // 2)

    def put(dst, y):
        for e in range(2):
            dst[slot0 + e, rows, :] = _pack(y[:, e * D:(e + 1) * D].astype(bf16))

    return [
        lambda: put(qb, _dot(_unpack(bxp[rows, :]), wq) * ((D ** -0.5) * LOG2E)),
        lambda: put(kb, _dot(_unpack(cp[rows, :]), wk)),
        lambda: put(vb, _dot(_unpack(cp[rows, :]), wv)),
    ]


HQ = TQ // 2


def _b_qk(i, qa, ka):
    k0 = i * TQ
    n = k0 + HQ
    q = qa[k0:k0 + TQ]
    s = _dot_nt(q, ka[0:n])
    s2 = _dot_nt(q[HQ:], ka[n:n + HQ])
    row = jax.lax.broadcasted_iota(jnp.int32, (HQ, 128), 0)
    col = jax.lax.broadcasted_iota(jnp.int32, (HQ, 128), 1)
    tri = col <= row
    nb = n // 128
    top = [s[:HQ, j * 128:(j + 1) * 128] for j in range(nb)]
    top[-1] = jnp.where(tri, top[-1], NEG)
    bot = [s[HQ:, j * 128:(j + 1) * 128] for j in range(nb)]
    bot.append(jnp.where(tri, s2, NEG))
    mps = []
    for blocks in (top, bot):
        mp = blocks[0]
        for c in blocks[1:]:
            mp = jnp.maximum(mp, c)
        mps.append(mp)
    return (top, bot), mps


def _b_softmax(blocks, mps, prev):
    ps, lps = [], []
    for half in range(2):
        mp = mps[half]
        if prev is not None:
            mp = jnp.maximum(mp, jnp.minimum(prev[half], NEG))
        m = jnp.max(mp, axis=1, keepdims=True)
        lp = None
        pl_ = []
        for jj, c in enumerate(blocks[half]):
            p = jnp.exp2(c - m)
            lp = p if lp is None else lp + p
            if jj == len(blocks[half]) - 1:
                p = p + jnp.minimum(lp, 0.0)
            pl_.append(p.astype(bf16))
        ps.append(pl_)
        lps.append(lp)
    return ps, lps


def _b_pv(i, ps, lps, va, ctx, h):
    k0 = i * TQ
    n = k0 + HQ
    nb = n // 128
    ls = [jnp.sum(lp, axis=1, keepdims=True) for lp in lps]
    pc = jnp.concatenate(
        [jnp.concatenate(ps[0], axis=1), jnp.concatenate(ps[1][:nb], axis=1)], axis=0)
    o = _dot(pc, va[0:n])
    o2 = _dot(ps[1][nb], va[n:n + HQ])
    o_top = o[:HQ] * (1.0 / ls[0])
    o_bot = (o[HQ:] + o2) * (1.0 / ls[1])
    ctx[h, k0 // 2:(k0 + HQ) // 2, :] = _pack(o_top.astype(bf16))
    ctx[h, (k0 + HQ) // 2:(k0 + TQ) // 2, :] = _pack(o_bot.astype(bf16))
    return (o_top, o_bot)


def _b_head(h, slot, qb, kb, vb, ctx, fillers):
    nT = S // TQ
    order = list(range(nT))[::-1]
    qa, ka, va = _unpack(qb[slot]), _unpack(kb[slot]), _unpack(vb[slot])
    cur = _b_qk(order[0], qa, ka)
    prev = None
    for t, i in enumerate(order):
        nxt = _b_qk(order[t + 1], qa, ka) if t + 1 < nT else None
        ps, lps = _b_softmax(cur[0], cur[1], prev)
        for f in fillers.get(t, ()):
            f()
        prev = _b_pv(i, ps, lps, va, ctx, h)
        cur = nxt


def _kernel(ax_h, wqkv_h, wo_h, bx_h, c_h, wq_h, wuk_h, wuv_h, wob_h, out_h,
            wob_v, wop, op, qp, kp, vp,
            wq_t, wk_t, wv_t, bxp, cp, out_s,
            sem_w, sem_ax, sem_f, sem_wob, sem_out):
    NR = S // TA

    def rows(ref, r, n):
        return ref.at[pl.ds(pl.multiple_of(r * n, n), n), :]

    wob_copy = pltpu.make_async_copy(wob_h, wob_v, sem_wob)

    def phase_a(ax_v, wqkv_v, wo_v, stage, wtp, bx_v, c_v, wq_raw, wuk_raw, wuv_raw):
        def w_copy(r):
            return pltpu.make_async_copy(rows(wqkv_h, r, 128), rows(wqkv_v, r, 128),
                                         sem_w.at[r])

        def ax_copy(r):
            return pltpu.make_async_copy(rows(ax_h, r, TA), rows(ax_v, r, TA),
                                         sem_ax.at[r])

        def f_copies(r):
            return [
                pltpu.make_async_copy(rows(wq_h, r, M * H // NR),
                                      rows(wq_raw, r, M * H // NR), sem_f.at[6 * r]),
                pltpu.make_async_copy(rows(wuk_h, r, C * H // NR),
                                      rows(wuk_raw, r, C * H // NR), sem_f.at[6 * r + 1]),
                pltpu.make_async_copy(rows(wuv_h, r, C * H // NR),
                                      rows(wuv_raw, r, C * H // NR), sem_f.at[6 * r + 2]),
                pltpu.make_async_copy(rows(bx_h, r, TA), rows(bx_v, r, TA),
                                      sem_f.at[6 * r + 3]),
                pltpu.make_async_copy(rows(c_h, r, TA), rows(c_v, r, TA),
                                      sem_f.at[6 * r + 4]),
            ]

        def wo_copy(r):
            c0 = pl.multiple_of(r * 128, 128)
            return pltpu.make_async_copy(wo_h.at[:, pl.ds(c0, 128)], wo_v.at[r],
                                         sem_f.at[6 * r + 5])

        for r in range(NR):
            w_copy(r).start()
        ax_copy(0).start()
        for ref in (kp, vp):
            ref[:, 0:PADR, :] = jnp.zeros((8, PADR, 128), f32)
        _prep_wqkv(wqkv_v, stage, wtp, lambda rb: w_copy(rb).wait())
        ax_copy(1).start()
        for cpy in f_copies(0):
            cpy.start()
        wo_copy(0).start()

        def body(r, carry):
            ax_copy(r).wait()

            @pl.when(r + 2 < NR)
            def _():
                ax_copy(r + 2).start()

            @pl.when(r + 1 < NR)
            def _():
                for cpy in f_copies(r + 1):
                    cpy.start()
                wo_copy(r + 1).start()
            for piece in range(3 * DA // NB):
                _a_proj_piece(r, piece, ax_v, wtp, qp, kp, vp)
            for g in range(TA // GA):
                _a_attn_group(r * TA + g * GA, qp, kp, vp, op)
            return carry

        jax.lax.fori_loop(0, NR, body, 0)
        wob_copy.start()

        for r in range(NR):
            for cpy in f_copies(r):
                cpy.wait()
            wo_copy(r).wait()

        def prep(r, carry):
            for i in range(16):
                _deinterleave_block(r * 16 + i, wq_raw, wq_t, M)
            for i in range(8):
                _deinterleave_block(r * 8 + i, wuk_raw, wk_t, C)
                _deinterleave_block(r * 8 + i, wuv_raw, wv_t, C)
            src = pl.ds(pl.multiple_of(r * TA, TA), TA)
            dst = pl.ds(pl.multiple_of(r * (TA // 2), TA // 2), TA // 2)
            bxp[dst, :] = _pack(bx_v[src, :])
            cp[dst, :] = _pack(c_v[src, :])
            _prep_wo_block(r, wo_v, stage, wop)
            return carry

        jax.lax.fori_loop(0, NR, prep, 0)

    pl.run_scoped(
        phase_a,
        pltpu.VMEM((S, DA), bf16), pltpu.VMEM((DA, 3 * DA), bf16),
        pltpu.VMEM((8, DA, 128), bf16), pltpu.VMEM((3 * HA * DP, 128), f32),
        pltpu.VMEM((8, 3 * DA // 2, 128), u32),
        pltpu.VMEM((S, M), bf16), pltpu.VMEM((S, C), bf16),
        pltpu.VMEM((M * H, D), bf16), pltpu.VMEM((C * H, D), bf16),
        pltpu.VMEM((C * H, D), bf16))

    def phase_b(qb, kb, vb, ctx):
        def weights(j):
            return (_pair_weights(wq_t, j, M), _pair_weights(wk_t, j, C),
                    _pair_weights(wv_t, j, C))

        ws0 = weights(0)
        for r in range(S // TP):
            for f in _b_proj_parts(r * (TP // 2), ws0, bxp, cp, qb, kb, vb, 0):
                f()

        def body(h, carry):
            e = h % 2
            ws = weights(h // 2 + 1)
            wslot = 2 * ((h // 2 + 1) % 2)
            half = S // 4
            nf = S // TP // 2
            fillers = {
                S // TQ - nf + r: _b_proj_parts(
                    pl.multiple_of(e * half + r * (TP // 2), TP // 2),
                    ws, bxp, cp, qb, kb, vb, wslot)
                for r in range(nf)}
            _b_head(h, h % 4, qb, kb, vb, ctx, fillers)
            return carry

        jax.lax.fori_loop(0, H - 2, body, 0)

        def tail(h, carry):
            _b_head(h, h % 4, qb, kb, vb, ctx, {})
            return carry

        jax.lax.fori_loop(H - 2, H, tail, 0)

        wob_copy.wait()

        def out_copy(r):
            r0 = pl.multiple_of(r * TO, TO)
            return pltpu.make_async_copy(
                out_s.at[pl.ds(r0, TO), :], out_h.at[pl.ds(r0, TO), :], sem_out)

        def obody(r, carry):
            r0 = pl.multiple_of(r * TO, TO)
            p0 = pl.multiple_of(r * (TO // 2), TO // 2)
            oa = _unpack(op[pl.ds(p0, TO // 2), :])
            woa = jnp.concatenate([_unpack(wop[nb]) for nb in range(8)], axis=1)
            out_s[pl.ds(r0, TO), 0:DA] = _dot(oa, woa).astype(bf16)
            cb = jnp.concatenate(
                [_unpack(ctx[h, pl.ds(p0, TO // 2), :]) for h in range(H)], axis=1)
            out_s[pl.ds(r0, TO), DA:DA + M] = _dot(cb, wob_v[...]).astype(bf16)
            out_copy(r).start()
            return carry

        jax.lax.fori_loop(0, S // TO, obody, 0)
        for r in range(S // TO):
            out_copy(r).wait()

    pl.run_scoped(
        phase_b,
        pltpu.VMEM((4, S // 2, D), u32), pltpu.VMEM((4, S // 2, D), u32),
        pltpu.VMEM((4, S // 2, D), u32), pltpu.VMEM((H, S // 2, D), u32))


@jax.jit
def pallas_concat_heads__sliding_local_dilated__compressed_kv_cla__prompt_kernel(
    A_x: jax.Array,
    A_wqkv: jax.Array,
    A_wo: jax.Array,
    B_x: jax.Array,
    B_c_kv: jax.Array,
    B_w_q: jax.Array,
    B_w_uk: jax.Array,
    B_w_uv: jax.Array,
    B_w_o: jax.Array,
):
    any_spec = pl.BlockSpec(memory_space=pl.ANY)
    out = pl.pallas_call(
        _kernel,
        out_shape=jax.ShapeDtypeStruct((S, DA + M), bf16),
        in_specs=[any_spec] * 9,
        out_specs=any_spec,
        scratch_shapes=[
            pltpu.VMEM((H * D, M), bf16),
            pltpu.VMEM((8, DA // 2, 128), u32),
            pltpu.VMEM((S // 2, DA), u32),
            pltpu.VMEM((8, S + PADR, 128), f32),
            pltpu.VMEM((8, S + PADR, 128), f32),
            pltpu.VMEM((8, S + PADR, 128), f32),
            pltpu.VMEM((H // 2 * (M + 1), D), u32),
            pltpu.VMEM((H // 2 * (C + 1), D), u32),
            pltpu.VMEM((H // 2 * (C + 1), D), u32),
            pltpu.VMEM((S // 2, M), u32),
            pltpu.VMEM((S // 2, C), u32),
            pltpu.VMEM((S, DA + M), bf16),
            pltpu.SemaphoreType.DMA((8,)),
            pltpu.SemaphoreType.DMA((8,)),
            pltpu.SemaphoreType.DMA((48,)),
            pltpu.SemaphoreType.DMA(()),
            pltpu.SemaphoreType.DMA(()),
        ],
        compiler_params=pltpu.CompilerParams(vmem_limit_bytes=120 * 1024 * 1024),
    )(
        A_x.reshape(S, DA), A_wqkv, A_wo,
        B_x.reshape(S, M), B_c_kv.reshape(S, C),
        B_w_q.reshape(M * H, D), B_w_uk.reshape(C * H, D), B_w_uv.reshape(C * H, D),
        B_w_o.reshape(H * D, M),
    )
    return out.reshape(1, S, DA + M)
```

```python
import math

import jax
import jax.numpy as jnp
import jax.experimental.pallas as pl
import jax.experimental.pallas.tpu as pltpu

bf16 = jnp.bfloat16
f32 = jnp.float32
u32 = jnp.uint32

S = 2048
DA = 1024
HA = 32
DH = 32
WIN = 8
DIL = 2
M = 1024
C = 512
H = 32
D = 128
LOG2E = math.log2(math.e)
NEG = -1e30
PADR = 16
DP = HA + 1
TA = 512
TQ = 256
TP = 256
TO = 256
NT = (((1,), (1,)), ((), ()))


def _unpack(x):
    return pltpu.bitcast(x, bf16)


def _pack(x):
    return pltpu.bitcast(x, u32)


def _dot(a, b):
    return jnp.dot(a, b, preferred_element_type=f32)


def _dot_nt(a, b):
    return jax.lax.dot_general(a, b, NT, preferred_element_type=f32)


def _prep_w_block(t, rb, wqkv_v, stage, wtp):
    r0 = pl.multiple_of(rb * 128, 128)
    for cb in range(8):
        c0 = t * DA + cb * 128
        tile = wqkv_v[pl.ds(r0, 128), c0:c0 + 128].astype(f32).T
        for hl in range(4):
            stage[pl.ds(4 * cb + hl, DH, stride=DP), :] = tile[hl * DH:(hl + 1) * DH, :]
    for d in range(DH):
        rows = stage[pl.ds(d * DP, HA), :]
        o0 = (t * DA + d * HA) // 2
        wtp[rb, o0:o0 + HA // 2, :] = _pack(rows.astype(bf16))


def _prep_wo_block(nb, wo_v, stage, wop):
    for h in range(HA):
        rows = wo_v[nb, h * DH:(h + 1) * DH, :].astype(f32)
        stage[pl.ds(h, DH, stride=DP), :] = rows
    for d in range(DH):
        rows = stage[pl.ds(d * DP, HA), :]
        wop[nb, d * (HA // 2):(d + 1) * (HA // 2), :] = _pack(rows.astype(bf16))


NB = 512


def _a_proj(t, r, ax_v, wtp, dst):
    r0 = pl.multiple_of(r * TA, TA)
    x = ax_v[pl.ds(r0, TA), :]
    for n in range(DA // NB):
        f0 = (t * DA + n * NB) // 2
        w = jnp.concatenate(
            [_unpack(wtp[rb, f0:f0 + NB // 2, :]) for rb in range(8)], axis=1)
        y = _dot_nt(x, w)
        if t == 0:
            y = y * ((DH ** -0.5) * LOG2E)
        for cc in range(NB // 128):
            dst[n * (NB // 128) + cc, pl.ds(r0 + PADR, TA), :] = (
                y[:, cc * 128:(cc + 1) * 128])


GA = 16


def _a_attn_group(row0, qp, kp, vp, op, masked):
    G = GA
    q = [qp[c, pl.ds(row0 + PADR, G), :] for c in range(8)]
    if masked:
        pos = row0 + jax.lax.broadcasted_iota(jnp.int32, (G, 128), 0)
    logits = []
    for w in range(WIN):
        z = None
        for c in range(8):
            p = q[c] * kp[c, pl.ds(row0 + PADR - DIL * w, G), :]
            z = p if z is None else z + p
        z = z + pltpu.roll(z, 64, 1)
        z = z + pltpu.roll(z, 32, 1)
        if masked and w > 0:
            z = jnp.where(pos >= DIL * w, z, NEG)
        logits.append(z)
    m = logits[0]
    for w in range(1, WIN):
        m = jnp.maximum(m, logits[w])
    es = [jnp.exp2(z - m) for z in logits]
    l = es[0]
    for w in range(1, WIN):
        l = l + es[w]
    inv = 1.0 / l
    attn = [e * inv for e in es]
    o0 = pl.multiple_of(row0 // 2, G // 2)
    for c in range(8):
        acc = None
        for w in range(WIN):
            v = vp[c, pl.ds(row0 + PADR - DIL * w, G), :]
            acc = attn[w] * v if acc is None else acc + attn[w] * v
        op[pl.ds(o0, G // 2), c * 128:(c + 1) * 128] = _pack(acc.astype(bf16))


def _deinterleave_block(mb, raw, dst, rows):
    pitch = rows + 1
    base = pl.multiple_of(mb * 8, 8)
    blk = _pack(raw[pl.ds(pl.multiple_of(base * H, 8 * H), 8 * H), :])
    for mm in range(8):
        dst[pl.ds(base + mm, H // 2, stride=pitch), :] = (
            blk[mm * (H // 2):(mm + 1) * (H // 2), :])


def _pair_weights(wt, j, rows):
    w = wt[pl.ds(j * (rows + 1), rows), :]
    lo = pltpu.bitcast(w << 16, f32).astype(bf16)
    hi = pltpu.bitcast(w & jnp.uint32(0xFFFF0000), f32).astype(bf16)
    return jnp.concatenate([lo, hi], axis=1)


def _b_proj_parts(p0, ws, bxp, cp, qb, kb, vb, slot0):
    wq, wk, wv = ws
    rows = pl.ds(p0, TP // 2)

    def put(dst, y):
        for e in range(2):
            dst[slot0 + e, rows, :] = _pack(y[:, e * D:(e + 1) * D].astype(bf16))

    return [
        lambda: put(qb, _dot(_unpack(bxp[rows, :]), wq) * ((D ** -0.5) * LOG2E)),
        lambda: put(kb, _dot(_unpack(cp[rows, :]), wk)),
        lambda: put(vb, _dot(_unpack(cp[rows, :]), wv)),
    ]


HQ = TQ // 2


def _b_qk(i, qa, ka):
    k0 = i * TQ
    n = k0 + HQ
    q = qa[k0:k0 + TQ]
    s = _dot_nt(q, ka[0:n])
    s2 = _dot_nt(q[HQ:], ka[n:n + HQ])
    row = jax.lax.broadcasted_iota(jnp.int32, (HQ, 128), 0)
    col = jax.lax.broadcasted_iota(jnp.int32, (HQ, 128), 1)
    tri = col <= row
    nb = n // 128
    top = [s[:HQ, j * 128:(j + 1) * 128] for j in range(nb)]
    top[-1] = jnp.where(tri, top[-1], NEG)
    bot = [s[HQ:, j * 128:(j + 1) * 128] for j in range(nb)]
    bot.append(jnp.where(tri, s2, NEG))
    mps = []
    for blocks in (top, bot):
        mp = blocks[0]
        for c in blocks[1:]:
            mp = jnp.maximum(mp, c)
        mps.append(mp)
    return (top, bot), mps


def _b_softmax(blocks, mps, prev):
    ps, lps = [], []
    for half in range(2):
        mp = mps[half]
        if prev is not None:
            mp = jnp.maximum(mp, jnp.minimum(prev[half], NEG))
        m = jnp.max(mp, axis=1, keepdims=True)
        lp = None
        pl_ = []
        for jj, c in enumerate(blocks[half]):
            p = jnp.exp2(c - m)
            lp = p if lp is None else lp + p
            if jj == len(blocks[half]) - 1:
                p = p + jnp.minimum(lp, 0.0)
            pl_.append(p.astype(bf16))
        ps.append(pl_)
        lps.append(lp)
    return ps, lps


def _b_pv(i, ps, lps, va, ctx, h):
    k0 = i * TQ
    n = k0 + HQ
    nb = n // 128
    ls = [jnp.sum(lp, axis=1, keepdims=True) for lp in lps]
    pc = jnp.concatenate(
        [jnp.concatenate(ps[0], axis=1), jnp.concatenate(ps[1][:nb], axis=1)], axis=0)
    o = _dot(pc, va[0:n])
    o2 = _dot(ps[1][nb], va[n:n + HQ])
    o_top = o[:HQ] * (1.0 / ls[0])
    o_bot = (o[HQ:] + o2) * (1.0 / ls[1])
    ctx[h, k0 // 2:(k0 + HQ) // 2, :] = _pack(o_top.astype(bf16))
    ctx[h, (k0 + HQ) // 2:(k0 + TQ) // 2, :] = _pack(o_bot.astype(bf16))
    return (o_top, o_bot)


def _b_head(h, slot, qb, kb, vb, ctx, fillers):
    nT = S // TQ
    order = list(range(nT))[::-1]
    qa, ka, va = _unpack(qb[slot]), _unpack(kb[slot]), _unpack(vb[slot])
    cur = _b_qk(order[0], qa, ka)
    prev = None
    for t, i in enumerate(order):
        nxt = _b_qk(order[t + 1], qa, ka) if t + 1 < nT else None
        ps, lps = _b_softmax(cur[0], cur[1], prev)
        for f in fillers.get(t, ()):
            f()
        prev = _b_pv(i, ps, lps, va, ctx, h)
        cur = nxt


def _kernel(ax_h, wqkv_h, wo_h, bx_h, c_h, wq_h, wuk_h, wuv_h, wob_h, out_h,
            qb, kb, vb, wop, op, qp, kp, vp,
            wq_t, wk_t, wv_t, bxp, cp, out_s,
            sem_w, sem_ax, sem_f, sem_wob, sem_out):
    NR = S // TA

    def rows(ref, r, n):
        return ref.at[pl.ds(pl.multiple_of(r * n, n), n), :]

    def phase_a(ax_v, wqkv_v, wo_v, stage, wtp, bx_v, c_v, wq_raw, wuk_raw, wuv_raw):
        def w_copy(t, rb):
            r0 = pl.multiple_of(rb * 128, 128)
            sl = (pl.ds(r0, 128), slice(t * DA, (t + 1) * DA))
            return pltpu.make_async_copy(wqkv_h.at[sl], wqkv_v.at[sl],
                                         sem_w.at[8 * t + rb])

        def ax_copy(r):
            return pltpu.make_async_copy(rows(ax_h, r, TA), rows(ax_v, r, TA),
                                         sem_ax.at[r])

        def f_copy(r, i):
            sem = sem_f.at[7 * r + i]
            if i < 3:
                src, dst, n = ((wq_h, wq_raw, M), (wuk_h, wuk_raw, C),
                               (wuv_h, wuv_raw, C))[i]
                n = n * H // NR
                return pltpu.make_async_copy(rows(src, r, n), rows(dst, r, n), sem)
            if i < 5:
                src, dst = ((bx_h, bx_v), (c_h, c_v))[i - 3]
                return pltpu.make_async_copy(rows(src, r, TA), rows(dst, r, TA), sem)
            nb = 2 * r + (i - 5)
            c0 = pl.multiple_of(nb * 128, 128)
            return pltpu.make_async_copy(wo_h.at[:, pl.ds(c0, 128)], wo_v.at[nb], sem)

        sched = {
            0: [lambda: ax_copy(1), lambda: w_copy(1, 2), lambda: w_copy(1, 3)],
            1: [lambda: ax_copy(2), lambda: w_copy(1, 4), lambda: w_copy(1, 5)],
            2: [lambda: ax_copy(3), lambda: w_copy(1, 6), lambda: w_copy(1, 7)],
            3: [lambda: w_copy(2, 0), lambda: w_copy(2, 1)],
            4: [lambda: w_copy(2, 2), lambda: w_copy(2, 3)],
            5: [lambda: w_copy(2, 4), lambda: w_copy(2, 5)],
            6: [lambda: w_copy(2, 6), lambda: w_copy(2, 7)],
        }
        fslots = [
            [(0, 0)], [(0, 1), (0, 2), (0, 4)], [(0, 3), (0, 5), (0, 6), (1, 1)],
            [(1, 0), (1, 2)], [(1, 3), (1, 4), (1, 5), (1, 6), (2, 1)],
            [(2, 0), (2, 2)], [(2, 3), (2, 4), (2, 5), (2, 6)],
            [(3, 0), (3, 1)], [(3, 2), (3, 3), (3, 4), (3, 5), (3, 6)],
        ]
        for slot, items in enumerate(fslots):
            sched.setdefault(slot, []).extend(
                (lambda r=r, i=i: f_copy(r, i)) for r, i in items)

        def issue(t, r):
            for k in range(NR):
                items = sched.get(NR * t + k, [])
                if items:
                    @pl.when(r == k)
                    def _():
                        for mk in items:
                            mk().start()

        for rb in range(8):
            w_copy(0, rb).start()
        ax_copy(0).start()
        w_copy(1, 0).start()
        w_copy(1, 1).start()
        for ref in (kp, vp):
            ref[:, 0:PADR, :] = jnp.zeros((8, PADR, 128), f32)

        def prep0(rb, carry):
            w_copy(0, rb).wait()
            _prep_w_block(0, rb, wqkv_v, stage.at[0], wtp)
            return carry

        jax.lax.fori_loop(0, 8, prep0, 0)

        def qk_step(t):
            def body(r, carry):
                if t == 0:
                    ax_copy(r).wait()
                w_copy(t + 1, 2 * r).wait()
                w_copy(t + 1, 2 * r + 1).wait()
                issue(t, r)
                _a_proj(t, r, ax_v, wtp, (qp, kp)[t])
                for i in range(2):
                    _prep_w_block(t + 1, 2 * r + i, wqkv_v, stage.at[i], wtp)
                return carry
            return body

        jax.lax.fori_loop(0, NR, qk_step(0), 0)
        jax.lax.fori_loop(0, NR, qk_step(1), 0)

        def v_step(r, carry):
            for i in range(7):
                f_copy(r, i).wait()
            issue(2, r)
            _a_proj(2, r, ax_v, wtp, vp)
            nq = M // 8 // NR
            nk = C // 8 // NR
            for i in range(nq):
                _deinterleave_block(r * nq + i, wq_raw, wq_t, M)
            for i in range(nk):
                _deinterleave_block(r * nk + i, wuk_raw, wk_t, C)
                _deinterleave_block(r * nk + i, wuv_raw, wv_t, C)
            src = pl.ds(pl.multiple_of(r * TA, TA), TA)
            dst = pl.ds(pl.multiple_of(r * (TA // 2), TA // 2), TA // 2)
            bxp[dst, :] = _pack(bx_v[src, :])
            cp[dst, :] = _pack(c_v[src, :])
            for i in range(2):
                _prep_wo_block(2 * r + i, wo_v, stage.at[i], wop)
            return carry

        jax.lax.fori_loop(0, NR, v_step, 0)

    pl.run_scoped(
        phase_a,
        pltpu.VMEM((S, DA), bf16), pltpu.VMEM((DA, 3 * DA), bf16),
        pltpu.VMEM((8, DA, 128), bf16), pltpu.VMEM((2, HA * DP, 128), f32),
        pltpu.VMEM((8, 3 * DA // 2, 128), u32),
        pltpu.VMEM((S, M), bf16), pltpu.VMEM((S, C), bf16),
        pltpu.VMEM((M * H, D), bf16), pltpu.VMEM((C * H, D), bf16),
        pltpu.VMEM((C * H, D), bf16))

    def phase_b(ctx, wob_v):
        wob_copy = pltpu.make_async_copy(wob_h, wob_v, sem_wob)
        wob_copy.start()

        def weights(j):
            return (_pair_weights(wq_t, j, M), _pair_weights(wk_t, j, C),
                    _pair_weights(wv_t, j, C))

        half = S // 4
        nf = S // TP // 2
        ga = 4

        def first(e, carry):
            ws = weights(0)
            for r in range(nf):
                p0 = pl.multiple_of(e * half + r * (TP // 2), TP // 2)
                for f in _b_proj_parts(p0, ws, bxp, cp, qb, kb, vb, 0):
                    f()
                _a_attn_group((e * ga + r) * GA, qp, kp, vp, op, True)
            return carry

        jax.lax.fori_loop(0, 2, first, 0)

        def body(h, carry):
            e = h % 2
            ws = weights(h // 2 + 1)
            wslot = 2 * ((h // 2 + 1) % 2)
            fillers = {}
            for r in range(nf):
                p0 = pl.multiple_of(e * half + r * (TP // 2), TP // 2)
                fillers[S // TQ - nf + r] = _b_proj_parts(
                    p0, ws, bxp, cp, qb, kb, vb, wslot) + [
                        lambda r=r: _a_attn_group(((h + 2) * ga + r) * GA,
                                                  qp, kp, vp, op, False)]
            _b_head(h, h % 4, qb, kb, vb, ctx, fillers)
            return carry

        jax.lax.fori_loop(0, H - 2, body, 0)

        def out_a(r):
            r0 = pl.multiple_of(r * TO, TO)
            p0 = pl.multiple_of(r * (TO // 2), TO // 2)
            oa = _unpack(op[pl.ds(p0, TO // 2), :])
            woa = jnp.concatenate([_unpack(wop[nb]) for nb in range(8)], axis=1)
            out_s[pl.ds(r0, TO), 0:DA] = _dot(oa, woa).astype(bf16)

        def tail(h, carry):
            fillers = {
                S // TQ - nf + r: [lambda r=r: out_a((h - (H - 2)) * nf + r)]
                for r in range(nf)}
            _b_head(h, h % 4, qb, kb, vb, ctx, fillers)
            return carry

        jax.lax.fori_loop(H - 2, H, tail, 0)

        wob_copy.wait()

        def out_copy(r):
            r0 = pl.multiple_of(r * TO, TO)
            return pltpu.make_async_copy(
                out_s.at[pl.ds(r0, TO), :], out_h.at[pl.ds(r0, TO), :], sem_out)

        def obody(r, carry):
            r0 = pl.multiple_of(r * TO, TO)
            p0 = pl.multiple_of(r * (TO // 2), TO // 2)
            cb = jnp.concatenate(
                [_unpack(ctx[h, pl.ds(p0, TO // 2), :]) for h in range(H)], axis=1)
            out_s[pl.ds(r0, TO), DA:DA + M] = _dot(cb, wob_v[...]).astype(bf16)
            out_copy(r).start()
            return carry

        jax.lax.fori_loop(0, S // TO, obody, 0)
        for r in range(S // TO):
            out_copy(r).wait()

    pl.run_scoped(
        phase_b,
        pltpu.VMEM((H, S // 2, D), u32), pltpu.VMEM((H * D, M), bf16))


@jax.jit
def pallas_concat_heads__sliding_local_dilated__compressed_kv_cla__prompt_kernel(
    A_x: jax.Array,
    A_wqkv: jax.Array,
    A_wo: jax.Array,
    B_x: jax.Array,
    B_c_kv: jax.Array,
    B_w_q: jax.Array,
    B_w_uk: jax.Array,
    B_w_uv: jax.Array,
    B_w_o: jax.Array,
):
    any_spec = pl.BlockSpec(memory_space=pl.ANY)
    out = pl.pallas_call(
        _kernel,
        out_shape=jax.ShapeDtypeStruct((S, DA + M), bf16),
        in_specs=[any_spec] * 9,
        out_specs=any_spec,
        scratch_shapes=[
            pltpu.VMEM((4, S // 2, D), u32),
            pltpu.VMEM((4, S // 2, D), u32),
            pltpu.VMEM((4, S // 2, D), u32),
            pltpu.VMEM((8, DA // 2, 128), u32),
            pltpu.VMEM((S // 2, DA), u32),
            pltpu.VMEM((8, S + PADR, 128), f32),
            pltpu.VMEM((8, S + PADR, 128), f32),
            pltpu.VMEM((8, S + PADR, 128), f32),
            pltpu.VMEM((H // 2 * (M + 1), D), u32),
            pltpu.VMEM((H // 2 * (C + 1), D), u32),
            pltpu.VMEM((H // 2 * (C + 1), D), u32),
            pltpu.VMEM((S // 2, M), u32),
            pltpu.VMEM((S // 2, C), u32),
            pltpu.VMEM((S, DA + M), bf16),
            pltpu.SemaphoreType.DMA((24,)),
            pltpu.SemaphoreType.DMA((4,)),
            pltpu.SemaphoreType.DMA((28,)),
            pltpu.SemaphoreType.DMA(()),
            pltpu.SemaphoreType.DMA(()),
        ],
        compiler_params=pltpu.CompilerParams(vmem_limit_bytes=120 * 1024 * 1024),
    )(
        A_x.reshape(S, DA), A_wqkv, A_wo,
        B_x.reshape(S, M), B_c_kv.reshape(S, C),
        B_w_q.reshape(M * H, D), B_w_uk.reshape(C * H, D), B_w_uv.reshape(C * H, D),
        B_w_o.reshape(H * D, M),
    )
    return out.reshape(1, S, DA + M)
```

```python
import math

import jax
import jax.numpy as jnp
import jax.experimental.pallas as pl
import jax.experimental.pallas.tpu as pltpu

bf16 = jnp.bfloat16
f32 = jnp.float32
u32 = jnp.uint32

S = 2048
DA = 1024
HA = 32
DH = 32
WIN = 8
DIL = 2
M = 1024
C = 512
H = 32
D = 128
LOG2E = math.log2(math.e)
NEG = -1e30
PADR = 16
DP = HA + 1
TA = 512
TQ = 256
TP = 256
TO = 256
NT = (((1,), (1,)), ((), ()))


def _unpack(x):
    return pltpu.bitcast(x, bf16)


def _pack(x):
    return pltpu.bitcast(x, u32)


def _dot(a, b):
    return jnp.dot(a, b, preferred_element_type=f32)


def _dot_nt(a, b):
    return jax.lax.dot_general(a, b, NT, preferred_element_type=f32)


def _prep_w_block(t, rb, wqkv_v, stage, wtp):
    r0 = pl.multiple_of(rb * 128, 128)
    for cb in range(8):
        c0 = t * DA + cb * 128
        tile = wqkv_v[pl.ds(r0, 128), c0:c0 + 128].astype(f32).T
        for hl in range(4):
            stage[pl.ds(4 * cb + hl, DH, stride=DP), :] = tile[hl * DH:(hl + 1) * DH, :]
    for d in range(DH):
        rows = stage[pl.ds(d * DP, HA), :]
        o0 = (t * DA + d * HA) // 2
        wtp[rb, o0:o0 + HA // 2, :] = _pack(rows.astype(bf16))


def _prep_wo_block(nb, wo_v, stage, wop):
    for h in range(HA):
        rows = wo_v[nb, h * DH:(h + 1) * DH, :].astype(f32)
        stage[pl.ds(h, DH, stride=DP), :] = rows
    for d in range(DH):
        rows = stage[pl.ds(d * DP, HA), :]
        wop[nb, d * (HA // 2):(d + 1) * (HA // 2), :] = _pack(rows.astype(bf16))


NB = 512


def _a_proj(t, r, ax_v, wtp, dst):
    r0 = pl.multiple_of(r * TA, TA)
    x = ax_v[pl.ds(r0, TA), :]
    for n in range(DA // NB):
        f0 = (t * DA + n * NB) // 2
        w = jnp.concatenate(
            [_unpack(wtp[rb, f0:f0 + NB // 2, :]) for rb in range(8)], axis=1)
        y = _dot_nt(x, w)
        if t == 0:
            y = y * ((DH ** -0.5) * LOG2E)
        for cc in range(NB // 128):
            dst[n * (NB // 128) + cc, pl.ds(r0 + PADR, TA), :] = (
                y[:, cc * 128:(cc + 1) * 128])


GA = 16


def _a_attn_rows(row0, qp, kp, vp, masked):
    G = 8
    q = [qp[c, pl.ds(row0 + PADR, G), :] for c in range(8)]
    if masked:
        pos = row0 + jax.lax.broadcasted_iota(jnp.int32, (G, 128), 0)
    logits = []
    for w in range(WIN):
        z = None
        for c in range(8):
            p = q[c] * kp[c, pl.ds(row0 + PADR - DIL * w, G), :]
            z = p if z is None else z + p
        z = z + pltpu.roll(z, 64, 1)
        z = z + pltpu.roll(z, 32, 1)
        if masked and w > 0:
            z = jnp.where(pos >= DIL * w, z, NEG)
        logits.append(z)
    m = logits[0]
    for w in range(1, WIN):
        m = jnp.maximum(m, logits[w])
    es = [jnp.exp2(z - m) for z in logits]
    l = es[0]
    for w in range(1, WIN):
        l = l + es[w]
    inv = 1.0 / l
    attn = [e * inv for e in es]
    outs = []
    for c in range(8):
        acc = None
        for w in range(WIN):
            v = vp[c, pl.ds(row0 + PADR - DIL * w, G), :]
            acc = attn[w] * v if acc is None else acc + attn[w] * v
        outs.append(acc)
    return outs


def _a_attn_group(row0, qp, kp, vp, op, masked):
    a = _a_attn_rows(row0, qp, kp, vp, masked)
    b = _a_attn_rows(row0 + 8, qp, kp, vp, masked)
    o0 = pl.multiple_of(row0 // 2, GA // 2)
    for c in range(8):
        op[pl.ds(o0, GA // 2), c * 128:(c + 1) * 128] = _pack(
            jnp.concatenate([a[c], b[c]], axis=0).astype(bf16))


def _deinterleave_block(mb, raw, dst, rows):
    pitch = rows + 1
    base = pl.multiple_of(mb * 8, 8)
    blk = _pack(raw[pl.ds(pl.multiple_of(base * H, 8 * H), 8 * H), :])
    for mm in range(8):
        dst[pl.ds(base + mm, H // 2, stride=pitch), :] = (
            blk[mm * (H // 2):(mm + 1) * (H // 2), :])


def _pair_weights(wt, j, rows):
    w = wt[pl.ds(j * (rows + 1), rows), :]
    lo = pltpu.bitcast(w << 16, f32).astype(bf16)
    hi = pltpu.bitcast(w & jnp.uint32(0xFFFF0000), f32).astype(bf16)
    return jnp.concatenate([lo, hi], axis=1)


def _b_proj_parts(p0, ws, bxp, cp, qb, kb, vb, slot0):
    wq, wk, wv = ws
    rows = pl.ds(p0, TP // 2)

    def put(dst, y):
        for e in range(2):
            dst[slot0 + e, rows, :] = _pack(y[:, e * D:(e + 1) * D].astype(bf16))

    return [
        lambda: put(qb, _dot(_unpack(bxp[rows, :]), wq) * ((D ** -0.5) * LOG2E)),
        lambda: put(kb, _dot(_unpack(cp[rows, :]), wk)),
        lambda: put(vb, _dot(_unpack(cp[rows, :]), wv)),
    ]


HQ = TQ // 2


def _b_qk(i, qa, ka):
    k0 = i * TQ
    n = k0 + HQ
    q = qa[k0:k0 + TQ]
    s = _dot_nt(q, ka[0:n])
    s2 = _dot_nt(q[HQ:], ka[n:n + HQ])
    row = jax.lax.broadcasted_iota(jnp.int32, (HQ, 128), 0)
    col = jax.lax.broadcasted_iota(jnp.int32, (HQ, 128), 1)
    tri = col <= row
    nb = n // 128
    top = [s[:HQ, j * 128:(j + 1) * 128] for j in range(nb)]
    top[-1] = jnp.where(tri, top[-1], NEG)
    bot = [s[HQ:, j * 128:(j + 1) * 128] for j in range(nb)]
    bot.append(jnp.where(tri, s2, NEG))
    mps = []
    for blocks in (top, bot):
        mp = blocks[0]
        for c in blocks[1:]:
            mp = jnp.maximum(mp, c)
        mps.append(mp)
    return (top, bot), mps


def _b_softmax(blocks, mps, prev):
    ps, lps = [], []
    for half in range(2):
        mp = mps[half]
        if prev is not None:
            mp = jnp.maximum(mp, jnp.minimum(prev[half], NEG))
        m = jnp.max(mp, axis=1, keepdims=True)
        lp = None
        pl_ = []
        for jj, c in enumerate(blocks[half]):
            p = jnp.exp2(c - m)
            lp = p if lp is None else lp + p
            if jj == len(blocks[half]) - 1:
                p = p + jnp.minimum(lp, 0.0)
            pl_.append(p.astype(bf16))
        ps.append(pl_)
        lps.append(lp)
    return ps, lps


def _b_pv(i, ps, lps, va, ctx, h):
    k0 = i * TQ
    n = k0 + HQ
    nb = n // 128
    ls = [jnp.sum(lp, axis=1, keepdims=True) for lp in lps]
    pc = jnp.concatenate(
        [jnp.concatenate(ps[0], axis=1), jnp.concatenate(ps[1][:nb], axis=1)], axis=0)
    o = _dot(pc, va[0:n])
    o2 = _dot(ps[1][nb], va[n:n + HQ])
    o_top = o[:HQ] * (1.0 / ls[0])
    o_bot = (o[HQ:] + o2) * (1.0 / ls[1])
    ctx[h, k0 // 2:(k0 + HQ) // 2, :] = _pack(o_top.astype(bf16))
    ctx[h, (k0 + HQ) // 2:(k0 + TQ) // 2, :] = _pack(o_bot.astype(bf16))
    return (o_top, o_bot)


def _b_head(h, slot, qb, kb, vb, ctx, fillers):
    nT = S // TQ
    order = list(range(nT))[::-1]
    qa, ka, va = _unpack(qb[slot]), _unpack(kb[slot]), _unpack(vb[slot])
    cur = _b_qk(order[0], qa, ka)
    prev = None
    for t, i in enumerate(order):
        nxt = _b_qk(order[t + 1], qa, ka) if t + 1 < nT else None
        ps, lps = _b_softmax(cur[0], cur[1], prev)
        for f in fillers.get(t, ()):
            f()
        prev = _b_pv(i, ps, lps, va, ctx, h)
        cur = nxt


def _kernel(ax_h, wqkv_h, wo_h, bx_h, c_h, wq_h, wuk_h, wuv_h, wob_h, out_h,
            qb, kb, vb, wop, op, qp, kp, vp,
            wq_t, wk_t, wv_t, bxp, cp, out_s,
            sem_w, sem_ax, sem_f, sem_wob, sem_out):
    NR = S // TA

    def rows(ref, r, n):
        return ref.at[pl.ds(pl.multiple_of(r * n, n), n), :]

    def phase_a(ax_v, wqkv_v, wo_v, stage, wtp, bx_v, c_v, wq_raw, wuk_raw, wuv_raw):
        def w_copy(t, rb):
            r0 = pl.multiple_of(rb * 128, 128)
            sl = (pl.ds(r0, 128), slice(t * DA, (t + 1) * DA))
            return pltpu.make_async_copy(wqkv_h.at[sl], wqkv_v.at[sl],
                                         sem_w.at[8 * t + rb])

        def ax_copy(r):
            return pltpu.make_async_copy(rows(ax_h, r, TA), rows(ax_v, r, TA),
                                         sem_ax.at[r])

        def f_copy(r, i):
            sem = sem_f.at[7 * r + i]
            if i < 3:
                src, dst, n = ((wq_h, wq_raw, M), (wuk_h, wuk_raw, C),
                               (wuv_h, wuv_raw, C))[i]
                n = n * H // NR
                return pltpu.make_async_copy(rows(src, r, n), rows(dst, r, n), sem)
            if i < 5:
                src, dst = ((bx_h, bx_v), (c_h, c_v))[i - 3]
                return pltpu.make_async_copy(rows(src, r, TA), rows(dst, r, TA), sem)
            nb = 2 * r + (i - 5)
            c0 = pl.multiple_of(nb * 128, 128)
            return pltpu.make_async_copy(wo_h.at[:, pl.ds(c0, 128)], wo_v.at[nb], sem)

        sched = {
            0: [lambda: ax_copy(1), lambda: w_copy(1, 2), lambda: w_copy(1, 3)],
            1: [lambda: ax_copy(2), lambda: w_copy(1, 4), lambda: w_copy(1, 5)],
            2: [lambda: ax_copy(3), lambda: w_copy(1, 6), lambda: w_copy(1, 7)],
            3: [lambda: w_copy(2, 0), lambda: w_copy(2, 1)],
            4: [lambda: w_copy(2, 2), lambda: w_copy(2, 3)],
            5: [lambda: w_copy(2, 4), lambda: w_copy(2, 5)],
            6: [lambda: w_copy(2, 6), lambda: w_copy(2, 7)],
        }
        fslots = [
            [(0, 0)], [(0, 1), (0, 2), (0, 4)], [(0, 3), (0, 5), (0, 6), (1, 1)],
            [(1, 0), (1, 2)], [(1, 3), (1, 4), (1, 5), (1, 6), (2, 1)],
            [(2, 0), (2, 2)], [(2, 3), (2, 4), (2, 5), (2, 6)],
            [(3, 0), (3, 1)], [(3, 2), (3, 3), (3, 4), (3, 5), (3, 6)],
        ]
        for slot, items in enumerate(fslots):
            sched.setdefault(slot, []).extend(
                (lambda r=r, i=i: f_copy(r, i)) for r, i in items)

        def issue(t, r):
            for k in range(NR):
                items = sched.get(NR * t + k, [])
                if items:
                    @pl.when(r == k)
                    def _():
                        for mk in items:
                            mk().start()

        for rb in range(8):
            w_copy(0, rb).start()
        ax_copy(0).start()
        w_copy(1, 0).start()
        w_copy(1, 1).start()
        for ref in (kp, vp):
            ref[:, 0:PADR, :] = jnp.zeros((8, PADR, 128), f32)

        def prep0(rb, carry):
            w_copy(0, rb).wait()
            _prep_w_block(0, rb, wqkv_v, stage.at[0], wtp)
            return carry

        jax.lax.fori_loop(0, 8, prep0, 0)

        def qk_step(t):
            def body(r, carry):
                if t == 0:
                    ax_copy(r).wait()
                w_copy(t + 1, 2 * r).wait()
                w_copy(t + 1, 2 * r + 1).wait()
                issue(t, r)
                _a_proj(t, r, ax_v, wtp, (qp, kp)[t])
                for i in range(2):
                    _prep_w_block(t + 1, 2 * r + i, wqkv_v, stage.at[i], wtp)
                return carry
            return body

        jax.lax.fori_loop(0, NR, qk_step(0), 0)
        jax.lax.fori_loop(0, NR, qk_step(1), 0)

        def v_step(r, carry):
            for i in range(7):
                f_copy(r, i).wait()
            issue(2, r)
            _a_proj(2, r, ax_v, wtp, vp)
            nq = M // 8 // NR
            nk = C // 8 // NR
            for i in range(nq):
                _deinterleave_block(r * nq + i, wq_raw, wq_t, M)
            for i in range(nk):
                _deinterleave_block(r * nk + i, wuk_raw, wk_t, C)
                _deinterleave_block(r * nk + i, wuv_raw, wv_t, C)
            src = pl.ds(pl.multiple_of(r * TA, TA), TA)
            dst = pl.ds(pl.multiple_of(r * (TA // 2), TA // 2), TA // 2)
            bxp[dst, :] = _pack(bx_v[src, :])
            cp[dst, :] = _pack(c_v[src, :])
            for i in range(2):
                _prep_wo_block(2 * r + i, wo_v, stage.at[i], wop)
            return carry

        jax.lax.fori_loop(0, NR, v_step, 0)

    pl.run_scoped(
        phase_a,
        pltpu.VMEM((S, DA), bf16), pltpu.VMEM((DA, 3 * DA), bf16),
        pltpu.VMEM((8, DA, 128), bf16), pltpu.VMEM((2, HA * DP, 128), f32),
        pltpu.VMEM((8, 3 * DA // 2, 128), u32),
        pltpu.VMEM((S, M), bf16), pltpu.VMEM((S, C), bf16),
        pltpu.VMEM((M * H, D), bf16), pltpu.VMEM((C * H, D), bf16),
        pltpu.VMEM((C * H, D), bf16))

    def phase_b(ctx, wob_v):
        wob_copy = pltpu.make_async_copy(wob_h, wob_v, sem_wob)
        wob_copy.start()

        def weights(j):
            return (_pair_weights(wq_t, j, M), _pair_weights(wk_t, j, C),
                    _pair_weights(wv_t, j, C))

        half = S // 4
        nf = S // TP // 2
        ga = 4

        def first(e, carry):
            ws = weights(0)
            for r in range(nf):
                p0 = pl.multiple_of(e * half + r * (TP // 2), TP // 2)
                for f in _b_proj_parts(p0, ws, bxp, cp, qb, kb, vb, 0):
                    f()
                _a_attn_group((e * ga + r) * GA, qp, kp, vp, op, True)
            return carry

        jax.lax.fori_loop(0, 2, first, 0)

        def body(h, carry):
            e = h % 2
            ws = weights(h // 2 + 1)
            wslot = 2 * ((h // 2 + 1) % 2)
            fillers = {}
            for r in range(nf):
                p0 = pl.multiple_of(e * half + r * (TP // 2), TP // 2)
                fillers[S // TQ - nf + r] = _b_proj_parts(
                    p0, ws, bxp, cp, qb, kb, vb, wslot) + [
                        lambda r=r: _a_attn_group(((h + 2) * ga + r) * GA,
                                                  qp, kp, vp, op, False)]
            _b_head(h, h % 4, qb, kb, vb, ctx, fillers)
            return carry

        jax.lax.fori_loop(0, H - 2, body, 0)

        def out_a(r):
            r0 = pl.multiple_of(r * TO, TO)
            p0 = pl.multiple_of(r * (TO // 2), TO // 2)
            oa = _unpack(op[pl.ds(p0, TO // 2), :])
            woa = jnp.concatenate([_unpack(wop[nb]) for nb in range(8)], axis=1)
            out_s[pl.ds(r0, TO), 0:DA] = _dot(oa, woa).astype(bf16)

        def tail(h, carry):
            fillers = {
                S // TQ - nf + r: [lambda r=r: out_a((h - (H - 2)) * nf + r)]
                for r in range(nf)}
            _b_head(h, h % 4, qb, kb, vb, ctx, fillers)
            return carry

        jax.lax.fori_loop(H - 2, H, tail, 0)

        wob_copy.wait()

        def out_copy(r):
            r0 = pl.multiple_of(r * TO, TO)
            return pltpu.make_async_copy(
                out_s.at[pl.ds(r0, TO), :], out_h.at[pl.ds(r0, TO), :], sem_out)

        def obody(r, carry):
            r0 = pl.multiple_of(r * TO, TO)
            p0 = pl.multiple_of(r * (TO // 2), TO // 2)
            cb = jnp.concatenate(
                [_unpack(ctx[h, pl.ds(p0, TO // 2), :]) for h in range(H)], axis=1)
            out_s[pl.ds(r0, TO), DA:DA + M] = _dot(cb, wob_v[...]).astype(bf16)
            out_copy(r).start()
            return carry

        jax.lax.fori_loop(0, S // TO, obody, 0)
        for r in range(S // TO):
            out_copy(r).wait()

    pl.run_scoped(
        phase_b,
        pltpu.VMEM((H, S // 2, D), u32), pltpu.VMEM((H * D, M), bf16))


@jax.jit
def pallas_concat_heads__sliding_local_dilated__compressed_kv_cla__prompt_kernel(
    A_x: jax.Array,
    A_wqkv: jax.Array,
    A_wo: jax.Array,
    B_x: jax.Array,
    B_c_kv: jax.Array,
    B_w_q: jax.Array,
    B_w_uk: jax.Array,
    B_w_uv: jax.Array,
    B_w_o: jax.Array,
):
    any_spec = pl.BlockSpec(memory_space=pl.ANY)
    out = pl.pallas_call(
        _kernel,
        out_shape=jax.ShapeDtypeStruct((S, DA + M), bf16),
        in_specs=[any_spec] * 9,
        out_specs=any_spec,
        scratch_shapes=[
            pltpu.VMEM((4, S // 2, D), u32),
            pltpu.VMEM((4, S // 2, D), u32),
            pltpu.VMEM((4, S // 2, D), u32),
            pltpu.VMEM((8, DA // 2, 128), u32),
            pltpu.VMEM((S // 2, DA), u32),
            pltpu.VMEM((8, S + PADR, 128), f32),
            pltpu.VMEM((8, S + PADR, 128), f32),
            pltpu.VMEM((8, S + PADR, 128), f32),
            pltpu.VMEM((H // 2 * (M + 1) + 48, D), u32),
            pltpu.VMEM((H // 2 * (C + 1) + 48, D), u32),
            pltpu.VMEM((H // 2 * (C + 1) + 48, D), u32),
            pltpu.VMEM((S // 2, M), u32),
            pltpu.VMEM((S // 2, C), u32),
            pltpu.VMEM((S, DA + M), bf16),
            pltpu.SemaphoreType.DMA((24,)),
            pltpu.SemaphoreType.DMA((4,)),
            pltpu.SemaphoreType.DMA((28,)),
            pltpu.SemaphoreType.DMA(()),
            pltpu.SemaphoreType.DMA(()),
        ],
        compiler_params=pltpu.CompilerParams(vmem_limit_bytes=120 * 1024 * 1024),
    )(
        A_x.reshape(S, DA), A_wqkv, A_wo,
        B_x.reshape(S, M), B_c_kv.reshape(S, C),
        B_w_q.reshape(M * H, D), B_w_uk.reshape(C * H, D), B_w_uv.reshape(C * H, D),
        B_w_o.reshape(H * D, M),
    )
    return out.reshape(1, S, DA + M)
```

```python
import math

import jax
import jax.numpy as jnp
import jax.experimental.pallas as pl
import jax.experimental.pallas.tpu as pltpu

bf16 = jnp.bfloat16
f32 = jnp.float32
u32 = jnp.uint32

S = 2048
DA = 1024
HA = 32
DH = 32
WIN = 8
DIL = 2
M = 1024
C = 512
H = 32
D = 128
LOG2E = math.log2(math.e)
NEG = -1e30
PADR = 16
DP = HA + 1
TA = 512
TQ = 256
TP = 256
TO = 256
NT = (((1,), (1,)), ((), ()))


def _unpack(x):
    return pltpu.bitcast(x, bf16)


def _pack(x):
    return pltpu.bitcast(x, u32)


def _dot(a, b):
    return jnp.dot(a, b, preferred_element_type=f32)


def _dot_nt(a, b):
    return jax.lax.dot_general(a, b, NT, preferred_element_type=f32)


def _prep_w_block(t, rb, wqkv_v, stage, wtp):
    r0 = pl.multiple_of(rb * 128, 128)
    for cb in range(8):
        c0 = t * DA + cb * 128
        tile = wqkv_v[pl.ds(r0, 128), c0:c0 + 128].astype(f32).T
        for hl in range(4):
            stage[pl.ds(4 * cb + hl, DH, stride=DP), :] = tile[hl * DH:(hl + 1) * DH, :]
    for d in range(DH):
        rows = stage[pl.ds(d * DP, HA), :]
        o0 = (t * DA + d * HA) // 2
        wtp[rb, o0:o0 + HA // 2, :] = _pack(rows.astype(bf16))


def _prep_wo_block(nb, wo_v, stage, wop):
    for h in range(HA):
        rows = wo_v[nb, h * DH:(h + 1) * DH, :].astype(f32)
        stage[pl.ds(h, DH, stride=DP), :] = rows
    for d in range(DH):
        rows = stage[pl.ds(d * DP, HA), :]
        wop[nb, d * (HA // 2):(d + 1) * (HA // 2), :] = _pack(rows.astype(bf16))


NB = 512


def _a_proj(t, r, ax_v, wtp, dst):
    r0 = pl.multiple_of(r * TA, TA)
    x = ax_v[pl.ds(r0, TA), :]
    for n in range(DA // NB):
        f0 = (t * DA + n * NB) // 2
        w = jnp.concatenate(
            [_unpack(wtp[rb, f0:f0 + NB // 2, :]) for rb in range(8)], axis=1)
        y = _dot_nt(x, w)
        if t == 0:
            y = y * ((DH ** -0.5) * LOG2E)
        for cc in range(NB // 128):
            dst[n * (NB // 128) + cc, pl.ds(r0 + PADR, TA), :] = (
                y[:, cc * 128:(cc + 1) * 128])


GA = 16


def _a_attn_rows(row0, qp, kp, vp, masked):
    G = 8
    q = [qp[c, pl.ds(row0 + PADR, G), :] for c in range(8)]
    if masked:
        pos = row0 + jax.lax.broadcasted_iota(jnp.int32, (G, 128), 0)
    logits = []
    for w in range(WIN):
        z = None
        for c in range(8):
            p = q[c] * kp[c, pl.ds(row0 + PADR - DIL * w, G), :]
            z = p if z is None else z + p
        z = z + pltpu.roll(z, 64, 1)
        z = z + pltpu.roll(z, 32, 1)
        if masked and w > 0:
            z = jnp.where(pos >= DIL * w, z, NEG)
        logits.append(z)
    m = logits[0]
    for w in range(1, WIN):
        m = jnp.maximum(m, logits[w])
    es = [jnp.exp2(z - m) for z in logits]
    l = es[0]
    for w in range(1, WIN):
        l = l + es[w]
    inv = 1.0 / l
    attn = [e * inv for e in es]
    outs = []
    for c in range(8):
        acc = None
        for w in range(WIN):
            v = vp[c, pl.ds(row0 + PADR - DIL * w, G), :]
            acc = attn[w] * v if acc is None else acc + attn[w] * v
        outs.append(acc)
    return outs


def _a_attn_group(row0, qp, kp, vp, op, masked):
    a = _a_attn_rows(row0, qp, kp, vp, masked)
    b = _a_attn_rows(row0 + 8, qp, kp, vp, masked)
    o0 = pl.multiple_of(row0 // 2, GA // 2)
    for c in range(8):
        op[pl.ds(o0, GA // 2), c * 128:(c + 1) * 128] = _pack(
            jnp.concatenate([a[c], b[c]], axis=0).astype(bf16))


def _deinterleave_block(mb, raw, dst, rows):
    pitch = rows + 1
    base = pl.multiple_of(mb * 8, 8)
    blk = _pack(raw[pl.ds(pl.multiple_of(base * H, 8 * H), 8 * H), :])
    for mm in range(8):
        dst[pl.ds(base + mm, H // 2, stride=pitch), :] = (
            blk[mm * (H // 2):(mm + 1) * (H // 2), :])


def _pair_weights(wt, j, rows):
    w = wt[pl.ds(j * (rows + 1), rows), :]
    lo = pltpu.bitcast(w << 16, f32).astype(bf16)
    hi = pltpu.bitcast(w & jnp.uint32(0xFFFF0000), f32).astype(bf16)
    return jnp.concatenate([lo, hi], axis=1)


def _b_proj_parts(p0, ws, bxp, cp, qb, kb, vb, slot0):
    wq, wk, wv = ws
    rows = pl.ds(p0, TP // 2)

    def put(dst, y):
        for e in range(2):
            dst[slot0 + e, rows, :] = _pack(y[:, e * D:(e + 1) * D].astype(bf16))

    return [
        lambda: put(qb, _dot(_unpack(bxp[rows, :]), wq) * ((D ** -0.5) * LOG2E)),
        lambda: put(kb, _dot(_unpack(cp[rows, :]), wk)),
        lambda: put(vb, _dot(_unpack(cp[rows, :]), wv)),
    ]


HQ = TQ // 2


def _b_qk(i, qa, ka):
    k0 = i * TQ
    n = k0 + HQ
    q = qa[k0:k0 + TQ]
    s = _dot_nt(q, ka[0:n])
    s2 = _dot_nt(q[HQ:], ka[n:n + HQ])
    row = jax.lax.broadcasted_iota(jnp.int32, (HQ, 128), 0)
    col = jax.lax.broadcasted_iota(jnp.int32, (HQ, 128), 1)
    tri = col <= row
    nb = n // 128
    top = [s[:HQ, j * 128:(j + 1) * 128] for j in range(nb)]
    top[-1] = jnp.where(tri, top[-1], NEG)
    bot = [s[HQ:, j * 128:(j + 1) * 128] for j in range(nb)]
    bot.append(jnp.where(tri, s2, NEG))
    mps = []
    for blocks in (top, bot):
        mp = blocks[0]
        for c in blocks[1:]:
            mp = jnp.maximum(mp, c)
        mps.append(mp)
    return (top, bot), mps


def _b_softmax(blocks, mps, prev):
    ps, lps = [], []
    for half in range(2):
        mp = mps[half]
        if prev is not None:
            mp = jnp.maximum(mp, jnp.minimum(prev[half], NEG))
        m = jnp.max(mp, axis=1, keepdims=True)
        lp = None
        pl_ = []
        for jj, c in enumerate(blocks[half]):
            p = jnp.exp2(c - m)
            lp = p if lp is None else lp + p
            if jj == len(blocks[half]) - 1:
                p = p + jnp.minimum(lp, 0.0)
            pl_.append(p.astype(bf16))
        ps.append(pl_)
        lps.append(lp)
    return ps, lps


def _b_pv(i, ps, lps, va, ctx, h):
    k0 = i * TQ
    n = k0 + HQ
    nb = n // 128
    ls = [jnp.sum(lp, axis=1, keepdims=True) for lp in lps]
    pc = jnp.concatenate(
        [jnp.concatenate(ps[0], axis=1), jnp.concatenate(ps[1][:nb], axis=1)], axis=0)
    o = _dot(pc, va[0:n])
    o2 = _dot(ps[1][nb], va[n:n + HQ])
    o_top = o[:HQ] * (1.0 / ls[0])
    o_bot = (o[HQ:] + o2) * (1.0 / ls[1])
    ctx[h, k0 // 2:(k0 + HQ) // 2, :] = _pack(o_top.astype(bf16))
    ctx[h, (k0 + HQ) // 2:(k0 + TQ) // 2, :] = _pack(o_bot.astype(bf16))
    return (o_top, o_bot)


def _b_head(h, slot, qb, kb, vb, ctx, fillers):
    nT = S // TQ
    order = list(range(nT))[::-1]
    qa, ka, va = _unpack(qb[slot]), _unpack(kb[slot]), _unpack(vb[slot])
    cur = _b_qk(order[0], qa, ka)
    prev = None
    for t, i in enumerate(order):
        nxt = _b_qk(order[t + 1], qa, ka) if t + 1 < nT else None
        ps, lps = _b_softmax(cur[0], cur[1], prev)
        for f in fillers.get(t, ()):
            f()
        prev = _b_pv(i, ps, lps, va, ctx, h)
        cur = nxt


def _kernel(ax_h, wqkv_h, wo_h, bx_h, c_h, wq_h, wuk_h, wuv_h, wob_h, out_h,
            qb, kb, vb, wop, op, qp, kp, vp,
            wq_t, wk_t, wv_t, bxp, cp, out_s,
            sem_w, sem_ax, sem_f, sem_wob, sem_out, sem_oa):
    NR = S // TA

    def rows(ref, r, n):
        return ref.at[pl.ds(pl.multiple_of(r * n, n), n), :]

    def phase_a(ax_v, wqkv_v, wo_v, stage, wtp, bx_v, c_v, wq_raw, wuk_raw, wuv_raw):
        def w_copy(t, rb):
            r0 = pl.multiple_of(rb * 128, 128)
            sl = (pl.ds(r0, 128), slice(t * DA, (t + 1) * DA))
            return pltpu.make_async_copy(wqkv_h.at[sl], wqkv_v.at[sl],
                                         sem_w.at[8 * t + rb])

        def ax_copy(r):
            return pltpu.make_async_copy(rows(ax_h, r, TA), rows(ax_v, r, TA),
                                         sem_ax.at[r])

        def f_copy(r, i):
            sem = sem_f.at[7 * r + i]
            if i < 3:
                src, dst, n = ((wq_h, wq_raw, M), (wuk_h, wuk_raw, C),
                               (wuv_h, wuv_raw, C))[i]
                n = n * H // NR
                return pltpu.make_async_copy(rows(src, r, n), rows(dst, r, n), sem)
            if i < 5:
                src, dst = ((bx_h, bx_v), (c_h, c_v))[i - 3]
                return pltpu.make_async_copy(rows(src, r, TA), rows(dst, r, TA), sem)
            nb = 2 * r + (i - 5)
            c0 = pl.multiple_of(nb * 128, 128)
            return pltpu.make_async_copy(wo_h.at[:, pl.ds(c0, 128)], wo_v.at[nb], sem)

        sched = {
            0: [lambda: ax_copy(1), lambda: w_copy(1, 2), lambda: w_copy(1, 3)],
            1: [lambda: ax_copy(2), lambda: w_copy(1, 4), lambda: w_copy(1, 5)],
            2: [lambda: ax_copy(3), lambda: w_copy(1, 6), lambda: w_copy(1, 7)],
            3: [lambda: w_copy(2, 0), lambda: w_copy(2, 1)],
            4: [lambda: w_copy(2, 2), lambda: w_copy(2, 3)],
            5: [lambda: w_copy(2, 4), lambda: w_copy(2, 5)],
            6: [lambda: w_copy(2, 6), lambda: w_copy(2, 7)],
        }
        fslots = [
            [(0, 0)], [(0, 1), (0, 2), (0, 4)], [(0, 3), (0, 5), (0, 6), (1, 1)],
            [(1, 0), (1, 2)], [(1, 3), (1, 4), (1, 5), (1, 6), (2, 1)],
            [(2, 0), (2, 2)], [(2, 3), (2, 4), (2, 5), (2, 6)],
            [(3, 0), (3, 1)], [(3, 2), (3, 3), (3, 4), (3, 5), (3, 6)],
        ]
        for slot, items in enumerate(fslots):
            sched.setdefault(slot, []).extend(
                (lambda r=r, i=i: f_copy(r, i)) for r, i in items)

        def issue(t, r):
            for k in range(NR):
                items = sched.get(NR * t + k, [])
                if items:
                    @pl.when(r == k)
                    def _():
                        for mk in items:
                            mk().start()

        for rb in range(8):
            w_copy(0, rb).start()
        ax_copy(0).start()
        w_copy(1, 0).start()
        w_copy(1, 1).start()
        for ref in (kp, vp):
            ref[:, 0:PADR, :] = jnp.zeros((8, PADR, 128), f32)

        def prep0(rb, carry):
            w_copy(0, rb).wait()
            _prep_w_block(0, rb, wqkv_v, stage.at[0], wtp)
            return carry

        jax.lax.fori_loop(0, 8, prep0, 0)

        def qk_step(t):
            def body(r, carry):
                if t == 0:
                    ax_copy(r).wait()
                w_copy(t + 1, 2 * r).wait()
                w_copy(t + 1, 2 * r + 1).wait()
                issue(t, r)
                _a_proj(t, r, ax_v, wtp, (qp, kp)[t])
                for i in range(2):
                    _prep_w_block(t + 1, 2 * r + i, wqkv_v, stage.at[i], wtp)
                return carry
            return body

        jax.lax.fori_loop(0, NR, qk_step(0), 0)
        jax.lax.fori_loop(0, NR, qk_step(1), 0)

        def v_step(r, carry):
            for i in range(7):
                f_copy(r, i).wait()
            issue(2, r)
            _a_proj(2, r, ax_v, wtp, vp)
            nq = M // 8 // NR
            nk = C // 8 // NR
            for i in range(nq):
                _deinterleave_block(r * nq + i, wq_raw, wq_t, M)
            for i in range(nk):
                _deinterleave_block(r * nk + i, wuk_raw, wk_t, C)
                _deinterleave_block(r * nk + i, wuv_raw, wv_t, C)
            src = pl.ds(pl.multiple_of(r * TA, TA), TA)
            dst = pl.ds(pl.multiple_of(r * (TA // 2), TA // 2), TA // 2)
            bxp[dst, :] = _pack(bx_v[src, :])
            cp[dst, :] = _pack(c_v[src, :])
            for i in range(2):
                _prep_wo_block(2 * r + i, wo_v, stage.at[i], wop)
            return carry

        jax.lax.fori_loop(0, NR, v_step, 0)

    pl.run_scoped(
        phase_a,
        pltpu.VMEM((S, DA), bf16), pltpu.VMEM((DA, 3 * DA), bf16),
        pltpu.VMEM((8, DA, 128), bf16), pltpu.VMEM((2, HA * DP, 128), f32),
        pltpu.VMEM((8, 3 * DA // 2, 128), u32),
        pltpu.VMEM((S, M), bf16), pltpu.VMEM((S, C), bf16),
        pltpu.VMEM((M * H, D), bf16), pltpu.VMEM((C * H, D), bf16),
        pltpu.VMEM((C * H, D), bf16))

    def phase_b(ctx, wob_v):
        wob_copy = pltpu.make_async_copy(wob_h, wob_v, sem_wob)
        wob_copy.start()

        def weights(j):
            return (_pair_weights(wq_t, j, M), _pair_weights(wk_t, j, C),
                    _pair_weights(wv_t, j, C))

        half = S // 4
        nf = S // TP // 2
        ga = 4

        def first(e, carry):
            ws = weights(0)
            for r in range(nf):
                p0 = pl.multiple_of(e * half + r * (TP // 2), TP // 2)
                for f in _b_proj_parts(p0, ws, bxp, cp, qb, kb, vb, 0):
                    f()
                _a_attn_group((e * ga + r) * GA, qp, kp, vp, op, True)
            return carry

        jax.lax.fori_loop(0, 2, first, 0)

        def body(h, carry):
            e = h % 2
            ws = weights(h // 2 + 1)
            wslot = 2 * ((h // 2 + 1) % 2)
            fillers = {}
            for r in range(nf):
                p0 = pl.multiple_of(e * half + r * (TP // 2), TP // 2)
                fillers[S // TQ - nf + r] = _b_proj_parts(
                    p0, ws, bxp, cp, qb, kb, vb, wslot) + [
                        lambda r=r: _a_attn_group(((h + 2) * ga + r) * GA,
                                                  qp, kp, vp, op, False)]
            _b_head(h, h % 4, qb, kb, vb, ctx, fillers)
            return carry

        jax.lax.fori_loop(0, H - 2, body, 0)

        def out_a(r):
            r0 = pl.multiple_of(r * TO, TO)
            p0 = pl.multiple_of(r * (TO // 2), TO // 2)
            oa = _unpack(op[pl.ds(p0, TO // 2), :])
            woa = jnp.concatenate([_unpack(wop[nb]) for nb in range(8)], axis=1)
            out_s[pl.ds(r0, TO), 0:DA] = _dot(oa, woa).astype(bf16)

        def tail(h, carry):
            fillers = {
                S // TQ - nf + r: [lambda r=r: out_a((h - (H - 2)) * nf + r)]
                for r in range(nf)}
            _b_head(h, h % 4, qb, kb, vb, ctx, fillers)
            return carry

        jax.lax.fori_loop(H - 2, H, tail, 0)

        out_a_copy = pltpu.make_async_copy(
            out_s.at[:, 0:DA], out_h.at[:, 0:DA], sem_oa)
        out_a_copy.start()
        wob_copy.wait()

        def out_copy(r):
            r0 = pl.multiple_of(r * TO, TO)
            return pltpu.make_async_copy(
                out_s.at[pl.ds(r0, TO), DA:DA + M],
                out_h.at[pl.ds(r0, TO), DA:DA + M], sem_out)

        def obody(r, carry):
            r0 = pl.multiple_of(r * TO, TO)
            p0 = pl.multiple_of(r * (TO // 2), TO // 2)
            cb = jnp.concatenate(
                [_unpack(ctx[h, pl.ds(p0, TO // 2), :]) for h in range(H)], axis=1)
            out_s[pl.ds(r0, TO), DA:DA + M] = _dot(cb, wob_v[...]).astype(bf16)
            out_copy(r).start()
            return carry

        jax.lax.fori_loop(0, S // TO, obody, 0)
        out_a_copy.wait()
        for r in range(S // TO):
            out_copy(r).wait()

    pl.run_scoped(
        phase_b,
        pltpu.VMEM((H, S // 2, D), u32), pltpu.VMEM((H * D, M), bf16))


@jax.jit
def pallas_concat_heads__sliding_local_dilated__compressed_kv_cla__prompt_kernel(
    A_x: jax.Array,
    A_wqkv: jax.Array,
    A_wo: jax.Array,
    B_x: jax.Array,
    B_c_kv: jax.Array,
    B_w_q: jax.Array,
    B_w_uk: jax.Array,
    B_w_uv: jax.Array,
    B_w_o: jax.Array,
):
    any_spec = pl.BlockSpec(memory_space=pl.ANY)
    out = pl.pallas_call(
        _kernel,
        out_shape=jax.ShapeDtypeStruct((S, DA + M), bf16),
        in_specs=[any_spec] * 9,
        out_specs=any_spec,
        scratch_shapes=[
            pltpu.VMEM((4, S // 2, D), u32),
            pltpu.VMEM((4, S // 2, D), u32),
            pltpu.VMEM((4, S // 2, D), u32),
            pltpu.VMEM((8, DA // 2, 128), u32),
            pltpu.VMEM((S // 2, DA), u32),
            pltpu.VMEM((8, S + PADR, 128), f32),
            pltpu.VMEM((8, S + PADR, 128), f32),
            pltpu.VMEM((8, S + PADR, 128), f32),
            pltpu.VMEM((H // 2 * (M + 1) + 48, D), u32),
            pltpu.VMEM((H // 2 * (C + 1) + 48, D), u32),
            pltpu.VMEM((H // 2 * (C + 1) + 48, D), u32),
            pltpu.VMEM((S // 2, M), u32),
            pltpu.VMEM((S // 2, C), u32),
            pltpu.VMEM((S, DA + M), bf16),
            pltpu.SemaphoreType.DMA((24,)),
            pltpu.SemaphoreType.DMA((4,)),
            pltpu.SemaphoreType.DMA((28,)),
            pltpu.SemaphoreType.DMA(()),
            pltpu.SemaphoreType.DMA(()),
            pltpu.SemaphoreType.DMA(()),
        ],
        compiler_params=pltpu.CompilerParams(vmem_limit_bytes=120 * 1024 * 1024),
    )(
        A_x.reshape(S, DA), A_wqkv, A_wo,
        B_x.reshape(S, M), B_c_kv.reshape(S, C),
        B_w_q.reshape(M * H, D), B_w_uk.reshape(C * H, D), B_w_uv.reshape(C * H, D),
        B_w_o.reshape(H * D, M),
    )
    return out.reshape(1, S, DA + M)
```

```python
import math

import jax
import jax.numpy as jnp
import jax.experimental.pallas as pl
import jax.experimental.pallas.tpu as pltpu

bf16 = jnp.bfloat16
f32 = jnp.float32
u32 = jnp.uint32

S = 2048
DA = 1024
HA = 32
DH = 32
WIN = 8
DIL = 2
M = 1024
C = 512
H = 32
D = 128
LOG2E = math.log2(math.e)
NEG = -1e30
PADR = 16
DP = HA + 1
TA = 512
TQ = 256
TP = 256
TO = 256
NT = (((1,), (1,)), ((), ()))


def _unpack(x):
    return pltpu.bitcast(x, bf16)


def _pack(x):
    return pltpu.bitcast(x, u32)


def _dot(a, b):
    return jnp.dot(a, b, preferred_element_type=f32)


def _dot_nt(a, b):
    return jax.lax.dot_general(a, b, NT, preferred_element_type=f32)


def _prep_w_block(t, rb, wqkv_v, stage, wtp):
    r0 = pl.multiple_of(rb * 128, 128)
    for cb in range(8):
        c0 = t * DA + cb * 128
        tile = wqkv_v[pl.ds(r0, 128), c0:c0 + 128].astype(f32).T
        for hl in range(4):
            stage[pl.ds(4 * cb + hl, DH, stride=DP), :] = tile[hl * DH:(hl + 1) * DH, :]
    for d in range(DH):
        rows = stage[pl.ds(d * DP, HA), :]
        o0 = (t * DA + d * HA) // 2
        wtp[rb, o0:o0 + HA // 2, :] = _pack(rows.astype(bf16))


def _prep_wo_block(nb, wo_v, stage, wop):
    for h in range(HA):
        rows = wo_v[nb, h * DH:(h + 1) * DH, :].astype(f32)
        stage[pl.ds(h, DH, stride=DP), :] = rows
    for d in range(DH):
        rows = stage[pl.ds(d * DP, HA), :]
        wop[nb, d * (HA // 2):(d + 1) * (HA // 2), :] = _pack(rows.astype(bf16))


NB = 512


def _a_proj(t, r, ax_v, wtp, dst):
    r0 = pl.multiple_of(r * TA, TA)
    x = ax_v[pl.ds(r0, TA), :]
    for n in range(DA // NB):
        f0 = (t * DA + n * NB) // 2
        w = jnp.concatenate(
            [_unpack(wtp[rb, f0:f0 + NB // 2, :]) for rb in range(8)], axis=1)
        y = _dot_nt(x, w)
        if t == 0:
            y = y * ((DH ** -0.5) * LOG2E)
        for cc in range(NB // 128):
            dst[n * (NB // 128) + cc, pl.ds(r0 + PADR, TA), :] = (
                y[:, cc * 128:(cc + 1) * 128])


GA = 16


def _a_attn_rows(row0, qp, kp, vp, masked):
    G = 8
    q = [qp[c, pl.ds(row0 + PADR, G), :] for c in range(8)]
    if masked:
        pos = row0 + jax.lax.broadcasted_iota(jnp.int32, (G, 128), 0)
    logits = []
    for w in range(WIN):
        z = None
        for c in range(8):
            p = q[c] * kp[c, pl.ds(row0 + PADR - DIL * w, G), :]
            z = p if z is None else z + p
        z = z + pltpu.roll(z, 64, 1)
        z = z + pltpu.roll(z, 32, 1)
        if masked and w > 0:
            z = jnp.where(pos >= DIL * w, z, NEG)
        logits.append(z)
    m = logits[0]
    for w in range(1, WIN):
        m = jnp.maximum(m, logits[w])
    es = [jnp.exp2(z - m) for z in logits]
    l = es[0]
    for w in range(1, WIN):
        l = l + es[w]
    inv = 1.0 / l
    attn = [e * inv for e in es]
    outs = []
    for c in range(8):
        acc = None
        for w in range(WIN):
            v = vp[c, pl.ds(row0 + PADR - DIL * w, G), :]
            acc = attn[w] * v if acc is None else acc + attn[w] * v
        outs.append(acc)
    return outs


def _a_attn_group(row0, qp, kp, vp, op, masked):
    a = _a_attn_rows(row0, qp, kp, vp, masked)
    b = _a_attn_rows(row0 + 8, qp, kp, vp, masked)
    o0 = pl.multiple_of(row0 // 2, GA // 2)
    for c in range(8):
        op[pl.ds(o0, GA // 2), c * 128:(c + 1) * 128] = _pack(
            jnp.concatenate([a[c], b[c]], axis=0).astype(bf16))


def _deinterleave_block(mb, raw, dst, rows):
    pitch = rows + 1
    base = pl.multiple_of(mb * 8, 8)
    blk = _pack(raw[pl.ds(pl.multiple_of(base * H, 8 * H), 8 * H), :])
    for mm in range(8):
        dst[pl.ds(base + mm, H // 2, stride=pitch), :] = (
            blk[mm * (H // 2):(mm + 1) * (H // 2), :])


def _pair_weights(wt, j, rows):
    w = wt[pl.ds(j * (rows + 1), rows), :]
    lo = pltpu.bitcast(w << 16, f32).astype(bf16)
    hi = pltpu.bitcast(w & jnp.uint32(0xFFFF0000), f32).astype(bf16)
    return jnp.concatenate([lo, hi], axis=1)


def _b_proj_parts(p0, ws, bxp, cp, qb, kb, vb, slot0):
    wq, wk, wv = ws
    rows = pl.ds(p0, TP // 2)

    def put(dst, y):
        for e in range(2):
            dst[slot0 + e, rows, :] = _pack(y[:, e * D:(e + 1) * D].astype(bf16))

    return [
        lambda: put(qb, _dot(_unpack(bxp[rows, :]), wq) * ((D ** -0.5) * LOG2E)),
        lambda: put(kb, _dot(_unpack(cp[rows, :]), wk)),
        lambda: put(vb, _dot(_unpack(cp[rows, :]), wv)),
    ]


HQ = TQ // 2


def _b_qk(i, qa, ka):
    k0 = i * TQ
    n = k0 + HQ
    q = qa[k0:k0 + TQ]
    s = _dot_nt(q, ka[0:n])
    s2 = _dot_nt(q[HQ:], ka[n:n + HQ])
    row = jax.lax.broadcasted_iota(jnp.int32, (HQ, 128), 0)
    col = jax.lax.broadcasted_iota(jnp.int32, (HQ, 128), 1)
    tri = col <= row
    nb = n // 128
    top = [s[:HQ, j * 128:(j + 1) * 128] for j in range(nb)]
    top[-1] = jnp.where(tri, top[-1], NEG)
    bot = [s[HQ:, j * 128:(j + 1) * 128] for j in range(nb)]
    bot.append(jnp.where(tri, s2, NEG))
    mps = []
    for blocks in (top, bot):
        mp = blocks[0]
        for c in blocks[1:]:
            mp = jnp.maximum(mp, c)
        mps.append(mp)
    return (top, bot), mps


def _b_softmax(blocks, mps, prev):
    ps, lps = [], []
    for half in range(2):
        mp = mps[half]
        if prev is not None:
            mp = jnp.maximum(mp, jnp.minimum(prev[half], NEG))
        m = jnp.max(mp, axis=1, keepdims=True)
        lp = None
        pl_ = []
        for jj, c in enumerate(blocks[half]):
            p = jnp.exp2(c - m)
            lp = p if lp is None else lp + p
            if jj == len(blocks[half]) - 1:
                p = p + jnp.minimum(lp, 0.0)
            pl_.append(p.astype(bf16))
        ps.append(pl_)
        lps.append(lp)
    return ps, lps


def _b_pv(i, ps, lps, va, ctx, h):
    k0 = i * TQ
    n = k0 + HQ
    nb = n // 128
    ls = [jnp.sum(lp, axis=1, keepdims=True) for lp in lps]
    pc = jnp.concatenate(
        [jnp.concatenate(ps[0], axis=1), jnp.concatenate(ps[1][:nb], axis=1)], axis=0)
    o = _dot(pc, va[0:n])
    o2 = _dot(ps[1][nb], va[n:n + HQ])
    o_top = o[:HQ] * (1.0 / ls[0])
    o_bot = (o[HQ:] + o2) * (1.0 / ls[1])
    ctx[h, k0 // 2:(k0 + HQ) // 2, :] = _pack(o_top.astype(bf16))
    ctx[h, (k0 + HQ) // 2:(k0 + TQ) // 2, :] = _pack(o_bot.astype(bf16))
    return (o_top, o_bot)


def _b_head(h, slot, qb, kb, vb, ctx, order, fillers):
    qa, ka, va = _unpack(qb[slot]), _unpack(kb[slot]), _unpack(vb[slot])
    cur = _b_qk(order[0], qa, ka)
    prev = None
    for t, i in enumerate(order):
        nxt = _b_qk(order[t + 1], qa, ka) if t + 1 < len(order) else None
        for f in fillers.get(('a', t), ()):
            f()
        ps, lps = _b_softmax(cur[0], cur[1], prev)
        for f in fillers.get(('m', t), ()):
            f()
        prev = _b_pv(i, ps, lps, va, ctx, h)
        for f in fillers.get(('p', t), ()):
            f()
        cur = nxt


MAIN_ORDER = (1, 7, 3, 6, 4, 2, 5, 0)
MAIN_PLACE = (
    (0, ('a', 4)), (1, ('p', 0)), (2, ('p', 6)), (3, ('m', 4)), (4, ('p', 0)),
    (12, ('a', 5)), (6, ('m', 6)), (7, ('m', 6)), (8, ('m', 7)), (9, ('m', 7)),
    (10, ('a', 5)), (11, ('m', 7)), (15, ('p', 1)), (13, ('a', 4)), (14, ('m', 6)),
    (5, ('m', 5)))
TAIL_ORDER = (7, 6, 5, 4, 3, 2, 1, 0)


def _kernel(ax_h, wqkv_h, wo_h, bx_h, c_h, wq_h, wuk_h, wuv_h, wob_h, out_h,
            qb, kb, vb, wop, op, qp, kp, vp,
            wq_t, wk_t, wv_t, bxp, cp, out_s,
            sem_w, sem_ax, sem_f, sem_wob, sem_out, sem_oa):
    NR = S // TA

    def rows(ref, r, n):
        return ref.at[pl.ds(pl.multiple_of(r * n, n), n), :]

    def phase_a(ax_v, wqkv_v, wo_v, stage, wtp, bx_v, c_v, wq_raw, wuk_raw, wuv_raw):
        def w_copy(t, rb):
            r0 = pl.multiple_of(rb * 128, 128)
            sl = (pl.ds(r0, 128), slice(t * DA, (t + 1) * DA))
            return pltpu.make_async_copy(wqkv_h.at[sl], wqkv_v.at[sl],
                                         sem_w.at[8 * t + rb])

        def ax_copy(r):
            return pltpu.make_async_copy(rows(ax_h, r, TA), rows(ax_v, r, TA),
                                         sem_ax.at[r])

        def f_copy(r, i):
            sem = sem_f.at[7 * r + i]
            if i < 3:
                src, dst, n = ((wq_h, wq_raw, M), (wuk_h, wuk_raw, C),
                               (wuv_h, wuv_raw, C))[i]
                n = n * H // NR
                return pltpu.make_async_copy(rows(src, r, n), rows(dst, r, n), sem)
            if i < 5:
                src, dst = ((bx_h, bx_v), (c_h, c_v))[i - 3]
                return pltpu.make_async_copy(rows(src, r, TA), rows(dst, r, TA), sem)
            nb = 2 * r + (i - 5)
            c0 = pl.multiple_of(nb * 128, 128)
            return pltpu.make_async_copy(wo_h.at[:, pl.ds(c0, 128)], wo_v.at[nb], sem)

        sched = {
            0: [lambda: ax_copy(1), lambda: w_copy(1, 2), lambda: w_copy(1, 3)],
            1: [lambda: ax_copy(2), lambda: w_copy(1, 4), lambda: w_copy(1, 5)],
            2: [lambda: ax_copy(3), lambda: w_copy(1, 6), lambda: w_copy(1, 7)],
            3: [lambda: w_copy(2, 0), lambda: w_copy(2, 1)],
            4: [lambda: w_copy(2, 2), lambda: w_copy(2, 3)],
            5: [lambda: w_copy(2, 4), lambda: w_copy(2, 5)],
            6: [lambda: w_copy(2, 6), lambda: w_copy(2, 7)],
        }
        fslots = [
            [(0, 0)], [(0, 1), (0, 2), (0, 4)], [(0, 3), (0, 5), (0, 6), (1, 1)],
            [(1, 0), (1, 2)], [(1, 3), (1, 4), (1, 5), (1, 6), (2, 1)],
            [(2, 0), (2, 2)], [(2, 3), (2, 4), (2, 5), (2, 6)],
            [(3, 0), (3, 1)], [(3, 2), (3, 3), (3, 4), (3, 5), (3, 6)],
        ]
        for slot, items in enumerate(fslots):
            sched.setdefault(slot, []).extend(
                (lambda r=r, i=i: f_copy(r, i)) for r, i in items)

        def issue(t, r):
            for k in range(NR):
                items = sched.get(NR * t + k, [])
                if items:
                    @pl.when(r == k)
                    def _():
                        for mk in items:
                            mk().start()

        for rb in range(8):
            w_copy(0, rb).start()
        ax_copy(0).start()
        w_copy(1, 0).start()
        w_copy(1, 1).start()
        for ref in (kp, vp):
            ref[:, 0:PADR, :] = jnp.zeros((8, PADR, 128), f32)

        def prep0(rb, carry):
            w_copy(0, rb).wait()
            _prep_w_block(0, rb, wqkv_v, stage.at[0], wtp)
            return carry

        jax.lax.fori_loop(0, 8, prep0, 0)

        def qk_step(t):
            def body(r, carry):
                if t == 0:
                    ax_copy(r).wait()
                w_copy(t + 1, 2 * r).wait()
                w_copy(t + 1, 2 * r + 1).wait()
                issue(t, r)
                _a_proj(t, r, ax_v, wtp, (qp, kp)[t])
                for i in range(2):
                    _prep_w_block(t + 1, 2 * r + i, wqkv_v, stage.at[i], wtp)
                return carry
            return body

        jax.lax.fori_loop(0, NR, qk_step(0), 0)
        jax.lax.fori_loop(0, NR, qk_step(1), 0)

        def v_step(r, carry):
            for i in range(7):
                f_copy(r, i).wait()
            issue(2, r)
            _a_proj(2, r, ax_v, wtp, vp)
            nq = M // 8 // NR
            nk = C // 8 // NR
            for i in range(nq):
                _deinterleave_block(r * nq + i, wq_raw, wq_t, M)
            for i in range(nk):
                _deinterleave_block(r * nk + i, wuk_raw, wk_t, C)
                _deinterleave_block(r * nk + i, wuv_raw, wv_t, C)
            src = pl.ds(pl.multiple_of(r * TA, TA), TA)
            dst = pl.ds(pl.multiple_of(r * (TA // 2), TA // 2), TA // 2)
            bxp[dst, :] = _pack(bx_v[src, :])
            cp[dst, :] = _pack(c_v[src, :])
            for i in range(2):
                _prep_wo_block(2 * r + i, wo_v, stage.at[i], wop)
            return carry

        jax.lax.fori_loop(0, NR, v_step, 0)

    pl.run_scoped(
        phase_a,
        pltpu.VMEM((S, DA), bf16), pltpu.VMEM((DA, 3 * DA), bf16),
        pltpu.VMEM((8, DA, 128), bf16), pltpu.VMEM((2, HA * DP, 128), f32),
        pltpu.VMEM((8, 3 * DA // 2, 128), u32),
        pltpu.VMEM((S, M), bf16), pltpu.VMEM((S, C), bf16),
        pltpu.VMEM((M * H, D), bf16), pltpu.VMEM((C * H, D), bf16),
        pltpu.VMEM((C * H, D), bf16))

    def phase_b(ctx, wob_v):
        wob_copy = pltpu.make_async_copy(wob_h, wob_v, sem_wob)
        wob_copy.start()

        def weights(j):
            return (_pair_weights(wq_t, j, M), _pair_weights(wk_t, j, C),
                    _pair_weights(wv_t, j, C))

        half = S // 4
        nf = S // TP // 2
        ga = 4

        def first(e, carry):
            ws = weights(0)
            for r in range(nf):
                p0 = pl.multiple_of(e * half + r * (TP // 2), TP // 2)
                for f in _b_proj_parts(p0, ws, bxp, cp, qb, kb, vb, 0):
                    f()
                _a_attn_group((e * ga + r) * GA, qp, kp, vp, op, True)
            return carry

        jax.lax.fori_loop(0, 2, first, 0)

        def body(h, carry):
            e = h % 2
            ws = weights(h // 2 + 1)
            wslot = 2 * ((h // 2 + 1) % 2)
            items = []
            for r in range(nf):
                p0 = pl.multiple_of(e * half + r * (TP // 2), TP // 2)
                items += _b_proj_parts(p0, ws, bxp, cp, qb, kb, vb, wslot)
            for r in range(ga):
                items.append(lambda r=r: _a_attn_group(
                    ((h + 2) * ga + r) * GA, qp, kp, vp, op, False))
            fillers = {}
            for j, pos in MAIN_PLACE:
                fillers.setdefault(pos, []).append(items[j])
            _b_head(h, h % 4, qb, kb, vb, ctx, MAIN_ORDER, fillers)
            return carry

        jax.lax.fori_loop(0, H - 2, body, 0)

        def out_a(r):
            r0 = pl.multiple_of(r * TO, TO)
            p0 = pl.multiple_of(r * (TO // 2), TO // 2)
            oa = _unpack(op[pl.ds(p0, TO // 2), :])
            woa = jnp.concatenate([_unpack(wop[nb]) for nb in range(8)], axis=1)
            out_s[pl.ds(r0, TO), 0:DA] = _dot(oa, woa).astype(bf16)

        def tail(h, carry):
            fillers = {
                ('m', S // TQ - nf + r): [lambda r=r: out_a((h - (H - 2)) * nf + r)]
                for r in range(nf)}
            _b_head(h, h % 4, qb, kb, vb, ctx, TAIL_ORDER, fillers)
            return carry

        jax.lax.fori_loop(H - 2, H, tail, 0)

        out_a_copy = pltpu.make_async_copy(
            out_s.at[:, 0:DA], out_h.at[:, 0:DA], sem_oa)
        out_a_copy.start()
        wob_copy.wait()

        def out_copy(r):
            r0 = pl.multiple_of(r * TO, TO)
            return pltpu.make_async_copy(
                out_s.at[pl.ds(r0, TO), DA:DA + M],
                out_h.at[pl.ds(r0, TO), DA:DA + M], sem_out)

        def obody(r, carry):
            r0 = pl.multiple_of(r * TO, TO)
            p0 = pl.multiple_of(r * (TO // 2), TO // 2)
            cb = jnp.concatenate(
                [_unpack(ctx[h, pl.ds(p0, TO // 2), :]) for h in range(H)], axis=1)
            out_s[pl.ds(r0, TO), DA:DA + M] = _dot(cb, wob_v[...]).astype(bf16)
            out_copy(r).start()
            return carry

        jax.lax.fori_loop(0, S // TO, obody, 0)
        out_a_copy.wait()
        for r in range(S // TO):
            out_copy(r).wait()

    pl.run_scoped(
        phase_b,
        pltpu.VMEM((H, S // 2, D), u32), pltpu.VMEM((H * D, M), bf16))


@jax.jit
def pallas_concat_heads__sliding_local_dilated__compressed_kv_cla__prompt_kernel(
    A_x: jax.Array,
    A_wqkv: jax.Array,
    A_wo: jax.Array,
    B_x: jax.Array,
    B_c_kv: jax.Array,
    B_w_q: jax.Array,
    B_w_uk: jax.Array,
    B_w_uv: jax.Array,
    B_w_o: jax.Array,
):
    any_spec = pl.BlockSpec(memory_space=pl.ANY)
    out = pl.pallas_call(
        _kernel,
        out_shape=jax.ShapeDtypeStruct((S, DA + M), bf16),
        in_specs=[any_spec] * 9,
        out_specs=any_spec,
        scratch_shapes=[
            pltpu.VMEM((4, S // 2, D), u32),
            pltpu.VMEM((4, S // 2, D), u32),
            pltpu.VMEM((4, S // 2, D), u32),
            pltpu.VMEM((8, DA // 2, 128), u32),
            pltpu.VMEM((S // 2, DA), u32),
            pltpu.VMEM((8, S + PADR, 128), f32),
            pltpu.VMEM((8, S + PADR, 128), f32),
            pltpu.VMEM((8, S + PADR, 128), f32),
            pltpu.VMEM((H // 2 * (M + 1) + 48, D), u32),
            pltpu.VMEM((H // 2 * (C + 1) + 48, D), u32),
            pltpu.VMEM((H // 2 * (C + 1) + 48, D), u32),
            pltpu.VMEM((S // 2, M), u32),
            pltpu.VMEM((S // 2, C), u32),
            pltpu.VMEM((S, DA + M), bf16),
            pltpu.SemaphoreType.DMA((24,)),
            pltpu.SemaphoreType.DMA((4,)),
            pltpu.SemaphoreType.DMA((28,)),
            pltpu.SemaphoreType.DMA(()),
            pltpu.SemaphoreType.DMA(()),
            pltpu.SemaphoreType.DMA(()),
        ],
        compiler_params=pltpu.CompilerParams(vmem_limit_bytes=120 * 1024 * 1024),
    )(
        A_x.reshape(S, DA), A_wqkv, A_wo,
        B_x.reshape(S, M), B_c_kv.reshape(S, C),
        B_w_q.reshape(M * H, D), B_w_uk.reshape(C * H, D), B_w_uv.reshape(C * H, D),
        B_w_o.reshape(H * D, M),
    )
    return out.reshape(1, S, DA + M)
```

```python
import functools
import math

import jax
import jax.numpy as jnp
import jax.experimental.pallas as pl
import jax.experimental.pallas.tpu as pltpu

bf16 = jnp.bfloat16
f32 = jnp.float32
u32 = jnp.uint32

S = 2048
DA = 1024
HA = 32
DH = 32
WIN = 8
DIL = 2
M = 1024
C = 512
H = 32
D = 128
LOG2E = math.log2(math.e)
NEG = -1e30
PADR = 16
DP = HA + 1
TA = 512
TQ = 256
TP = 256
TO = 256
PACE = 6
NT = (((1,), (1,)), ((), ()))


def _unpack(x):
    return pltpu.bitcast(x, bf16)


def _pack(x):
    return pltpu.bitcast(x, u32)


def _dot(a, b):
    return jnp.dot(a, b, preferred_element_type=f32)


def _dot_nt(a, b):
    return jax.lax.dot_general(a, b, NT, preferred_element_type=f32)


def _zero_after(dep):
    dep = pltpu.roll(pltpu.roll(dep, 1, 1), 1, 1)
    return (dep >> 16) >> 16


def _or_tiled(x, z):
    row = jnp.concatenate([z] * (x.shape[1] // 128), axis=1)
    return x | jnp.concatenate([row] * (x.shape[0] // 8), axis=0)


def _prep_w_block(t, rb, wqkv_v, stage, wtp):
    r0 = pl.multiple_of(rb * 128, 128)
    for cb in range(8):
        c0 = t * DA + cb * 128
        tile = wqkv_v[pl.ds(r0, 128), c0:c0 + 128].astype(f32).T
        for hl in range(4):
            stage[pl.ds(4 * cb + hl, DH, stride=DP), :] = tile[hl * DH:(hl + 1) * DH, :]
    for d in range(DH):
        rows = stage[pl.ds(d * DP, HA), :]
        o0 = (t * DA + d * HA) // 2
        wtp[rb, o0:o0 + HA // 2, :] = _pack(rows.astype(bf16))


def _prep_wo_block(nb, wo_v, stage, wop, dep=None):
    z = None if dep is None else _zero_after(dep)
    for h in range(HA):
        rows = wo_v[nb, h * DH:(h + 1) * DH, :].astype(f32)
        if z is not None:
            rows = pltpu.bitcast(_or_tiled(pltpu.bitcast(rows, u32), z), f32)
        stage[pl.ds(h, DH, stride=DP), :] = rows
    for d in range(DH):
        rows = stage[pl.ds(d * DP, HA), :]
        wop[nb, d * (HA // 2):(d + 1) * (HA // 2), :] = _pack(rows.astype(bf16))
    return wop[nb, DA // 2 - 8:DA // 2, :]


NB = 512


def _a_proj(t, r, ax_v, wtp, dst):
    r0 = pl.multiple_of(r * TA, TA)
    x = ax_v[pl.ds(r0, TA), :]
    for n in range(DA // NB):
        f0 = (t * DA + n * NB) // 2
        w = jnp.concatenate(
            [_unpack(wtp[rb, f0:f0 + NB // 2, :]) for rb in range(8)], axis=1)
        y = _dot_nt(x, w)
        if t == 0:
            y = y * ((DH ** -0.5) * LOG2E)
        for cc in range(NB // 128):
            dst[n * (NB // 128) + cc, pl.ds(r0 + PADR, TA), :] = (
                y[:, cc * 128:(cc + 1) * 128])


GA = 16


def _a_attn_rows(row0, qp, kp, vp, masked):
    G = 8
    q = [qp[c, pl.ds(row0 + PADR, G), :] for c in range(8)]
    if masked:
        pos = row0 + jax.lax.broadcasted_iota(jnp.int32, (G, 128), 0)
    logits = []
    for w in range(WIN):
        z = None
        for c in range(8):
            p = q[c] * kp[c, pl.ds(row0 + PADR - DIL * w, G), :]
            z = p if z is None else z + p
        z = z + pltpu.roll(z, 64, 1)
        z = z + pltpu.roll(z, 32, 1)
        if masked and w > 0:
            z = jnp.where(pos >= DIL * w, z, NEG)
        logits.append(z)
    m = logits[0]
    for w in range(1, WIN):
        m = jnp.maximum(m, logits[w])
    es = [jnp.exp2(z - m) for z in logits]
    l = es[0]
    for w in range(1, WIN):
        l = l + es[w]
    inv = 1.0 / l
    attn = [e * inv for e in es]
    outs = []
    for c in range(8):
        acc = None
        for w in range(WIN):
            v = vp[c, pl.ds(row0 + PADR - DIL * w, G), :]
            acc = attn[w] * v if acc is None else acc + attn[w] * v
        outs.append(acc)
    return outs


def _a_attn_group(row0, qp, kp, vp, op, masked):
    a = _a_attn_rows(row0, qp, kp, vp, masked)
    b = _a_attn_rows(row0 + 8, qp, kp, vp, masked)
    o0 = pl.multiple_of(row0 // 2, GA // 2)
    for c in range(8):
        op[pl.ds(o0, GA // 2), c * 128:(c + 1) * 128] = _pack(
            jnp.concatenate([a[c], b[c]], axis=0).astype(bf16))


def _deinterleave_block(mb, raw, dst, rows, dep=None):
    pitch = rows + 1
    base = pl.multiple_of(mb * 8, 8)
    blk = _pack(raw[pl.ds(pl.multiple_of(base * H, 8 * H), 8 * H), :])
    if dep is not None:
        blk = _or_tiled(blk, _zero_after(dep))
    for mm in range(8):
        dst[pl.ds(base + mm, H // 2, stride=pitch), :] = (
            blk[mm * (H // 2):(mm + 1) * (H // 2), :])
    return dst[pl.ds(base + (H // 2 - 1) * pitch, 8), :]


def _repack_rows(row0, n, src, dst, dep=None):
    val = _pack(src[pl.ds(pl.multiple_of(row0, n), n), :])
    if dep is not None:
        val = _or_tiled(val, _zero_after(dep))
    dst[pl.ds(pl.multiple_of(row0 // 2, n // 2), n // 2), :] = val
    last = pl.multiple_of((row0 + n) // 2 - 8, 8)
    return dst[pl.ds(last, 8), val.shape[1] - 128:val.shape[1]]


def _pair_weights(wt, j, rows):
    w = wt[pl.ds(j * (rows + 1), rows), :]
    lo = pltpu.bitcast(w << 16, f32).astype(bf16)
    hi = pltpu.bitcast(w & jnp.uint32(0xFFFF0000), f32).astype(bf16)
    return jnp.concatenate([lo, hi], axis=1)


def _b_proj_parts(p0, ws, bxp, cp, qb, kb, vb, slot0):
    wq, wk, wv = ws
    rows = pl.ds(p0, TP // 2)

    def put(dst, y):
        for e in range(2):
            dst[slot0 + e, rows, :] = _pack(y[:, e * D:(e + 1) * D].astype(bf16))

    return [
        lambda: put(qb, _dot(_unpack(bxp[rows, :]), wq) * ((D ** -0.5) * LOG2E)),
        lambda: put(kb, _dot(_unpack(cp[rows, :]), wk)),
        lambda: put(vb, _dot(_unpack(cp[rows, :]), wv)),
    ]


HQ = TQ // 2


def _b_qk(i, qa, ka):
    k0 = i * TQ
    n = k0 + HQ
    q = qa[k0:k0 + TQ]
    s = _dot_nt(q, ka[0:n])
    s2 = _dot_nt(q[HQ:], ka[n:n + HQ])
    row = jax.lax.broadcasted_iota(jnp.int32, (HQ, 128), 0)
    col = jax.lax.broadcasted_iota(jnp.int32, (HQ, 128), 1)
    tri = col <= row
    nb = n // 128
    top = [s[:HQ, j * 128:(j + 1) * 128] for j in range(nb)]
    top[-1] = jnp.where(tri, top[-1], NEG)
    bot = [s[HQ:, j * 128:(j + 1) * 128] for j in range(nb)]
    bot.append(jnp.where(tri, s2, NEG))
    mps = []
    for blocks in (top, bot):
        mp = blocks[0]
        for c in blocks[1:]:
            mp = jnp.maximum(mp, c)
        mps.append(mp)
    return (top, bot), mps


def _b_softmax(blocks, mps, prev):
    ps, lps = [], []
    for half in range(2):
        mp = mps[half]
        if prev is not None:
            mp = jnp.maximum(mp, jnp.minimum(prev[half], NEG))
        m = jnp.max(mp, axis=1, keepdims=True)
        lp = None
        pl_ = []
        for jj, c in enumerate(blocks[half]):
            p = jnp.exp2(c - m)
            lp = p if lp is None else lp + p
            if jj == len(blocks[half]) - 1:
                p = p + jnp.minimum(lp, 0.0)
            pl_.append(p.astype(bf16))
        ps.append(pl_)
        lps.append(lp)
    return ps, lps


def _b_pv(i, ps, lps, va, ctx, h):
    k0 = i * TQ
    n = k0 + HQ
    nb = n // 128
    ls = [jnp.sum(lp, axis=1, keepdims=True) for lp in lps]
    pc = jnp.concatenate(
        [jnp.concatenate(ps[0], axis=1), jnp.concatenate(ps[1][:nb], axis=1)], axis=0)
    o = _dot(pc, va[0:n])
    o2 = _dot(ps[1][nb], va[n:n + HQ])
    o_top = o[:HQ] * (1.0 / ls[0])
    o_bot = (o[HQ:] + o2) * (1.0 / ls[1])
    ctx[h, k0 // 2:(k0 + HQ) // 2, :] = _pack(o_top.astype(bf16))
    ctx[h, (k0 + HQ) // 2:(k0 + TQ) // 2, :] = _pack(o_bot.astype(bf16))
    return (o_top, o_bot)


def _b_head(h, slot, qb, kb, vb, ctx, order, fillers):
    qa, ka, va = _unpack(qb[slot]), _unpack(kb[slot]), _unpack(vb[slot])
    cur = _b_qk(order[0], qa, ka)
    prev = None
    for t, i in enumerate(order):
        nxt = _b_qk(order[t + 1], qa, ka) if t + 1 < len(order) else None
        for f in fillers.get(('a', t), ()):
            f()
        ps, lps = _b_softmax(cur[0], cur[1], prev)
        for f in fillers.get(('m', t), ()):
            f()
        prev = _b_pv(i, ps, lps, va, ctx, h)
        for f in fillers.get(('p', t), ()):
            f()
        cur = nxt


MAIN_ORDER = (1, 7, 3, 6, 4, 2, 5, 0)
MAIN_PLACE = (
    (0, ('a', 4)), (1, ('p', 0)), (2, ('p', 6)), (3, ('m', 4)), (4, ('p', 0)),
    (12, ('a', 5)), (6, ('m', 6)), (7, ('m', 6)), (8, ('m', 7)), (9, ('m', 7)),
    (10, ('a', 5)), (11, ('m', 7)), (15, ('p', 1)), (13, ('a', 4)), (14, ('m', 6)),
    (5, ('m', 5)))
TAIL_ORDER = (1, 7, 3, 6, 4, 2, 5, 0)
TAIL_CHUNKS = 3
TAIL_PLACE = ((2, ('m', 6)), (5, ('p', 6)), (0, ('p', 0)), (3, ('m', 6)),
              (4, ('m', 7)), (1, ('m', 4)))


def _kernel(ax_h, wqkv_h, wo_h, bx_h, c_h, wq_h, wuk_h, wuv_h, wob_h, out_h,
            qb, kb, vb, wop, op, qp, kp, vp,
            wq_t, wk_t, wv_t, bxp, cp, out_s,
            sem_w, sem_ax, sem_f, sem_wob, sem_out, sem_oa):
    NR = S // TA

    def rows(ref, r, n):
        return ref.at[pl.ds(pl.multiple_of(r * n, n), n), :]

    def phase_a(ax_v, wqkv_v, wo_v, stage, wtp, bx_v, c_v, wq_raw, wuk_raw, wuv_raw):
        def w_copy(t, rb):
            r0 = pl.multiple_of(rb * 128, 128)
            sl = (pl.ds(r0, 128), slice(t * DA, (t + 1) * DA))
            return pltpu.make_async_copy(wqkv_h.at[sl], wqkv_v.at[sl],
                                         sem_w.at[8 * t + rb])

        def ax_copy(r):
            return pltpu.make_async_copy(rows(ax_h, r, TA), rows(ax_v, r, TA),
                                         sem_ax.at[r])

        def f_copy(r, i):
            sem = sem_f.at[7 * r + i]
            if i < 3:
                src, dst, n = ((wq_h, wq_raw, M), (wuk_h, wuk_raw, C),
                               (wuv_h, wuv_raw, C))[i]
                n = n * H // NR
                return pltpu.make_async_copy(rows(src, r, n), rows(dst, r, n), sem)
            if i < 5:
                src, dst = ((bx_h, bx_v), (c_h, c_v))[i - 3]
                return pltpu.make_async_copy(rows(src, r, TA), rows(dst, r, TA), sem)
            nb = 2 * r + (i - 5)
            c0 = pl.multiple_of(nb * 128, 128)
            return pltpu.make_async_copy(wo_h.at[:, pl.ds(c0, 128)], wo_v.at[nb], sem)

        sched = {
            0: [lambda: ax_copy(1), lambda: w_copy(1, 2), lambda: w_copy(1, 3)],
            1: [lambda: ax_copy(2), lambda: w_copy(1, 4), lambda: w_copy(1, 5)],
            2: [lambda: ax_copy(3), lambda: w_copy(1, 6), lambda: w_copy(1, 7)],
            3: [lambda: w_copy(2, 0), lambda: w_copy(2, 1)],
            4: [lambda: w_copy(2, 2), lambda: w_copy(2, 3)],
            5: [lambda: w_copy(2, 4), lambda: w_copy(2, 5)],
            6: [lambda: w_copy(2, 6), lambda: w_copy(2, 7)],
        }
        fslots = [
            [(0, 0)], [(0, 1), (0, 2), (0, 4)], [(0, 3), (0, 5), (0, 6), (1, 1)],
            [(1, 0), (1, 2)], [(1, 3), (1, 4), (1, 5), (1, 6), (2, 1)],
            [(2, 0), (2, 2)], [(2, 3), (2, 4), (2, 5), (2, 6)],
            [(3, 0), (3, 1)], [(3, 2), (3, 3), (3, 4), (3, 5), (3, 6)],
        ]
        for slot, items in enumerate(fslots):
            sched.setdefault(slot, []).extend(
                (lambda r=r, i=i: f_copy(r, i)) for r, i in items)

        def issue(t, r):
            for k in range(NR):
                items = sched.get(NR * t + k, [])
                if items:
                    @pl.when(r == k)
                    def _():
                        for mk in items:
                            mk().start()

        for rb in range(8):
            w_copy(0, rb).start()
        ax_copy(0).start()
        w_copy(1, 0).start()
        w_copy(1, 1).start()
        for ref in (kp, vp):
            ref[:, 0:PADR, :] = jnp.zeros((8, PADR, 128), f32)

        def prep0(rb, carry):
            w_copy(0, rb).wait()
            _prep_w_block(0, rb, wqkv_v, stage.at[0], wtp)
            return carry

        jax.lax.fori_loop(0, 8, prep0, 0)

        def qk_step(t):
            def body(r, carry):
                if t == 0:
                    ax_copy(r).wait()
                w_copy(t + 1, 2 * r).wait()
                w_copy(t + 1, 2 * r + 1).wait()
                issue(t, r)
                _a_proj(t, r, ax_v, wtp, (qp, kp)[t])
                for i in range(2):
                    _prep_w_block(t + 1, 2 * r + i, wqkv_v, stage.at[i], wtp)
                return carry
            return body

        jax.lax.fori_loop(0, NR, qk_step(0), 0)
        jax.lax.fori_loop(0, NR, qk_step(1), 0)

        def v_step(r, carry):
            for i in range(7):
                f_copy(r, i).wait()
            issue(2, r)
            _a_proj(2, r, ax_v, wtp, vp)
            nq = M // 8 // NR
            nk = C // 8 // NR
            items = (
                [functools.partial(_deinterleave_block, r * nq + i, wq_raw, wq_t, M)
                 for i in range(nq)]
                + [functools.partial(_deinterleave_block, r * nk + i, wuk_raw, wk_t, C)
                   for i in range(nk)]
                + [functools.partial(_deinterleave_block, r * nk + i, wuv_raw, wv_t, C)
                   for i in range(nk)]
                + [functools.partial(_prep_wo_block, 2 * r + i, wo_v, stage.at[i], wop)
                   for i in range(2)]
                + [functools.partial(_repack_rows, r * TA + i * 32, 32, bx_v, bxp)
                   for i in range(TA // 32)]
                + [functools.partial(_repack_rows, r * TA + i * 64, 64, c_v, cp)
                   for i in range(TA // 64)])
            backs = []
            for idx, f in enumerate(items):
                backs.append(f(backs[idx - PACE] if idx >= PACE else None))
            return carry

        jax.lax.fori_loop(0, NR, v_step, 0)

    pl.run_scoped(
        phase_a,
        pltpu.VMEM((S, DA), bf16), pltpu.VMEM((DA, 3 * DA), bf16),
        pltpu.VMEM((8, DA, 128), bf16), pltpu.VMEM((2, HA * DP, 128), f32),
        pltpu.VMEM((8, 3 * DA // 2, 128), u32),
        pltpu.VMEM((S, M), bf16), pltpu.VMEM((S, C), bf16),
        pltpu.VMEM((M * H, D), bf16), pltpu.VMEM((C * H, D), bf16),
        pltpu.VMEM((C * H, D), bf16))

    def phase_b(ctx, wob_v):
        wob_copy = pltpu.make_async_copy(wob_h, wob_v, sem_wob)
        wob_copy.start()

        def weights(j):
            return (_pair_weights(wq_t, j, M), _pair_weights(wk_t, j, C),
                    _pair_weights(wv_t, j, C))

        half = S // 4
        nf = S // TP // 2
        ga = 4

        def first(e, carry):
            ws = weights(0)
            for r in range(nf):
                p0 = pl.multiple_of(e * half + r * (TP // 2), TP // 2)
                for f in _b_proj_parts(p0, ws, bxp, cp, qb, kb, vb, 0):
                    f()
                _a_attn_group((e * ga + r) * GA, qp, kp, vp, op, True)
            return carry

        jax.lax.fori_loop(0, 2, first, 0)

        def body(h, carry):
            e = h % 2
            ws = weights(h // 2 + 1)
            wslot = 2 * ((h // 2 + 1) % 2)
            items = []
            for r in range(nf):
                p0 = pl.multiple_of(e * half + r * (TP // 2), TP // 2)
                items += _b_proj_parts(p0, ws, bxp, cp, qb, kb, vb, wslot)
            for r in range(ga):
                items.append(lambda r=r: _a_attn_group(
                    ((h + 2) * ga + r) * GA, qp, kp, vp, op, False))
            fillers = {}
            for j, pos in MAIN_PLACE:
                fillers.setdefault(pos, []).append(items[j])
            _b_head(h, h % 4, qb, kb, vb, ctx, MAIN_ORDER, fillers)
            return carry

        jax.lax.fori_loop(0, H - 2, body, 0)

        def out_a(r, n):
            r0 = pl.multiple_of(r * TO, TO)
            p0 = pl.multiple_of(r * (TO // 2), TO // 2)
            oa = _unpack(op[pl.ds(p0, TO // 2), :])
            woa = jnp.concatenate(
                [_unpack(wop[nb]) for nb in range(4 * n, 4 * n + 4)], axis=1)
            out_s[pl.ds(r0, TO), n * (DA // 2):(n + 1) * (DA // 2)] = (
                _dot(oa, woa).astype(bf16))

        def tail(h, carry):
            fillers = {}
            for j, pos in TAIL_PLACE:
                fillers.setdefault(pos, []).append(functools.partial(
                    out_a, (h - (H - 2)) * TAIL_CHUNKS + j // 2, j % 2))
            _b_head(h, h % 4, qb, kb, vb, ctx, TAIL_ORDER, fillers)
            return carry

        jax.lax.fori_loop(H - 2, H, tail, 0)

        def rest_a(r, carry):
            out_a(r, 0)
            out_a(r, 1)
            return carry

        jax.lax.fori_loop(2 * TAIL_CHUNKS, S // TO, rest_a, 0)

        out_a_copy = pltpu.make_async_copy(
            out_s.at[:, 0:DA], out_h.at[:, 0:DA], sem_oa)
        out_a_copy.start()
        wob_copy.wait()

        def out_copy(r):
            r0 = pl.multiple_of(r * TO, TO)
            return pltpu.make_async_copy(
                out_s.at[pl.ds(r0, TO), DA:DA + M],
                out_h.at[pl.ds(r0, TO), DA:DA + M], sem_out)

        def obody(r, carry):
            r0 = pl.multiple_of(r * TO, TO)
            p0 = pl.multiple_of(r * (TO // 2), TO // 2)
            cb = jnp.concatenate(
                [_unpack(ctx[h, pl.ds(p0, TO // 2), :]) for h in range(H)], axis=1)
            out_s[pl.ds(r0, TO), DA:DA + M] = _dot(cb, wob_v[...]).astype(bf16)
            out_copy(r).start()
            return carry

        jax.lax.fori_loop(0, S // TO, obody, 0)
        out_a_copy.wait()
        for r in range(S // TO):
            out_copy(r).wait()

    pl.run_scoped(
        phase_b,
        pltpu.VMEM((H, S // 2, D), u32), pltpu.VMEM((H * D, M), bf16))


@jax.jit
def pallas_concat_heads__sliding_local_dilated__compressed_kv_cla__prompt_kernel(
    A_x: jax.Array,
    A_wqkv: jax.Array,
    A_wo: jax.Array,
    B_x: jax.Array,
    B_c_kv: jax.Array,
    B_w_q: jax.Array,
    B_w_uk: jax.Array,
    B_w_uv: jax.Array,
    B_w_o: jax.Array,
):
    any_spec = pl.BlockSpec(memory_space=pl.ANY)
    out = pl.pallas_call(
        _kernel,
        out_shape=jax.ShapeDtypeStruct((S, DA + M), bf16),
        in_specs=[any_spec] * 9,
        out_specs=any_spec,
        scratch_shapes=[
            pltpu.VMEM((4, S // 2, D), u32),
            pltpu.VMEM((4, S // 2, D), u32),
            pltpu.VMEM((4, S // 2, D), u32),
            pltpu.VMEM((8, DA // 2, 128), u32),
            pltpu.VMEM((S // 2, DA), u32),
            pltpu.VMEM((8, S + PADR, 128), f32),
            pltpu.VMEM((8, S + PADR, 128), f32),
            pltpu.VMEM((8, S + PADR, 128), f32),
            pltpu.VMEM((H // 2 * (M + 1) + 48, D), u32),
            pltpu.VMEM((H // 2 * (C + 1) + 48, D), u32),
            pltpu.VMEM((H // 2 * (C + 1) + 48, D), u32),
            pltpu.VMEM((S // 2, M), u32),
            pltpu.VMEM((S // 2, C), u32),
            pltpu.VMEM((S, DA + M), bf16),
            pltpu.SemaphoreType.DMA((24,)),
            pltpu.SemaphoreType.DMA((4,)),
            pltpu.SemaphoreType.DMA((28,)),
            pltpu.SemaphoreType.DMA(()),
            pltpu.SemaphoreType.DMA(()),
            pltpu.SemaphoreType.DMA(()),
        ],
        compiler_params=pltpu.CompilerParams(vmem_limit_bytes=120 * 1024 * 1024),
    )(
        A_x.reshape(S, DA), A_wqkv, A_wo,
        B_x.reshape(S, M), B_c_kv.reshape(S, C),
        B_w_q.reshape(M * H, D), B_w_uk.reshape(C * H, D), B_w_uv.reshape(C * H, D),
        B_w_o.reshape(H * D, M),
    )
    return out.reshape(1, S, DA + M)
```

```python
import functools
import math

import jax
import jax.numpy as jnp
import jax.experimental.pallas as pl
import jax.experimental.pallas.tpu as pltpu

bf16 = jnp.bfloat16
f32 = jnp.float32
u32 = jnp.uint32

S = 2048
DA = 1024
HA = 32
DH = 32
WIN = 8
DIL = 2
M = 1024
C = 512
H = 32
D = 128
LOG2E = math.log2(math.e)
NEG = -1e30
PADR = 16
DP = HA + 1
TA = 512
TQ = 256
TP = 256
TO = 256
PACE = 6
A_PACE = 3
A_ROLLS = 5
NT = (((1,), (1,)), ((), ()))


def _unpack(x):
    return pltpu.bitcast(x, bf16)


def _pack(x):
    return pltpu.bitcast(x, u32)


def _dot(a, b):
    return jnp.dot(a, b, preferred_element_type=f32)


def _dot_nt(a, b):
    return jax.lax.dot_general(a, b, NT, preferred_element_type=f32)


def _zero_after(dep, rolls=2):
    for _ in range(rolls):
        dep = pltpu.roll(dep, 1, 1)
    return (dep >> 16) >> 16


def _or_tiled(x, z):
    row = jnp.concatenate([z] * (x.shape[1] // 128), axis=1)
    return x | jnp.concatenate([row] * (x.shape[0] // 8), axis=0)


def _prep_w_block(t, rb, wqkv_v, stage, wtp):
    r0 = pl.multiple_of(rb * 128, 128)
    for cb in range(8):
        c0 = t * DA + cb * 128
        tile = wqkv_v[pl.ds(r0, 128), c0:c0 + 128].astype(f32).T
        for hl in range(4):
            stage[pl.ds(4 * cb + hl, DH, stride=DP), :] = tile[hl * DH:(hl + 1) * DH, :]
    for d in range(DH):
        rows = stage[pl.ds(d * DP, HA), :]
        o0 = (t * DA + d * HA) // 2
        wtp[rb, o0:o0 + HA // 2, :] = _pack(rows.astype(bf16))


def _prep_wo_block(nb, wo_v, stage, wop, dep=None):
    z = None if dep is None else _zero_after(dep)
    for h in range(HA):
        rows = wo_v[nb, h * DH:(h + 1) * DH, :].astype(f32)
        if z is not None:
            rows = pltpu.bitcast(_or_tiled(pltpu.bitcast(rows, u32), z), f32)
        stage[pl.ds(h, DH, stride=DP), :] = rows
    for d in range(DH):
        rows = stage[pl.ds(d * DP, HA), :]
        wop[nb, d * (HA // 2):(d + 1) * (HA // 2), :] = _pack(rows.astype(bf16))
    return wop[nb, DA // 2 - 8:DA // 2, :]


NB = 512


def _a_proj(t, r, ax_v, wtp, dst):
    r0 = pl.multiple_of(r * TA, TA)
    x = ax_v[pl.ds(r0, TA), :]
    for n in range(DA // NB):
        f0 = (t * DA + n * NB) // 2
        w = jnp.concatenate(
            [_unpack(wtp[rb, f0:f0 + NB // 2, :]) for rb in range(8)], axis=1)
        y = _dot_nt(x, w)
        if t == 0:
            y = y * ((DH ** -0.5) * LOG2E)
        for cc in range(NB // 128):
            dst[n * (NB // 128) + cc, pl.ds(r0 + PADR, TA), :] = (
                y[:, cc * 128:(cc + 1) * 128])


def _a_attn_rows(row0, qp, kp, vp, masked, dep):
    G = 8
    q = [qp[c, pl.ds(row0 + PADR, G), :] for c in range(8)]
    if dep is not None:
        z = _zero_after(pltpu.bitcast(dep, u32), A_ROLLS)
        q = [pltpu.bitcast(pltpu.bitcast(x, u32) | z, f32) for x in q]
    if masked:
        pos = row0 + jax.lax.broadcasted_iota(jnp.int32, (G, 128), 0)
    logits = []
    for w in range(WIN):
        z = None
        for c in range(8):
            p = q[c] * kp[c, pl.ds(row0 + PADR - DIL * w, G), :]
            z = p if z is None else z + p
        z = z + pltpu.roll(z, 64, 1)
        z = z + pltpu.roll(z, 32, 1)
        if masked and w > 0:
            z = jnp.where(pos >= DIL * w, z, NEG)
        logits.append(z)
    m = logits[0]
    for w in range(1, WIN):
        m = jnp.maximum(m, logits[w])
    es = [jnp.exp2(z - m) for z in logits]
    l = es[0]
    for w in range(1, WIN):
        l = l + es[w]
    inv = 1.0 / l
    attn = [e * inv for e in es]
    outs = []
    for c in range(8):
        acc = None
        for w in range(WIN):
            v = vp[c, pl.ds(row0 + PADR - DIL * w, G), :]
            acc = attn[w] * v if acc is None else acc + attn[w] * v
        outs.append(acc)
    return outs


def _a_attn_chunk(row0, n, qp, kp, vp):
    units = []
    for g in range(n // 8):
        dep = units[g - A_PACE][7] if g >= A_PACE else None
        units.append(_a_attn_rows(row0 + g * 8, qp, kp, vp, g < 2, dep))
    return jnp.concatenate(
        [jnp.concatenate(u, axis=1) for u in units], axis=0).astype(bf16)


def _deinterleave_block(mb, raw, dst, rows, dep=None):
    pitch = rows + 1
    base = pl.multiple_of(mb * 8, 8)
    blk = _pack(raw[pl.ds(pl.multiple_of(base * H, 8 * H), 8 * H), :])
    if dep is not None:
        blk = _or_tiled(blk, _zero_after(dep))
    for mm in range(8):
        dst[pl.ds(base + mm, H // 2, stride=pitch), :] = (
            blk[mm * (H // 2):(mm + 1) * (H // 2), :])
    return dst[pl.ds(base + (H // 2 - 1) * pitch, 8), :]


def _repack_rows(row0, n, src, dst, dep=None):
    val = _pack(src[pl.ds(pl.multiple_of(row0, n), n), :])
    if dep is not None:
        val = _or_tiled(val, _zero_after(dep))
    dst[pl.ds(pl.multiple_of(row0 // 2, n // 2), n // 2), :] = val
    last = pl.multiple_of((row0 + n) // 2 - 8, 8)
    return dst[pl.ds(last, 8), val.shape[1] - 128:val.shape[1]]


def _pair_weights(wt, j, rows):
    w = wt[pl.ds(j * (rows + 1), rows), :]
    lo = pltpu.bitcast(w << 16, f32).astype(bf16)
    hi = pltpu.bitcast(w & jnp.uint32(0xFFFF0000), f32).astype(bf16)
    return jnp.concatenate([lo, hi], axis=1)


def _b_proj_parts(p0, ws, bxp, cp, qb, kb, vb, slot0):
    wq, wk, wv = ws
    rows = pl.ds(p0, TP // 2)

    def put(dst, y):
        for e in range(2):
            dst[slot0 + e, rows, :] = _pack(y[:, e * D:(e + 1) * D].astype(bf16))

    return [
        lambda: put(qb, _dot(_unpack(bxp[rows, :]), wq) * ((D ** -0.5) * LOG2E)),
        lambda: put(kb, _dot(_unpack(cp[rows, :]), wk)),
        lambda: put(vb, _dot(_unpack(cp[rows, :]), wv)),
    ]


HQ = TQ // 2


def _b_qk(i, qa, ka):
    k0 = i * TQ
    n = k0 + HQ
    q = qa[k0:k0 + TQ]
    s = _dot_nt(q, ka[0:n])
    s2 = _dot_nt(q[HQ:], ka[n:n + HQ])
    row = jax.lax.broadcasted_iota(jnp.int32, (HQ, 128), 0)
    col = jax.lax.broadcasted_iota(jnp.int32, (HQ, 128), 1)
    tri = col <= row
    nb = n // 128
    top = [s[:HQ, j * 128:(j + 1) * 128] for j in range(nb)]
    top[-1] = jnp.where(tri, top[-1], NEG)
    bot = [s[HQ:, j * 128:(j + 1) * 128] for j in range(nb)]
    bot.append(jnp.where(tri, s2, NEG))
    mps = []
    for blocks in (top, bot):
        mp = blocks[0]
        for c in blocks[1:]:
            mp = jnp.maximum(mp, c)
        mps.append(mp)
    return (top, bot), mps


def _b_softmax(blocks, mps, prev):
    ps, lps = [], []
    for half in range(2):
        mp = mps[half]
        if prev is not None:
            mp = jnp.maximum(mp, jnp.minimum(prev[half], NEG))
        m = jnp.max(mp, axis=1, keepdims=True)
        lp = None
        pl_ = []
        for jj, c in enumerate(blocks[half]):
            p = jnp.exp2(c - m)
            lp = p if lp is None else lp + p
            if jj == len(blocks[half]) - 1:
                p = p + jnp.minimum(lp, 0.0)
            pl_.append(p.astype(bf16))
        ps.append(pl_)
        lps.append(lp)
    return ps, lps


def _b_pv(i, ps, lps, va, ctx, h):
    k0 = i * TQ
    n = k0 + HQ
    nb = n // 128
    ls = [jnp.sum(lp, axis=1, keepdims=True) for lp in lps]
    pc = jnp.concatenate(
        [jnp.concatenate(ps[0], axis=1), jnp.concatenate(ps[1][:nb], axis=1)], axis=0)
    o = _dot(pc, va[0:n])
    o2 = _dot(ps[1][nb], va[n:n + HQ])
    o_top = o[:HQ] * (1.0 / ls[0])
    o_bot = (o[HQ:] + o2) * (1.0 / ls[1])
    ctx[h, k0 // 2:(k0 + HQ) // 2, :] = _pack(o_top.astype(bf16))
    ctx[h, (k0 + HQ) // 2:(k0 + TQ) // 2, :] = _pack(o_bot.astype(bf16))
    return (o_top, o_bot)


def _b_head(h, slot, qb, kb, vb, ctx, order, lags, fillers):
    qa, ka, va = _unpack(qb[slot]), _unpack(kb[slot]), _unpack(vb[slot])
    cur = _b_qk(order[0], qa, ka)
    outs = []
    for t, i in enumerate(order):
        nxt = _b_qk(order[t + 1], qa, ka) if t + 1 < len(order) else None
        for f in fillers.get(('a', t), ()):
            f()
        prev = outs[-lags[t]] if 0 < lags[t] <= len(outs) else None
        ps, lps = _b_softmax(cur[0], cur[1], prev)
        for f in fillers.get(('m', t), ()):
            f()
        outs.append(_b_pv(i, ps, lps, va, ctx, h))
        for f in fillers.get(('p', t), ()):
            f()
        cur = nxt


MAIN_ORDER = (1, 7, 3, 4, 6, 2, 5, 0)
MAIN_LAGS = (1, 1, 1, 1, 1, 0, 1, 1)
MAIN_PLACE = (
    (6, ('a', 6)), (0, ('m', 4)), (1, ('p', 0)), (4, ('p', 0)), (11, ('m', 7)),
    (3, ('m', 4)), (10, ('p', 3)), (7, ('m', 6)), (9, ('m', 4)), (2, ('a', 4)),
    (8, ('p', 6)), (5, ('m', 1)))
TAIL_ORDER = (1, 7, 3, 4, 2, 5, 6, 0)
TAIL_LAGS = (1, 1, 1, 1, 1, 1, 0, 2)


def _kernel(ax_h, wqkv_h, wo_h, bx_h, c_h, wq_h, wuk_h, wuv_h, wob_h, out_h,
            qb, kb, vb, wop, qp, kp, vp,
            wq_t, wk_t, wv_t, bxp, cp, out_s,
            sem_w, sem_ax, sem_f, sem_wob, sem_out):
    NR = S // TA

    def rows(ref, r, n):
        return ref.at[pl.ds(pl.multiple_of(r * n, n), n), :]

    def phase_a(ax_v, wqkv_v, wo_v, stage, wtp, bx_v, c_v, wq_raw, wuk_raw, wuv_raw):
        def w_copy(t, rb):
            r0 = pl.multiple_of(rb * 128, 128)
            sl = (pl.ds(r0, 128), slice(t * DA, (t + 1) * DA))
            return pltpu.make_async_copy(wqkv_h.at[sl], wqkv_v.at[sl],
                                         sem_w.at[8 * t + rb])

        def ax_copy(r):
            return pltpu.make_async_copy(rows(ax_h, r, TA), rows(ax_v, r, TA),
                                         sem_ax.at[r])

        def f_copy(r, i):
            sem = sem_f.at[7 * r + i]
            if i < 3:
                src, dst, n = ((wq_h, wq_raw, M), (wuk_h, wuk_raw, C),
                               (wuv_h, wuv_raw, C))[i]
                n = n * H // NR
                return pltpu.make_async_copy(rows(src, r, n), rows(dst, r, n), sem)
            if i < 5:
                src, dst = ((bx_h, bx_v), (c_h, c_v))[i - 3]
                return pltpu.make_async_copy(rows(src, r, TA), rows(dst, r, TA), sem)
            nb = 2 * r + (i - 5)
            c0 = pl.multiple_of(nb * 128, 128)
            return pltpu.make_async_copy(wo_h.at[:, pl.ds(c0, 128)], wo_v.at[nb], sem)

        sched = {
            0: [lambda: ax_copy(1), lambda: w_copy(1, 2), lambda: w_copy(1, 3)],
            1: [lambda: ax_copy(2), lambda: w_copy(1, 4), lambda: w_copy(1, 5)],
            2: [lambda: ax_copy(3), lambda: w_copy(1, 6), lambda: w_copy(1, 7)],
            3: [lambda: w_copy(2, 0), lambda: w_copy(2, 1)],
            4: [lambda: w_copy(2, 2), lambda: w_copy(2, 3)],
            5: [lambda: w_copy(2, 4), lambda: w_copy(2, 5)],
            6: [lambda: w_copy(2, 6), lambda: w_copy(2, 7)],
        }
        fslots = [
            [(0, 0)], [(0, 1), (0, 2), (0, 4)], [(0, 3), (0, 5), (0, 6), (1, 1)],
            [(1, 0), (1, 2)], [(1, 3), (1, 4), (1, 5), (1, 6), (2, 1)],
            [(2, 0), (2, 2)], [(2, 3), (2, 4), (2, 5), (2, 6)],
            [(3, 0), (3, 1)], [(3, 2), (3, 3), (3, 4), (3, 5), (3, 6)],
        ]
        for slot, items in enumerate(fslots):
            sched.setdefault(slot, []).extend(
                (lambda r=r, i=i: f_copy(r, i)) for r, i in items)

        def issue(t, r):
            for k in range(NR):
                items = sched.get(NR * t + k, [])
                if items:
                    @pl.when(r == k)
                    def _():
                        for mk in items:
                            mk().start()

        for rb in range(8):
            w_copy(0, rb).start()
        ax_copy(0).start()
        w_copy(1, 0).start()
        w_copy(1, 1).start()
        for ref in (kp, vp):
            ref[:, 0:PADR, :] = jnp.zeros((8, PADR, 128), f32)

        def prep0(rb, carry):
            w_copy(0, rb).wait()
            _prep_w_block(0, rb, wqkv_v, stage.at[0], wtp)
            return carry

        jax.lax.fori_loop(0, 8, prep0, 0)

        def qk_step(t):
            def body(r, carry):
                if t == 0:
                    ax_copy(r).wait()
                w_copy(t + 1, 2 * r).wait()
                w_copy(t + 1, 2 * r + 1).wait()
                issue(t, r)
                _a_proj(t, r, ax_v, wtp, (qp, kp)[t])
                for i in range(2):
                    _prep_w_block(t + 1, 2 * r + i, wqkv_v, stage.at[i], wtp)
                return carry
            return body

        jax.lax.fori_loop(0, NR, qk_step(0), 0)
        jax.lax.fori_loop(0, NR, qk_step(1), 0)

        def v_step(r, carry):
            for i in range(7):
                f_copy(r, i).wait()
            issue(2, r)
            _a_proj(2, r, ax_v, wtp, vp)
            nq = M // 8 // NR
            nk = C // 8 // NR
            items = (
                [functools.partial(_deinterleave_block, r * nq + i, wq_raw, wq_t, M)
                 for i in range(nq)]
                + [functools.partial(_deinterleave_block, r * nk + i, wuk_raw, wk_t, C)
                   for i in range(nk)]
                + [functools.partial(_deinterleave_block, r * nk + i, wuv_raw, wv_t, C)
                   for i in range(nk)]
                + [functools.partial(_prep_wo_block, 2 * r + i, wo_v, stage.at[i], wop)
                   for i in range(2)]
                + [functools.partial(_repack_rows, r * TA + i * 32, 32, bx_v, bxp)
                   for i in range(TA // 32)]
                + [functools.partial(_repack_rows, r * TA + i * 64, 64, c_v, cp)
                   for i in range(TA // 64)])
            backs = []
            for idx, f in enumerate(items):
                backs.append(f(backs[idx - PACE] if idx >= PACE else None))
            return carry

        jax.lax.fori_loop(0, NR, v_step, 0)

    pl.run_scoped(
        phase_a,
        pltpu.VMEM((S, DA), bf16), pltpu.VMEM((DA, 3 * DA), bf16),
        pltpu.VMEM((8, DA, 128), bf16), pltpu.VMEM((2, HA * DP, 128), f32),
        pltpu.VMEM((8, 3 * DA // 2, 128), u32),
        pltpu.VMEM((S, M), bf16), pltpu.VMEM((S, C), bf16),
        pltpu.VMEM((M * H, D), bf16), pltpu.VMEM((C * H, D), bf16),
        pltpu.VMEM((C * H, D), bf16))

    def phase_b(ctx, wob_v):
        wob_copy = pltpu.make_async_copy(wob_h, wob_v, sem_wob)
        wob_copy.start()

        def weights(j):
            return (_pair_weights(wq_t, j, M), _pair_weights(wk_t, j, C),
                    _pair_weights(wv_t, j, C))

        half = S // 4
        nf = S // TP // 2

        def first(e, carry):
            ws = weights(0)
            for r in range(nf):
                p0 = pl.multiple_of(e * half + r * (TP // 2), TP // 2)
                for f in _b_proj_parts(p0, ws, bxp, cp, qb, kb, vb, 0):
                    f()
            return carry

        jax.lax.fori_loop(0, 2, first, 0)

        def body(h, carry):
            e = h % 2
            ws = weights(h // 2 + 1)
            wslot = 2 * ((h // 2 + 1) % 2)
            items = []
            for r in range(nf):
                p0 = pl.multiple_of(e * half + r * (TP // 2), TP // 2)
                items += _b_proj_parts(p0, ws, bxp, cp, qb, kb, vb, wslot)
            fillers = {}
            for j, pos in MAIN_PLACE:
                fillers.setdefault(pos, []).append(items[j])
            _b_head(h, h % 4, qb, kb, vb, ctx, MAIN_ORDER, MAIN_LAGS, fillers)
            return carry

        jax.lax.fori_loop(0, H - 2, body, 0)

        for h in range(H - 2, H):
            _b_head(h, h % 4, qb, kb, vb, ctx, TAIL_ORDER, TAIL_LAGS, {})

        wob_copy.wait()

        def out_copy(r):
            r0 = pl.multiple_of(r * TO, TO)
            return pltpu.make_async_copy(
                out_s.at[pl.ds(r0, TO), :], out_h.at[pl.ds(r0, TO), :], sem_out)

        def obody(r, carry):
            r0 = pl.multiple_of(r * TO, TO)
            p0 = pl.multiple_of(r * (TO // 2), TO // 2)
            oa = _a_attn_chunk(r * TO, TO, qp, kp, vp)
            cb = jnp.concatenate(
                [_unpack(ctx[h, pl.ds(p0, TO // 2), :]) for h in range(H)], axis=1)
            out_s[pl.ds(r0, TO), DA:DA + M] = _dot(cb, wob_v[...]).astype(bf16)
            woa = jnp.concatenate([_unpack(wop[nb]) for nb in range(8)], axis=1)
            out_s[pl.ds(r0, TO), 0:DA] = _dot(oa, woa).astype(bf16)
            out_copy(r).start()
            return carry

        jax.lax.fori_loop(0, S // TO, obody, 0)
        for r in range(S // TO):
            out_copy(r).wait()

    pl.run_scoped(
        phase_b,
        pltpu.VMEM((H, S // 2, D), u32), pltpu.VMEM((H * D, M), bf16))


@jax.jit
def pallas_concat_heads__sliding_local_dilated__compressed_kv_cla__prompt_kernel(
    A_x: jax.Array,
    A_wqkv: jax.Array,
    A_wo: jax.Array,
    B_x: jax.Array,
    B_c_kv: jax.Array,
    B_w_q: jax.Array,
    B_w_uk: jax.Array,
    B_w_uv: jax.Array,
    B_w_o: jax.Array,
):
    any_spec = pl.BlockSpec(memory_space=pl.ANY)
    out = pl.pallas_call(
        _kernel,
        out_shape=jax.ShapeDtypeStruct((S, DA + M), bf16),
        in_specs=[any_spec] * 9,
        out_specs=any_spec,
        scratch_shapes=[
            pltpu.VMEM((4, S // 2, D), u32),
            pltpu.VMEM((4, S // 2, D), u32),
            pltpu.VMEM((4, S // 2, D), u32),
            pltpu.VMEM((8, DA // 2, 128), u32),
            pltpu.VMEM((8, S + PADR, 128), f32),
            pltpu.VMEM((8, S + PADR, 128), f32),
            pltpu.VMEM((8, S + PADR, 128), f32),
            pltpu.VMEM((H // 2 * (M + 1) + 48, D), u32),
            pltpu.VMEM((H // 2 * (C + 1) + 48, D), u32),
            pltpu.VMEM((H // 2 * (C + 1) + 48, D), u32),
            pltpu.VMEM((S // 2, M), u32),
            pltpu.VMEM((S // 2, C), u32),
            pltpu.VMEM((S, DA + M), bf16),
            pltpu.SemaphoreType.DMA((24,)),
            pltpu.SemaphoreType.DMA((4,)),
            pltpu.SemaphoreType.DMA((28,)),
            pltpu.SemaphoreType.DMA(()),
            pltpu.SemaphoreType.DMA(()),
        ],
        compiler_params=pltpu.CompilerParams(vmem_limit_bytes=120 * 1024 * 1024),
    )(
        A_x.reshape(S, DA), A_wqkv, A_wo,
        B_x.reshape(S, M), B_c_kv.reshape(S, C),
        B_w_q.reshape(M * H, D), B_w_uk.reshape(C * H, D), B_w_uv.reshape(C * H, D),
        B_w_o.reshape(H * D, M),
    )
    return out.reshape(1, S, DA + M)
```

```python
import functools
import math

import jax
import jax.numpy as jnp
import jax.experimental.pallas as pl
import jax.experimental.pallas.tpu as pltpu

bf16 = jnp.bfloat16
f32 = jnp.float32
u32 = jnp.uint32

S = 2048
DA = 1024
HA = 32
DH = 32
WIN = 8
DIL = 2
M = 1024
C = 512
H = 32
D = 128
LOG2E = math.log2(math.e)
NEG = -1e30
PADR = 16
DP = HA + 1
TA = 512
TQ = 256
TP = 256
TO = 256
PACE = 6
A_PACE = 3
A_ROLLS = 5
NT = (((1,), (1,)), ((), ()))


def _unpack(x):
    return pltpu.bitcast(x, bf16)


def _pack(x):
    return pltpu.bitcast(x, u32)


def _dot(a, b):
    return jnp.dot(a, b, preferred_element_type=f32)


def _dot_nt(a, b):
    return jax.lax.dot_general(a, b, NT, preferred_element_type=f32)


def _zero_after(dep, rolls=2):
    for _ in range(rolls):
        dep = pltpu.roll(dep, 1, 1)
    return (dep >> 16) >> 16


def _or_tiled(x, z):
    row = jnp.concatenate([z] * (x.shape[1] // 128), axis=1)
    return x | jnp.concatenate([row] * (x.shape[0] // 8), axis=0)


def _prep_w_block(t, rb, wqkv_v, stage, wtp):
    r0 = pl.multiple_of(rb * 128, 128)
    for cb in range(8):
        c0 = t * DA + cb * 128
        tile = wqkv_v[pl.ds(r0, 128), c0:c0 + 128].astype(f32).T
        for hl in range(4):
            stage[pl.ds(4 * cb + hl, DH, stride=DP), :] = tile[hl * DH:(hl + 1) * DH, :]
    for d in range(DH):
        rows = stage[pl.ds(d * DP, HA), :]
        o0 = (t * DA + d * HA) // 2
        wtp[rb, o0:o0 + HA // 2, :] = _pack(rows.astype(bf16))


def _prep_wo_block(nb, wo_v, stage, wop, dep=None):
    z = None if dep is None else _zero_after(dep)
    for h in range(HA):
        rows = wo_v[nb, h * DH:(h + 1) * DH, :].astype(f32)
        if z is not None:
            rows = pltpu.bitcast(_or_tiled(pltpu.bitcast(rows, u32), z), f32)
        stage[pl.ds(h, DH, stride=DP), :] = rows
    for d in range(DH):
        rows = stage[pl.ds(d * DP, HA), :]
        wop[nb, d * (HA // 2):(d + 1) * (HA // 2), :] = _pack(rows.astype(bf16))
    return wop[nb, DA // 2 - 8:DA // 2, :]


NB = 512


def _a_proj(t, r, ax_v, wtp, dst):
    r0 = pl.multiple_of(r * TA, TA)
    x = ax_v[pl.ds(r0, TA), :]
    for n in range(DA // NB):
        f0 = (t * DA + n * NB) // 2
        w = jnp.concatenate(
            [_unpack(wtp[rb, f0:f0 + NB // 2, :]) for rb in range(8)], axis=1)
        y = _dot_nt(x, w)
        if t == 0:
            y = y * ((DH ** -0.5) * LOG2E)
        for cc in range(NB // 128):
            dst[n * (NB // 128) + cc, pl.ds(r0 + PADR, TA), :] = (
                y[:, cc * 128:(cc + 1) * 128])


def _a_attn_rows(row0, qp, kp, vp, masked, dep):
    G = 8
    q = [qp[c, pl.ds(row0 + PADR, G), :] for c in range(8)]
    if dep is not None:
        z = _zero_after(pltpu.bitcast(dep, u32), A_ROLLS)
        q = [pltpu.bitcast(pltpu.bitcast(x, u32) | z, f32) for x in q]
    if masked:
        pos = row0 + jax.lax.broadcasted_iota(jnp.int32, (G, 128), 0)
    logits = []
    for w in range(WIN):
        z = None
        for c in range(8):
            p = q[c] * kp[c, pl.ds(row0 + PADR - DIL * w, G), :]
            z = p if z is None else z + p
        z = z + pltpu.roll(z, 64, 1)
        z = z + pltpu.roll(z, 32, 1)
        if masked and w > 0:
            z = jnp.where(pos >= DIL * w, z, NEG)
        logits.append(z)
    m = logits[0]
    for w in range(1, WIN):
        m = jnp.maximum(m, logits[w])
    es = [jnp.exp2(z - m) for z in logits]
    l = es[0]
    for w in range(1, WIN):
        l = l + es[w]
    inv = 1.0 / l
    attn = [e * inv for e in es]
    outs = []
    for c in range(8):
        acc = None
        for w in range(WIN):
            v = vp[c, pl.ds(row0 + PADR - DIL * w, G), :]
            acc = attn[w] * v if acc is None else acc + attn[w] * v
        outs.append(acc)
    return outs


def _a_attn_chunk(row0, n, qp, kp, vp):
    units = []
    for g in range(n // 8):
        dep = units[g - A_PACE][7] if g >= A_PACE else None
        units.append(_a_attn_rows(row0 + g * 8, qp, kp, vp, g < 2, dep))
    return jnp.concatenate(
        [jnp.concatenate(u, axis=1) for u in units], axis=0).astype(bf16)


def _deinterleave_block(mb, raw, dst, rows, dep=None):
    pitch = rows + 1
    base = pl.multiple_of(mb * 8, 8)
    blk = _pack(raw[pl.ds(pl.multiple_of(base * H, 8 * H), 8 * H), :])
    if dep is not None:
        blk = _or_tiled(blk, _zero_after(dep))
    for mm in range(8):
        dst[pl.ds(base + mm, H // 2, stride=pitch), :] = (
            blk[mm * (H // 2):(mm + 1) * (H // 2), :])
    return dst[pl.ds(base + (H // 2 - 1) * pitch, 8), :]


def _repack_rows(row0, n, src, dst, dep=None):
    val = _pack(src[pl.ds(pl.multiple_of(row0, n), n), :])
    if dep is not None:
        val = _or_tiled(val, _zero_after(dep))
    dst[pl.ds(pl.multiple_of(row0 // 2, n // 2), n // 2), :] = val
    last = pl.multiple_of((row0 + n) // 2 - 8, 8)
    return dst[pl.ds(last, 8), val.shape[1] - 128:val.shape[1]]


def _pair_weights(wt, j, rows):
    w = wt[pl.ds(j * (rows + 1), rows), :]
    lo = pltpu.bitcast(w << 16, f32).astype(bf16)
    hi = pltpu.bitcast(w & jnp.uint32(0xFFFF0000), f32).astype(bf16)
    return jnp.concatenate([lo, hi], axis=1)


def _b_proj_parts(p0, ws, bxp, cp, qb, kb, vb, slot0):
    wq, wk, wv = ws
    rows = pl.ds(p0, TP // 2)

    def put(dst, y):
        for e in range(2):
            dst[slot0 + e, rows, :] = _pack(y[:, e * D:(e + 1) * D].astype(bf16))

    return [
        lambda: put(qb, _dot(_unpack(bxp[rows, :]), wq) * ((D ** -0.5) * LOG2E)),
        lambda: put(kb, _dot(_unpack(cp[rows, :]), wk)),
        lambda: put(vb, _dot(_unpack(cp[rows, :]), wv)),
    ]


HQ = TQ // 2


def _b_qk(i, qa, ka):
    k0 = i * TQ
    n = k0 + HQ
    q = qa[k0:k0 + TQ]
    s = _dot_nt(q, ka[0:n])
    s2 = _dot_nt(q[HQ:], ka[n:n + HQ])
    row = jax.lax.broadcasted_iota(jnp.int32, (HQ, 128), 0)
    col = jax.lax.broadcasted_iota(jnp.int32, (HQ, 128), 1)
    tri = col <= row
    nb = n // 128
    top = [s[:HQ, j * 128:(j + 1) * 128] for j in range(nb)]
    top[-1] = jnp.where(tri, top[-1], NEG)
    bot = [s[HQ:, j * 128:(j + 1) * 128] for j in range(nb)]
    bot.append(jnp.where(tri, s2, NEG))
    mps = []
    for blocks in (top, bot):
        mp = blocks[0]
        for c in blocks[1:]:
            mp = jnp.maximum(mp, c)
        mps.append(mp)
    return (top, bot), mps


def _b_softmax(blocks, mps, prev):
    ps, lps = [], []
    for half in range(2):
        mp = mps[half]
        if prev is not None:
            mp = jnp.maximum(mp, jnp.minimum(prev[half], NEG))
        m = jnp.max(mp, axis=1, keepdims=True)
        lp = None
        pl_ = []
        for jj, c in enumerate(blocks[half]):
            p = jnp.exp2(c - m)
            lp = p if lp is None else lp + p
            if jj == len(blocks[half]) - 1:
                p = p + jnp.minimum(lp, 0.0)
            pl_.append(p.astype(bf16))
        ps.append(pl_)
        lps.append(lp)
    return ps, lps


def _b_pv(i, ps, lps, va, ctx, h):
    k0 = i * TQ
    n = k0 + HQ
    nb = n // 128
    ls = [jnp.sum(lp, axis=1, keepdims=True) for lp in lps]
    pc = jnp.concatenate(
        [jnp.concatenate(ps[0], axis=1), jnp.concatenate(ps[1][:nb], axis=1)], axis=0)
    o = _dot(pc, va[0:n])
    o2 = _dot(ps[1][nb], va[n:n + HQ])
    o_top = o[:HQ] * (1.0 / ls[0])
    o_bot = (o[HQ:] + o2) * (1.0 / ls[1])
    ctx[h, k0 // 2:(k0 + HQ) // 2, :] = _pack(o_top.astype(bf16))
    ctx[h, (k0 + HQ) // 2:(k0 + TQ) // 2, :] = _pack(o_bot.astype(bf16))
    return (o_top, o_bot)


def _b_head(h, slot, qb, kb, vb, ctx, order, lags, fillers):
    qa, ka, va = _unpack(qb[slot]), _unpack(kb[slot]), _unpack(vb[slot])
    cur = _b_qk(order[0], qa, ka)
    outs = []
    for t, i in enumerate(order):
        nxt = _b_qk(order[t + 1], qa, ka) if t + 1 < len(order) else None
        for f in fillers.get(('a', t), ()):
            f()
        prev = outs[-lags[t]] if 0 < lags[t] <= len(outs) else None
        ps, lps = _b_softmax(cur[0], cur[1], prev)
        for f in fillers.get(('m', t), ()):
            f()
        outs.append(_b_pv(i, ps, lps, va, ctx, h))
        for f in fillers.get(('p', t), ()):
            f()
        cur = nxt


MAIN_ORDER = (1, 7, 3, 4, 6, 2, 5, 0)
MAIN_LAGS = (1, 1, 1, 1, 1, 0, 1, 1)
MAIN_PLACE = (
    (6, ('a', 6)), (0, ('m', 4)), (1, ('p', 0)), (4, ('p', 0)), (11, ('m', 7)),
    (3, ('m', 4)), (10, ('p', 3)), (7, ('m', 6)), (9, ('m', 4)), (2, ('a', 4)),
    (8, ('p', 6)), (5, ('m', 1)))
TAIL_ORDER = (1, 7, 3, 4, 2, 5, 6, 0)
TAIL_LAGS = (1, 1, 1, 1, 1, 1, 0, 2)


def _kernel(ax_h, wqkv_h, wo_h, bx_h, c_h, wq_h, wuk_h, wuv_h, wob_h, out_h,
            qb, kb, vb, wop, qp, kp, vp,
            wq_t, wk_t, wv_t, bxp, cp, out_s,
            sem_w, sem_ax, sem_f, sem_wob, sem_out, sem_oa):
    NR = S // TA

    def rows(ref, r, n):
        return ref.at[pl.ds(pl.multiple_of(r * n, n), n), :]

    def phase_a(ax_v, wqkv_v, wo_v, stage, wtp, bx_v, c_v, wq_raw, wuk_raw, wuv_raw):
        def w_copy(t, rb):
            r0 = pl.multiple_of(rb * 128, 128)
            sl = (pl.ds(r0, 128), slice(t * DA, (t + 1) * DA))
            return pltpu.make_async_copy(wqkv_h.at[sl], wqkv_v.at[sl],
                                         sem_w.at[8 * t + rb])

        def ax_copy(r):
            return pltpu.make_async_copy(rows(ax_h, r, TA), rows(ax_v, r, TA),
                                         sem_ax.at[r])

        def f_copy(r, i):
            sem = sem_f.at[7 * r + i]
            if i < 3:
                src, dst, n = ((wq_h, wq_raw, M), (wuk_h, wuk_raw, C),
                               (wuv_h, wuv_raw, C))[i]
                n = n * H // NR
                return pltpu.make_async_copy(rows(src, r, n), rows(dst, r, n), sem)
            if i < 5:
                src, dst = ((bx_h, bx_v), (c_h, c_v))[i - 3]
                return pltpu.make_async_copy(rows(src, r, TA), rows(dst, r, TA), sem)
            nb = 2 * r + (i - 5)
            c0 = pl.multiple_of(nb * 128, 128)
            return pltpu.make_async_copy(wo_h.at[:, pl.ds(c0, 128)], wo_v.at[nb], sem)

        sched = {
            0: [lambda: ax_copy(1), lambda: w_copy(1, 2), lambda: w_copy(1, 3)],
            1: [lambda: ax_copy(2), lambda: w_copy(1, 4), lambda: w_copy(1, 5)],
            2: [lambda: ax_copy(3), lambda: w_copy(1, 6), lambda: w_copy(1, 7)],
            3: [lambda: w_copy(2, 0), lambda: w_copy(2, 1)],
            4: [lambda: w_copy(2, 2), lambda: w_copy(2, 3)],
            5: [lambda: w_copy(2, 4), lambda: w_copy(2, 5)],
            6: [lambda: w_copy(2, 6), lambda: w_copy(2, 7)],
        }
        fslots = [
            [(0, 0)], [(0, 1), (0, 2), (0, 4)], [(0, 3), (0, 5), (0, 6), (1, 1)],
            [(1, 0), (1, 2)], [(1, 3), (1, 4), (1, 5), (1, 6), (2, 1)],
            [(2, 0), (2, 2)], [(2, 3), (2, 4), (2, 5), (2, 6)],
            [(3, 0), (3, 1)], [(3, 2), (3, 3), (3, 4), (3, 5), (3, 6)],
        ]
        for slot, items in enumerate(fslots):
            sched.setdefault(slot, []).extend(
                (lambda r=r, i=i: f_copy(r, i)) for r, i in items)

        def issue(t, r):
            for k in range(NR):
                items = sched.get(NR * t + k, [])
                if items:
                    @pl.when(r == k)
                    def _():
                        for mk in items:
                            mk().start()

        for rb in range(8):
            w_copy(0, rb).start()
        ax_copy(0).start()
        w_copy(1, 0).start()
        w_copy(1, 1).start()
        for ref in (kp, vp):
            ref[:, 0:PADR, :] = jnp.zeros((8, PADR, 128), f32)

        def prep0(rb, carry):
            w_copy(0, rb).wait()
            _prep_w_block(0, rb, wqkv_v, stage.at[0], wtp)
            return carry

        jax.lax.fori_loop(0, 8, prep0, 0)

        def qk_step(t):
            def body(r, carry):
                if t == 0:
                    ax_copy(r).wait()
                w_copy(t + 1, 2 * r).wait()
                w_copy(t + 1, 2 * r + 1).wait()
                issue(t, r)
                _a_proj(t, r, ax_v, wtp, (qp, kp)[t])
                for i in range(2):
                    _prep_w_block(t + 1, 2 * r + i, wqkv_v, stage.at[i], wtp)
                return carry
            return body

        jax.lax.fori_loop(0, NR, qk_step(0), 0)
        jax.lax.fori_loop(0, NR, qk_step(1), 0)

        def v_step(r, carry):
            for i in range(7):
                f_copy(r, i).wait()
            issue(2, r)
            _a_proj(2, r, ax_v, wtp, vp)
            nq = M // 8 // NR
            nk = C // 8 // NR
            items = (
                [functools.partial(_deinterleave_block, r * nq + i, wq_raw, wq_t, M)
                 for i in range(nq)]
                + [functools.partial(_deinterleave_block, r * nk + i, wuk_raw, wk_t, C)
                   for i in range(nk)]
                + [functools.partial(_deinterleave_block, r * nk + i, wuv_raw, wv_t, C)
                   for i in range(nk)]
                + [functools.partial(_prep_wo_block, 2 * r + i, wo_v, stage.at[i], wop)
                   for i in range(2)]
                + [functools.partial(_repack_rows, r * TA + i * 32, 32, bx_v, bxp)
                   for i in range(TA // 32)]
                + [functools.partial(_repack_rows, r * TA + i * 64, 64, c_v, cp)
                   for i in range(TA // 64)])
            backs = []
            for idx, f in enumerate(items):
                backs.append(f(backs[idx - PACE] if idx >= PACE else None))
            return carry

        jax.lax.fori_loop(0, NR, v_step, 0)

    pl.run_scoped(
        phase_a,
        pltpu.VMEM((S, DA), bf16), pltpu.VMEM((DA, 3 * DA), bf16),
        pltpu.VMEM((8, DA, 128), bf16), pltpu.VMEM((2, HA * DP, 128), f32),
        pltpu.VMEM((8, 3 * DA // 2, 128), u32),
        pltpu.VMEM((S, M), bf16), pltpu.VMEM((S, C), bf16),
        pltpu.VMEM((M * H, D), bf16), pltpu.VMEM((C * H, D), bf16),
        pltpu.VMEM((C * H, D), bf16))

    def phase_b(ctx, wob_v):
        wob_copy = pltpu.make_async_copy(wob_h, wob_v, sem_wob)
        wob_copy.start()

        def weights(j):
            return (_pair_weights(wq_t, j, M), _pair_weights(wk_t, j, C),
                    _pair_weights(wv_t, j, C))

        half = S // 4
        nf = S // TP // 2

        def first(e, carry):
            ws = weights(0)
            for r in range(nf):
                p0 = pl.multiple_of(e * half + r * (TP // 2), TP // 2)
                for f in _b_proj_parts(p0, ws, bxp, cp, qb, kb, vb, 0):
                    f()
            return carry

        jax.lax.fori_loop(0, 2, first, 0)

        def body(h, carry):
            e = h % 2
            ws = weights(h // 2 + 1)
            wslot = 2 * ((h // 2 + 1) % 2)
            items = []
            for r in range(nf):
                p0 = pl.multiple_of(e * half + r * (TP // 2), TP // 2)
                items += _b_proj_parts(p0, ws, bxp, cp, qb, kb, vb, wslot)
            fillers = {}
            for j, pos in MAIN_PLACE:
                fillers.setdefault(pos, []).append(items[j])
            _b_head(h, h % 4, qb, kb, vb, ctx, MAIN_ORDER, MAIN_LAGS, fillers)
            return carry

        jax.lax.fori_loop(0, H - 2, body, 0)

        for h in range(H - 2, H):
            _b_head(h, h % 4, qb, kb, vb, ctx, TAIL_ORDER, TAIL_LAGS, {})

        wob_copy.wait()

        def out_copy(r, c0, n, sem):
            sl = (pl.ds(pl.multiple_of(r * TO, TO), TO), slice(c0, c0 + n))
            return pltpu.make_async_copy(out_s.at[sl], out_h.at[sl], sem)

        def obody(r, carry):
            r0 = pl.multiple_of(r * TO, TO)
            p0 = pl.multiple_of(r * (TO // 2), TO // 2)
            oa = _a_attn_chunk(r * TO, TO, qp, kp, vp)
            cb = jnp.concatenate(
                [_unpack(ctx[h, pl.ds(p0, TO // 2), :]) for h in range(H)], axis=1)
            out_s[pl.ds(r0, TO), DA:DA + M] = _dot(cb, wob_v[...]).astype(bf16)
            out_copy(r, DA, M, sem_out).start()
            for n in range(2):
                c0 = n * (DA // 2)
                woa = jnp.concatenate(
                    [_unpack(wop[nb]) for nb in range(4 * n, 4 * n + 4)], axis=1)
                out_s[pl.ds(r0, TO), c0:c0 + DA // 2] = _dot(oa, woa).astype(bf16)
                out_copy(r, c0, DA // 2, sem_oa).start()
            return carry

        jax.lax.fori_loop(0, S // TO, obody, 0)
        for r in range(S // TO):
            out_copy(r, DA, M, sem_out).wait()
            for n in range(2):
                out_copy(r, n * (DA // 2), DA // 2, sem_oa).wait()

    pl.run_scoped(
        phase_b,
        pltpu.VMEM((H, S // 2, D), u32), pltpu.VMEM((H * D, M), bf16))


@jax.jit
def pallas_concat_heads__sliding_local_dilated__compressed_kv_cla__prompt_kernel(
    A_x: jax.Array,
    A_wqkv: jax.Array,
    A_wo: jax.Array,
    B_x: jax.Array,
    B_c_kv: jax.Array,
    B_w_q: jax.Array,
    B_w_uk: jax.Array,
    B_w_uv: jax.Array,
    B_w_o: jax.Array,
):
    any_spec = pl.BlockSpec(memory_space=pl.ANY)
    out = pl.pallas_call(
        _kernel,
        out_shape=jax.ShapeDtypeStruct((S, DA + M), bf16),
        in_specs=[any_spec] * 9,
        out_specs=any_spec,
        scratch_shapes=[
            pltpu.VMEM((4, S // 2, D), u32),
            pltpu.VMEM((4, S // 2, D), u32),
            pltpu.VMEM((4, S // 2, D), u32),
            pltpu.VMEM((8, DA // 2, 128), u32),
            pltpu.VMEM((8, S + PADR, 128), f32),
            pltpu.VMEM((8, S + PADR, 128), f32),
            pltpu.VMEM((8, S + PADR, 128), f32),
            pltpu.VMEM((H // 2 * (M + 1) + 48, D), u32),
            pltpu.VMEM((H // 2 * (C + 1) + 48, D), u32),
            pltpu.VMEM((H // 2 * (C + 1) + 48, D), u32),
            pltpu.VMEM((S // 2, M), u32),
            pltpu.VMEM((S // 2, C), u32),
            pltpu.VMEM((S, DA + M), bf16),
            pltpu.SemaphoreType.DMA((24,)),
            pltpu.SemaphoreType.DMA((4,)),
            pltpu.SemaphoreType.DMA((28,)),
            pltpu.SemaphoreType.DMA(()),
            pltpu.SemaphoreType.DMA(()),
            pltpu.SemaphoreType.DMA(()),
        ],
        compiler_params=pltpu.CompilerParams(vmem_limit_bytes=120 * 1024 * 1024),
    )(
        A_x.reshape(S, DA), A_wqkv, A_wo,
        B_x.reshape(S, M), B_c_kv.reshape(S, C),
        B_w_q.reshape(M * H, D), B_w_uk.reshape(C * H, D), B_w_uv.reshape(C * H, D),
        B_w_o.reshape(H * D, M),
    )
    return out.reshape(1, S, DA + M)
```

```python
import functools
import math

import jax
import jax.numpy as jnp
import jax.experimental.pallas as pl
import jax.experimental.pallas.tpu as pltpu

bf16 = jnp.bfloat16
f32 = jnp.float32
u32 = jnp.uint32

S = 2048
DA = 1024
HA = 32
DH = 32
WIN = 8
DIL = 2
M = 1024
C = 512
H = 32
D = 128
LOG2E = math.log2(math.e)
NEG = -1e30
PADR = 16
DP = HA + 1
TA = 512
TQ = 256
TP = 256
TO = 256
PACE = 6
A_PACE = 3
A_ROLLS = 5
NT = (((1,), (1,)), ((), ()))


def _unpack(x):
    return pltpu.bitcast(x, bf16)


def _pack(x):
    return pltpu.bitcast(x, u32)


def _dot(a, b):
    return jnp.dot(a, b, preferred_element_type=f32)


def _dot_nt(a, b):
    return jax.lax.dot_general(a, b, NT, preferred_element_type=f32)


def _zero_after(dep, rolls=2):
    for _ in range(rolls):
        dep = pltpu.roll(dep, 1, 1)
    return (dep >> 16) >> 16


def _or_tiled(x, z):
    row = jnp.concatenate([z] * (x.shape[1] // 128), axis=1)
    return x | jnp.concatenate([row] * (x.shape[0] // 8), axis=0)


def _prep_w_block(t, rb, wqkv_v, stage, wtp):
    r0 = pl.multiple_of(rb * 128, 128)
    for cb in range(8):
        c0 = t * DA + cb * 128
        tile = wqkv_v[pl.ds(r0, 128), c0:c0 + 128].astype(f32).T
        for hl in range(4):
            stage[pl.ds(4 * cb + hl, DH, stride=DP), :] = tile[hl * DH:(hl + 1) * DH, :]
    for d in range(DH):
        rows = stage[pl.ds(d * DP, HA), :]
        o0 = (t * DA + d * HA) // 2
        wtp[rb, o0:o0 + HA // 2, :] = _pack(rows.astype(bf16))


def _prep_wo_block(nb, wo_v, stage, wop, dep=None):
    z = None if dep is None else _zero_after(dep)
    for h in range(HA):
        rows = wo_v[nb, h * DH:(h + 1) * DH, :].astype(f32)
        if z is not None:
            rows = pltpu.bitcast(_or_tiled(pltpu.bitcast(rows, u32), z), f32)
        stage[pl.ds(h, DH, stride=DP), :] = rows
    for d in range(DH):
        rows = stage[pl.ds(d * DP, HA), :]
        wop[nb, d * (HA // 2):(d + 1) * (HA // 2), :] = _pack(rows.astype(bf16))
    return wop[nb, DA // 2 - 8:DA // 2, :]


NB = 512


def _a_proj(t, r, ax_v, wtp, dst):
    r0 = pl.multiple_of(r * TA, TA)
    x = ax_v[pl.ds(r0, TA), :]
    for n in range(DA // NB):
        f0 = (t * DA + n * NB) // 2
        w = jnp.concatenate(
            [_unpack(wtp[rb, f0:f0 + NB // 2, :]) for rb in range(8)], axis=1)
        y = _dot_nt(x, w)
        if t == 0:
            y = y * ((DH ** -0.5) * LOG2E)
        for cc in range(NB // 128):
            dst[n * (NB // 128) + cc, pl.ds(r0 + PADR, TA), :] = (
                y[:, cc * 128:(cc + 1) * 128])


def _a_attn_rows(row0, qp, kp, vp, masked, dep):
    G = 8
    q = [qp[c, pl.ds(row0 + PADR, G), :] for c in range(8)]
    if dep is not None:
        z = _zero_after(pltpu.bitcast(dep, u32), A_ROLLS)
        q = [pltpu.bitcast(pltpu.bitcast(x, u32) | z, f32) for x in q]
    if masked:
        pos = row0 + jax.lax.broadcasted_iota(jnp.int32, (G, 128), 0)
    logits = []
    for w in range(WIN):
        z = None
        for c in range(8):
            p = q[c] * kp[c, pl.ds(row0 + PADR - DIL * w, G), :]
            z = p if z is None else z + p
        z = z + pltpu.roll(z, 64, 1)
        z = z + pltpu.roll(z, 32, 1)
        if masked and w > 0:
            z = jnp.where(pos >= DIL * w, z, NEG)
        logits.append(z)
    m = logits[0]
    for w in range(1, WIN):
        m = jnp.maximum(m, logits[w])
    es = [jnp.exp2(z - m) for z in logits]
    l = es[0]
    for w in range(1, WIN):
        l = l + es[w]
    inv = 1.0 / l
    attn = [e * inv for e in es]
    outs = []
    for c in range(8):
        acc = None
        for w in range(WIN):
            v = vp[c, pl.ds(row0 + PADR - DIL * w, G), :]
            acc = attn[w] * v if acc is None else acc + attn[w] * v
        outs.append(acc)
    return outs


def _a_attn_chunk(row0, n, qp, kp, vp):
    units = []
    for g in range(n // 8):
        dep = units[g - A_PACE][7] if g >= A_PACE else None
        units.append(_a_attn_rows(row0 + g * 8, qp, kp, vp, g < 2, dep))
    return jnp.concatenate(
        [jnp.concatenate(u, axis=1) for u in units], axis=0).astype(bf16)


def _deinterleave_block(mb, raw, dst, rows, dep=None):
    pitch = rows + 1
    base = pl.multiple_of(mb * 8, 8)
    blk = _pack(raw[pl.ds(pl.multiple_of(base * H, 8 * H), 8 * H), :])
    if dep is not None:
        blk = _or_tiled(blk, _zero_after(dep))
    for mm in range(8):
        dst[pl.ds(base + mm, H // 2, stride=pitch), :] = (
            blk[mm * (H // 2):(mm + 1) * (H // 2), :])
    return dst[pl.ds(base + (H // 2 - 1) * pitch, 8), :]


def _repack_rows(row0, n, src, dst, dep=None):
    val = _pack(src[pl.ds(pl.multiple_of(row0, n), n), :])
    if dep is not None:
        val = _or_tiled(val, _zero_after(dep))
    dst[pl.ds(pl.multiple_of(row0 // 2, n // 2), n // 2), :] = val
    last = pl.multiple_of((row0 + n) // 2 - 8, 8)
    return dst[pl.ds(last, 8), val.shape[1] - 128:val.shape[1]]


def _pair_weights(wt, j, rows):
    w = wt[pl.ds(j * (rows + 1), rows), :]
    lo = pltpu.bitcast(w << 16, f32).astype(bf16)
    hi = pltpu.bitcast(w & jnp.uint32(0xFFFF0000), f32).astype(bf16)
    return jnp.concatenate([lo, hi], axis=1)


def _b_proj_parts(p0, ws, bxp, cp, qb, kb, vb, slot0):
    wq, wk, wv = ws
    rows = pl.ds(p0, TP // 2)

    def put(dst, y):
        for e in range(2):
            dst[slot0 + e, rows, :] = _pack(y[:, e * D:(e + 1) * D].astype(bf16))

    return [
        lambda: put(qb, _dot(_unpack(bxp[rows, :]), wq) * ((D ** -0.5) * LOG2E)),
        lambda: put(kb, _dot(_unpack(cp[rows, :]), wk)),
        lambda: put(vb, _dot(_unpack(cp[rows, :]), wv)),
    ]


HQ = TQ // 2


def _b_qk(i, qa, ka):
    k0 = i * TQ
    n = k0 + HQ
    q = qa[k0:k0 + TQ]
    s = _dot_nt(q, ka[0:n])
    s2 = _dot_nt(q[HQ:], ka[n:n + HQ])
    row = jax.lax.broadcasted_iota(jnp.int32, (HQ, 128), 0)
    col = jax.lax.broadcasted_iota(jnp.int32, (HQ, 128), 1)
    tri = col <= row
    nb = n // 128
    top = [s[:HQ, j * 128:(j + 1) * 128] for j in range(nb)]
    top[-1] = jnp.where(tri, top[-1], NEG)
    bot = [s[HQ:, j * 128:(j + 1) * 128] for j in range(nb)]
    bot.append(jnp.where(tri, s2, NEG))
    mps = []
    for blocks in (top, bot):
        mp = blocks[0]
        for c in blocks[1:]:
            mp = jnp.maximum(mp, c)
        mps.append(mp)
    return (top, bot), mps


def _b_softmax(blocks, mps, prev):
    ps, lps = [], []
    for half in range(2):
        mp = mps[half]
        if prev is not None:
            mp = jnp.maximum(mp, jnp.minimum(prev[half], NEG))
        m = jnp.max(mp, axis=1, keepdims=True)
        lp = None
        pl_ = []
        for jj, c in enumerate(blocks[half]):
            p = jnp.exp2(c - m)
            lp = p if lp is None else lp + p
            if jj == len(blocks[half]) - 1:
                p = p + jnp.minimum(lp, 0.0)
            pl_.append(p.astype(bf16))
        ps.append(pl_)
        lps.append(lp)
    return ps, lps


def _b_pv(i, ps, lps, va, ctx, h):
    k0 = i * TQ
    n = k0 + HQ
    nb = n // 128
    ls = [jnp.sum(lp, axis=1, keepdims=True) for lp in lps]
    pc = jnp.concatenate(
        [jnp.concatenate(ps[0], axis=1), jnp.concatenate(ps[1][:nb], axis=1)], axis=0)
    o = _dot(pc, va[0:n])
    o2 = _dot(ps[1][nb], va[n:n + HQ])
    o_top = o[:HQ] * (1.0 / ls[0])
    o_bot = (o[HQ:] + o2) * (1.0 / ls[1])
    ctx[h, k0 // 2:(k0 + HQ) // 2, :] = _pack(o_top.astype(bf16))
    ctx[h, (k0 + HQ) // 2:(k0 + TQ) // 2, :] = _pack(o_bot.astype(bf16))
    return (o_top, o_bot)


def _b_head(h, slot, qb, kb, vb, ctx, order, lags, fillers):
    qa, ka, va = _unpack(qb[slot]), _unpack(kb[slot]), _unpack(vb[slot])
    cur = _b_qk(order[0], qa, ka)
    outs = []
    for t, i in enumerate(order):
        nxt = _b_qk(order[t + 1], qa, ka) if t + 1 < len(order) else None
        for f in fillers.get(('a', t), ()):
            f()
        prev = outs[-lags[t]] if 0 < lags[t] <= len(outs) else None
        ps, lps = _b_softmax(cur[0], cur[1], prev)
        for f in fillers.get(('m', t), ()):
            f()
        outs.append(_b_pv(i, ps, lps, va, ctx, h))
        for f in fillers.get(('p', t), ()):
            f()
        cur = nxt


MAIN_ORDER = (1, 7, 3, 4, 6, 2, 5, 0)
MAIN_LAGS = (1, 1, 1, 1, 1, 0, 1, 1)
MAIN_PLACE = (
    (6, ('a', 6)), (0, ('m', 4)), (1, ('p', 0)), (4, ('p', 0)), (11, ('m', 7)),
    (3, ('m', 4)), (10, ('p', 3)), (7, ('m', 6)), (9, ('m', 4)), (2, ('a', 4)),
    (8, ('p', 6)), (5, ('m', 1)))
TAIL_ORDER = (1, 7, 3, 4, 2, 5, 6, 0)
TAIL_LAGS = (1, 1, 1, 1, 1, 1, 0, 2)


def _kernel(ax_h, wqkv_h, wo_h, bx_h, c_h, wq_h, wuk_h, wuv_h, wob_h, out_h,
            qb, kb, vb, wop, qp, kp, vp,
            wq_t, wk_t, wv_t, bxp, cp, out_s,
            sem_w, sem_ax, sem_x0, sem_f, sem_wob, sem_out, sem_oa):
    NR = S // TA

    def rows(ref, r, n):
        return ref.at[pl.ds(pl.multiple_of(r * n, n), n), :]

    def phase_a(ax_v, x0, wqkv_v, wo_v, stage, wtp, bx_v, c_v,
                wq_raw, wuk_raw, wuv_raw):
        def w_copy(t, rb):
            r0 = pl.multiple_of(rb * 128, 128)
            sl = (pl.ds(r0, 128), slice(t * DA, (t + 1) * DA))
            return pltpu.make_async_copy(wqkv_h.at[sl], wqkv_v.at[sl],
                                         sem_w.at[8 * t + rb])

        def ax_copy(r):
            return pltpu.make_async_copy(rows(ax_h, r, TA), rows(ax_v, r, TA),
                                         sem_ax.at[r])

        def x0_copy(rb):
            c0 = pl.multiple_of(rb * 128, 128)
            return pltpu.make_async_copy(ax_h.at[0:TA, pl.ds(c0, 128)], x0.at[rb],
                                         sem_x0.at[rb])

        def f_copy(r, i):
            sem = sem_f.at[7 * r + i]
            if i < 3:
                src, dst, n = ((wq_h, wq_raw, M), (wuk_h, wuk_raw, C),
                               (wuv_h, wuv_raw, C))[i]
                n = n * H // NR
                return pltpu.make_async_copy(rows(src, r, n), rows(dst, r, n), sem)
            if i < 5:
                src, dst = ((bx_h, bx_v), (c_h, c_v))[i - 3]
                return pltpu.make_async_copy(rows(src, r, TA), rows(dst, r, TA), sem)
            nb = 2 * r + (i - 5)
            c0 = pl.multiple_of(nb * 128, 128)
            return pltpu.make_async_copy(wo_h.at[:, pl.ds(c0, 128)], wo_v.at[nb], sem)

        W = lambda t, rb: (lambda: w_copy(t, rb))
        X = lambda r: (lambda: ax_copy(r))
        F = lambda r, i: (lambda: f_copy(r, i))
        sched = {
            1: [X(2), W(1, 3), W(1, 4), W(1, 5), F(0, 0)],
            2: [X(3), W(1, 6), W(1, 7), X(0), F(0, 1)],
            3: [W(2, 0), W(2, 1), F(0, 2), F(0, 4), F(0, 3), F(0, 5), F(0, 6)],
            4: [W(2, 2), W(2, 3), F(1, 0), F(1, 1)],
            5: [W(2, 4), W(2, 5), F(1, 2), F(1, 3), F(1, 4), F(1, 5), F(1, 6)],
            6: [W(2, 6), W(2, 7), F(2, 0), F(2, 1)],
            7: [F(2, 2), F(2, 3), F(2, 4), F(2, 5), F(2, 6)],
            8: [F(3, 0), F(3, 1)],
            9: [F(3, 2), F(3, 3), F(3, 4), F(3, 5), F(3, 6)],
        }

        def issue_at(table, idx, keys):
            for k in keys:
                items = table.get(k, [])
                if items:
                    @pl.when(idx == k)
                    def _():
                        for mk in items:
                            mk().start()

        def issue(t, r):
            issue_at({k - NR * t: v for k, v in sched.items()}, r, range(NR))

        w_copy(0, 0).start()
        x0_copy(0).start()
        w_copy(0, 1).start()
        x0_copy(1).start()
        w_copy(0, 2).start()
        for ref in (kp, vp):
            ref[:, 0:PADR, :] = jnp.zeros((8, PADR, 128), f32)
        qp[:, PADR:PADR + TA, :] = jnp.zeros((8, TA, 128), f32)
        w_copy(0, 0).wait()
        _prep_w_block(0, 0, wqkv_v, stage.at[0], wtp)
        early = {k: ([lambda k=k: x0_copy(k + 2)] if k + 2 < 8 else [])
                 + ([W(0, k + 3)] if k + 3 < 8 else []) for k in range(8)}
        early[4].append(X(1))
        early[5] += [W(1, 0), W(1, 1)]
        early[6].append(W(1, 2))

        def q0_step(rb, carry):
            x0_copy(rb).wait()

            @pl.when(rb < 7)
            def _():
                w_copy(0, rb + 1).wait()

            issue_at(early, rb, range(8))
            y = _dot_nt(x0[rb], _unpack(wtp[rb, 0:DA // 2, :]))
            y = y * ((DH ** -0.5) * LOG2E)
            for c in range(8):
                qp[c, PADR:PADR + TA, :] += y[:, c * 128:(c + 1) * 128]
            _prep_w_block(0, jnp.minimum(rb + 1, 7), wqkv_v, stage.at[1], wtp)
            return carry

        jax.lax.fori_loop(0, 8, q0_step, 0)

        def q_step(r, carry):
            ax_copy(r).wait()
            for i in range(3):
                @pl.when(3 * (r - 1) + i < 8)
                def _():
                    w_copy(1, 3 * (r - 1) + i).wait()
            issue(0, r)
            _a_proj(0, r, ax_v, wtp, qp)
            for i in range(3):
                _prep_w_block(1, jnp.minimum(3 * (r - 1) + i, 7), wqkv_v,
                              stage.at[i], wtp)
            return carry

        jax.lax.fori_loop(1, NR, q_step, 0)

        def k_step(r, carry):
            @pl.when(r == 0)
            def _():
                ax_copy(0).wait()

            w_copy(2, 2 * r).wait()
            w_copy(2, 2 * r + 1).wait()
            issue(1, r)
            _a_proj(1, r, ax_v, wtp, kp)
            for i in range(2):
                _prep_w_block(2, 2 * r + i, wqkv_v, stage.at[i], wtp)
            return carry

        jax.lax.fori_loop(0, NR, k_step, 0)

        def v_step(r, carry):
            for i in range(7):
                f_copy(r, i).wait()
            issue(2, r)
            _a_proj(2, r, ax_v, wtp, vp)
            nq = M // 8 // NR
            nk = C // 8 // NR
            items = (
                [functools.partial(_deinterleave_block, r * nq + i, wq_raw, wq_t, M)
                 for i in range(nq)]
                + [functools.partial(_deinterleave_block, r * nk + i, wuk_raw, wk_t, C)
                   for i in range(nk)]
                + [functools.partial(_deinterleave_block, r * nk + i, wuv_raw, wv_t, C)
                   for i in range(nk)]
                + [functools.partial(_prep_wo_block, 2 * r + i, wo_v, stage.at[i], wop)
                   for i in range(2)]
                + [functools.partial(_repack_rows, r * TA + i * 32, 32, bx_v, bxp)
                   for i in range(TA // 32)]
                + [functools.partial(_repack_rows, r * TA + i * 64, 64, c_v, cp)
                   for i in range(TA // 64)])
            backs = []
            for idx, f in enumerate(items):
                backs.append(f(backs[idx - PACE] if idx >= PACE else None))
            return carry

        jax.lax.fori_loop(0, NR, v_step, 0)

    pl.run_scoped(
        phase_a,
        pltpu.VMEM((S, DA), bf16), pltpu.VMEM((8, TA, 128), bf16),
        pltpu.VMEM((DA, 3 * DA), bf16),
        pltpu.VMEM((8, DA, 128), bf16), pltpu.VMEM((4, HA * DP, 128), f32),
        pltpu.VMEM((8, 3 * DA // 2, 128), u32),
        pltpu.VMEM((S, M), bf16), pltpu.VMEM((S, C), bf16),
        pltpu.VMEM((M * H, D), bf16), pltpu.VMEM((C * H, D), bf16),
        pltpu.VMEM((C * H, D), bf16))

    def phase_b(ctx, wob_v):
        wob_copy = pltpu.make_async_copy(wob_h, wob_v, sem_wob)
        wob_copy.start()

        def weights(j):
            return (_pair_weights(wq_t, j, M), _pair_weights(wk_t, j, C),
                    _pair_weights(wv_t, j, C))

        half = S // 4
        nf = S // TP // 2

        def first(e, carry):
            ws = weights(0)
            for r in range(nf):
                p0 = pl.multiple_of(e * half + r * (TP // 2), TP // 2)
                for f in _b_proj_parts(p0, ws, bxp, cp, qb, kb, vb, 0):
                    f()
            return carry

        jax.lax.fori_loop(0, 2, first, 0)

        def body(h, carry):
            e = h % 2
            ws = weights(h // 2 + 1)
            wslot = 2 * ((h // 2 + 1) % 2)
            items = []
            for r in range(nf):
                p0 = pl.multiple_of(e * half + r * (TP // 2), TP // 2)
                items += _b_proj_parts(p0, ws, bxp, cp, qb, kb, vb, wslot)
            fillers = {}
            for j, pos in MAIN_PLACE:
                fillers.setdefault(pos, []).append(items[j])
            _b_head(h, h % 4, qb, kb, vb, ctx, MAIN_ORDER, MAIN_LAGS, fillers)
            return carry

        jax.lax.fori_loop(0, H - 2, body, 0)

        for h in range(H - 2, H):
            _b_head(h, h % 4, qb, kb, vb, ctx, TAIL_ORDER, TAIL_LAGS, {})

        wob_copy.wait()

        def out_copy(r, c0, n, sem):
            sl = (pl.ds(pl.multiple_of(r * TO, TO), TO), slice(c0, c0 + n))
            return pltpu.make_async_copy(out_s.at[sl], out_h.at[sl], sem)

        def obody(r, carry):
            r0 = pl.multiple_of(r * TO, TO)
            p0 = pl.multiple_of(r * (TO // 2), TO // 2)
            oa = _a_attn_chunk(r * TO, TO, qp, kp, vp)
            cb = jnp.concatenate(
                [_unpack(ctx[h, pl.ds(p0, TO // 2), :]) for h in range(H)], axis=1)
            out_s[pl.ds(r0, TO), DA:DA + M] = _dot(cb, wob_v[...]).astype(bf16)
            out_copy(r, DA, M, sem_out).start()
            for n in range(2):
                c0 = n * (DA // 2)
                woa = jnp.concatenate(
                    [_unpack(wop[nb]) for nb in range(4 * n, 4 * n + 4)], axis=1)
                out_s[pl.ds(r0, TO), c0:c0 + DA // 2] = _dot(oa, woa).astype(bf16)
                out_copy(r, c0, DA // 2, sem_oa).start()
            return carry

        jax.lax.fori_loop(0, S // TO, obody, 0)
        for r in range(S // TO):
            out_copy(r, DA, M, sem_out).wait()
            for n in range(2):
                out_copy(r, n * (DA // 2), DA // 2, sem_oa).wait()

    pl.run_scoped(
        phase_b,
        pltpu.VMEM((H, S // 2, D), u32), pltpu.VMEM((H * D, M), bf16))


@jax.jit
def pallas_concat_heads__sliding_local_dilated__compressed_kv_cla__prompt_kernel(
    A_x: jax.Array,
    A_wqkv: jax.Array,
    A_wo: jax.Array,
    B_x: jax.Array,
    B_c_kv: jax.Array,
    B_w_q: jax.Array,
    B_w_uk: jax.Array,
    B_w_uv: jax.Array,
    B_w_o: jax.Array,
):
    any_spec = pl.BlockSpec(memory_space=pl.ANY)
    out = pl.pallas_call(
        _kernel,
        out_shape=jax.ShapeDtypeStruct((S, DA + M), bf16),
        in_specs=[any_spec] * 9,
        out_specs=any_spec,
        scratch_shapes=[
            pltpu.VMEM((4, S // 2, D), u32),
            pltpu.VMEM((4, S // 2, D), u32),
            pltpu.VMEM((4, S // 2, D), u32),
            pltpu.VMEM((8, DA // 2, 128), u32),
            pltpu.VMEM((8, S + PADR, 128), f32),
            pltpu.VMEM((8, S + PADR, 128), f32),
            pltpu.VMEM((8, S + PADR, 128), f32),
            pltpu.VMEM((H // 2 * (M + 1) + 48, D), u32),
            pltpu.VMEM((H // 2 * (C + 1) + 48, D), u32),
            pltpu.VMEM((H // 2 * (C + 1) + 48, D), u32),
            pltpu.VMEM((S // 2, M), u32),
            pltpu.VMEM((S // 2, C), u32),
            pltpu.VMEM((S, DA + M), bf16),
            pltpu.SemaphoreType.DMA((24,)),
            pltpu.SemaphoreType.DMA((4,)),
            pltpu.SemaphoreType.DMA((8,)),
            pltpu.SemaphoreType.DMA((28,)),
            pltpu.SemaphoreType.DMA(()),
            pltpu.SemaphoreType.DMA(()),
            pltpu.SemaphoreType.DMA(()),
        ],
        compiler_params=pltpu.CompilerParams(vmem_limit_bytes=120 * 1024 * 1024),
    )(
        A_x.reshape(S, DA), A_wqkv, A_wo,
        B_x.reshape(S, M), B_c_kv.reshape(S, C),
        B_w_q.reshape(M * H, D), B_w_uk.reshape(C * H, D), B_w_uv.reshape(C * H, D),
        B_w_o.reshape(H * D, M),
    )
    return out.reshape(1, S, DA + M)
```

```python
import functools
import math

import jax
import jax.numpy as jnp
import jax.experimental.pallas as pl
import jax.experimental.pallas.tpu as pltpu

bf16 = jnp.bfloat16
f32 = jnp.float32
u32 = jnp.uint32

S = 2048
DA = 1024
HA = 32
DH = 32
WIN = 8
DIL = 2
M = 1024
C = 512
H = 32
D = 128
LOG2E = math.log2(math.e)
NEG = -1e30
PADR = 16
DP = HA + 1
TA = 512
Q0 = 1024
TQ = 256
TP = 256
TO = 256
PACE = 6
A_PACE = 3
A_ROLLS = 5
NT = (((1,), (1,)), ((), ()))


def _unpack(x):
    return pltpu.bitcast(x, bf16)


def _pack(x):
    return pltpu.bitcast(x, u32)


def _dot(a, b):
    return jnp.dot(a, b, preferred_element_type=f32)


def _dot_nt(a, b):
    return jax.lax.dot_general(a, b, NT, preferred_element_type=f32)


def _zero_after(dep, rolls=2):
    for _ in range(rolls):
        dep = pltpu.roll(dep, 1, 1)
    return (dep >> 16) >> 16


def _or_tiled(x, z):
    row = jnp.concatenate([z] * (x.shape[1] // 128), axis=1)
    return x | jnp.concatenate([row] * (x.shape[0] // 8), axis=0)


def _prep_w_block(t, rb, wqkv_v, stage, wtp):
    r0 = pl.multiple_of(rb * 128, 128)
    for cb in range(8):
        c0 = t * DA + cb * 128
        tile = wqkv_v[pl.ds(r0, 128), c0:c0 + 128].astype(f32).T
        for hl in range(4):
            stage[pl.ds(4 * cb + hl, DH, stride=DP), :] = tile[hl * DH:(hl + 1) * DH, :]
    for d in range(DH):
        rows = stage[pl.ds(d * DP, HA), :]
        o0 = (t * DA + d * HA) // 2
        wtp[rb, o0:o0 + HA // 2, :] = _pack(rows.astype(bf16))


def _prep_wo_block(nb, wo_v, stage, wop, dep=None):
    z = None if dep is None else _zero_after(dep)
    for h in range(HA):
        rows = wo_v[nb, h * DH:(h + 1) * DH, :].astype(f32)
        if z is not None:
            rows = pltpu.bitcast(_or_tiled(pltpu.bitcast(rows, u32), z), f32)
        stage[pl.ds(h, DH, stride=DP), :] = rows
    for d in range(DH):
        rows = stage[pl.ds(d * DP, HA), :]
        wop[nb, d * (HA // 2):(d + 1) * (HA // 2), :] = _pack(rows.astype(bf16))
    return wop[nb, DA // 2 - 8:DA // 2, :]


NB = 512


def _a_proj(t, r, ax_v, wtp, dst):
    r0 = pl.multiple_of(r * TA, TA)
    x = ax_v[pl.ds(r0, TA), :]
    for n in range(DA // NB):
        f0 = (t * DA + n * NB) // 2
        w = jnp.concatenate(
            [_unpack(wtp[rb, f0:f0 + NB // 2, :]) for rb in range(8)], axis=1)
        y = _dot_nt(x, w)
        if t == 0:
            y = y * ((DH ** -0.5) * LOG2E)
        for cc in range(NB // 128):
            dst[n * (NB // 128) + cc, pl.ds(r0 + PADR, TA), :] = (
                y[:, cc * 128:(cc + 1) * 128])


def _a_attn_rows(row0, qp, kp, vp, masked, dep):
    G = 8
    q = [qp[c, pl.ds(row0 + PADR, G), :] for c in range(8)]
    if dep is not None:
        z = _zero_after(pltpu.bitcast(dep, u32), A_ROLLS)
        q = [pltpu.bitcast(pltpu.bitcast(x, u32) | z, f32) for x in q]
    if masked:
        pos = row0 + jax.lax.broadcasted_iota(jnp.int32, (G, 128), 0)
    logits = []
    for w in range(WIN):
        z = None
        for c in range(8):
            p = q[c] * kp[c, pl.ds(row0 + PADR - DIL * w, G), :]
            z = p if z is None else z + p
        z = z + pltpu.roll(z, 64, 1)
        z = z + pltpu.roll(z, 32, 1)
        if masked and w > 0:
            z = jnp.where(pos >= DIL * w, z, NEG)
        logits.append(z)
    m = logits[0]
    for w in range(1, WIN):
        m = jnp.maximum(m, logits[w])
    es = [jnp.exp2(z - m) for z in logits]
    l = es[0]
    for w in range(1, WIN):
        l = l + es[w]
    inv = 1.0 / l
    attn = [e * inv for e in es]
    outs = []
    for c in range(8):
        acc = None
        for w in range(WIN):
            v = vp[c, pl.ds(row0 + PADR - DIL * w, G), :]
            acc = attn[w] * v if acc is None else acc + attn[w] * v
        outs.append(acc)
    return outs


def _a_attn_chunk(row0, n, qp, kp, vp):
    units = []
    for g in range(n // 8):
        dep = units[g - A_PACE][7] if g >= A_PACE else None
        units.append(_a_attn_rows(row0 + g * 8, qp, kp, vp, g < 2, dep))
    return jnp.concatenate(
        [jnp.concatenate(u, axis=1) for u in units], axis=0).astype(bf16)


def _deinterleave_block(mb, raw, dst, rows, dep=None):
    pitch = rows + 1
    base = pl.multiple_of(mb * 8, 8)
    blk = _pack(raw[pl.ds(pl.multiple_of(base * H, 8 * H), 8 * H), :])
    if dep is not None:
        blk = _or_tiled(blk, _zero_after(dep))
    for mm in range(8):
        dst[pl.ds(base + mm, H // 2, stride=pitch), :] = (
            blk[mm * (H // 2):(mm + 1) * (H // 2), :])
    return dst[pl.ds(base + (H // 2 - 1) * pitch, 8), :]


def _repack_rows(row0, n, src, dst, dep=None):
    val = _pack(src[pl.ds(pl.multiple_of(row0, n), n), :])
    if dep is not None:
        val = _or_tiled(val, _zero_after(dep))
    dst[pl.ds(pl.multiple_of(row0 // 2, n // 2), n // 2), :] = val
    last = pl.multiple_of((row0 + n) // 2 - 8, 8)
    return dst[pl.ds(last, 8), val.shape[1] - 128:val.shape[1]]


def _pair_weights(wt, j, rows):
    w = wt[pl.ds(j * (rows + 1), rows), :]
    lo = pltpu.bitcast(w << 16, f32).astype(bf16)
    hi = pltpu.bitcast(w & jnp.uint32(0xFFFF0000), f32).astype(bf16)
    return jnp.concatenate([lo, hi], axis=1)


def _b_proj_parts(p0, ws, bxp, cp, qb, kb, vb, slot0):
    wq, wk, wv = ws
    rows = pl.ds(p0, TP // 2)

    def put(dst, y):
        for e in range(2):
            dst[slot0 + e, rows, :] = _pack(y[:, e * D:(e + 1) * D].astype(bf16))

    return [
        lambda: put(qb, _dot(_unpack(bxp[rows, :]), wq) * ((D ** -0.5) * LOG2E)),
        lambda: put(kb, _dot(_unpack(cp[rows, :]), wk)),
        lambda: put(vb, _dot(_unpack(cp[rows, :]), wv)),
    ]


HQ = TQ // 2


def _b_qk(i, qa, ka):
    k0 = i * TQ
    n = k0 + HQ
    q = qa[k0:k0 + TQ]
    s = _dot_nt(q, ka[0:n])
    s2 = _dot_nt(q[HQ:], ka[n:n + HQ])
    row = jax.lax.broadcasted_iota(jnp.int32, (HQ, 128), 0)
    col = jax.lax.broadcasted_iota(jnp.int32, (HQ, 128), 1)
    tri = col <= row
    nb = n // 128
    top = [s[:HQ, j * 128:(j + 1) * 128] for j in range(nb)]
    top[-1] = jnp.where(tri, top[-1], NEG)
    bot = [s[HQ:, j * 128:(j + 1) * 128] for j in range(nb)]
    bot.append(jnp.where(tri, s2, NEG))
    mps = []
    for blocks in (top, bot):
        mp = blocks[0]
        for c in blocks[1:]:
            mp = jnp.maximum(mp, c)
        mps.append(mp)
    return (top, bot), mps


def _b_softmax(blocks, mps, prev):
    ps, lps = [], []
    for half in range(2):
        mp = mps[half]
        if prev is not None:
            mp = jnp.maximum(mp, jnp.minimum(prev[half], NEG))
        m = jnp.max(mp, axis=1, keepdims=True)
        lp = None
        pl_ = []
        for jj, c in enumerate(blocks[half]):
            p = jnp.exp2(c - m)
            lp = p if lp is None else lp + p
            if jj == len(blocks[half]) - 1:
                p = p + jnp.minimum(lp, 0.0)
            pl_.append(p.astype(bf16))
        ps.append(pl_)
        lps.append(lp)
    return ps, lps


def _b_pv(i, ps, lps, va, ctx, h):
    k0 = i * TQ
    n = k0 + HQ
    nb = n // 128
    ls = [jnp.sum(lp, axis=1, keepdims=True) for lp in lps]
    pc = jnp.concatenate(
        [jnp.concatenate(ps[0], axis=1), jnp.concatenate(ps[1][:nb], axis=1)], axis=0)
    o = _dot(pc, va[0:n])
    o2 = _dot(ps[1][nb], va[n:n + HQ])
    o_top = o[:HQ] * (1.0 / ls[0])
    o_bot = (o[HQ:] + o2) * (1.0 / ls[1])
    ctx[h, k0 // 2:(k0 + HQ) // 2, :] = _pack(o_top.astype(bf16))
    ctx[h, (k0 + HQ) // 2:(k0 + TQ) // 2, :] = _pack(o_bot.astype(bf16))
    return (o_top, o_bot)


def _b_head(h, slot, qb, kb, vb, ctx, order, lags, fillers):
    qa, ka, va = _unpack(qb[slot]), _unpack(kb[slot]), _unpack(vb[slot])
    cur = _b_qk(order[0], qa, ka)
    outs = []
    for t, i in enumerate(order):
        nxt = _b_qk(order[t + 1], qa, ka) if t + 1 < len(order) else None
        for f in fillers.get(('a', t), ()):
            f()
        prev = outs[-lags[t]] if 0 < lags[t] <= len(outs) else None
        ps, lps = _b_softmax(cur[0], cur[1], prev)
        for f in fillers.get(('m', t), ()):
            f()
        outs.append(_b_pv(i, ps, lps, va, ctx, h))
        for f in fillers.get(('p', t), ()):
            f()
        cur = nxt


MAIN_ORDER = (1, 7, 3, 4, 6, 2, 5, 0)
MAIN_LAGS = (1, 1, 1, 1, 1, 0, 1, 1)
MAIN_PLACE = (
    (6, ('a', 6)), (0, ('m', 4)), (1, ('p', 0)), (4, ('p', 0)), (11, ('m', 7)),
    (3, ('m', 4)), (10, ('p', 3)), (7, ('m', 6)), (9, ('m', 4)), (2, ('a', 4)),
    (8, ('p', 6)), (5, ('m', 1)))
TAIL_ORDER = (1, 7, 3, 4, 2, 5, 6, 0)
TAIL_LAGS = (1, 1, 1, 1, 1, 1, 0, 2)


def _kernel(ax_h, wqkv_h, wo_h, bx_h, c_h, wq_h, wuk_h, wuv_h, wob_h, out_h,
            qb, kb, vb, wop, qp, kp, vp,
            wq_t, wk_t, wv_t, bxp, cp, out_s,
            sem_w, sem_ax, sem_x0, sem_f, sem_wob, sem_out, sem_oa):
    NR = S // TA

    def rows(ref, r, n):
        return ref.at[pl.ds(pl.multiple_of(r * n, n), n), :]

    def phase_a(ax_v, x0, wqkv_v, wo_v, stage, wtp, bx_v, c_v,
                wq_raw, wuk_raw, wuv_raw):
        def w_copy(t, rb):
            r0 = pl.multiple_of(rb * 128, 128)
            sl = (pl.ds(r0, 128), slice(t * DA, (t + 1) * DA))
            return pltpu.make_async_copy(wqkv_h.at[sl], wqkv_v.at[sl],
                                         sem_w.at[8 * t + rb])

        def ax_copy(r):
            return pltpu.make_async_copy(rows(ax_h, r, TA), rows(ax_v, r, TA),
                                         sem_ax.at[r])

        def x0_copy(rb):
            c0 = pl.multiple_of(rb * 128, 128)
            return pltpu.make_async_copy(ax_h.at[0:Q0, pl.ds(c0, 128)], x0.at[rb],
                                         sem_x0.at[rb])

        def f_copy(r, i):
            sem = sem_f.at[7 * r + i]
            if i < 3:
                src, dst, n = ((wq_h, wq_raw, M), (wuk_h, wuk_raw, C),
                               (wuv_h, wuv_raw, C))[i]
                n = n * H // NR
                return pltpu.make_async_copy(rows(src, r, n), rows(dst, r, n), sem)
            if i < 5:
                src, dst = ((bx_h, bx_v), (c_h, c_v))[i - 3]
                return pltpu.make_async_copy(rows(src, r, TA), rows(dst, r, TA), sem)
            nb = 2 * r + (i - 5)
            c0 = pl.multiple_of(nb * 128, 128)
            return pltpu.make_async_copy(wo_h.at[:, pl.ds(c0, 128)], wo_v.at[nb], sem)

        W = lambda t, rb: (lambda: w_copy(t, rb))
        X = lambda r: (lambda: ax_copy(r))
        F = lambda r, i: (lambda: f_copy(r, i))
        sched = {
            2: [X(3), W(1, 4), W(1, 5), W(1, 6), W(1, 7), F(0, 2), F(0, 4)],
            3: [W(2, 0), W(2, 1), X(0), X(1), F(0, 3)],
            4: [W(2, 2), W(2, 3), F(0, 5), F(0, 6), F(1, 0), F(1, 4)],
            5: [W(2, 4), W(2, 5), F(1, 1), F(1, 2), F(1, 3)],
            6: [W(2, 6), W(2, 7), F(1, 5), F(1, 6), F(2, 0), F(2, 4)],
            7: [F(2, 1), F(2, 2), F(2, 3), F(2, 5), F(2, 6)],
            8: [F(3, 0), F(3, 1)],
            9: [F(3, 2), F(3, 3), F(3, 4), F(3, 5), F(3, 6)],
        }

        def issue_at(table, idx, keys):
            for k in keys:
                items = table.get(k, [])
                if items:
                    @pl.when(idx == k)
                    def _():
                        for mk in items:
                            mk().start()

        def issue(t, r):
            issue_at({k - NR * t: v for k, v in sched.items()}, r, range(NR))

        w_copy(0, 0).start()
        x0_copy(0).start()
        w_copy(0, 1).start()
        x0_copy(1).start()
        w_copy(0, 2).start()
        for ref in (kp, vp):
            ref[:, 0:PADR, :] = jnp.zeros((8, PADR, 128), f32)
        qp[:, PADR:PADR + Q0, :] = jnp.zeros((8, Q0, 128), f32)
        w_copy(0, 0).wait()
        _prep_w_block(0, 0, wqkv_v, stage.at[0], wtp)
        early = {k: ([lambda k=k: x0_copy(k + 2)] if k + 2 < 8 else [])
                 + ([W(0, k + 3)] if k + 3 < 8 else []) for k in range(8)}
        early[2].append(X(2))
        early[4] += [W(1, 0), W(1, 1)]
        early[5] += [W(1, 2), W(1, 3)]
        early[6].append(F(0, 0))
        early[7].append(F(0, 1))

        def q0_step(rb, carry):
            x0_copy(rb).wait()

            @pl.when(rb < 7)
            def _():
                w_copy(0, rb + 1).wait()

            issue_at(early, rb, range(8))
            y = _dot_nt(x0[rb], _unpack(wtp[rb, 0:DA // 2, :]))
            y = y * ((DH ** -0.5) * LOG2E)
            for c in range(8):
                qp[c, PADR:PADR + Q0, :] += y[:, c * 128:(c + 1) * 128]
            _prep_w_block(0, jnp.minimum(rb + 1, 7), wqkv_v, stage.at[1], wtp)
            return carry

        jax.lax.fori_loop(0, 8, q0_step, 0)

        r1 = Q0 // TA
        nw = 8 // (NR - r1)

        def q_step(r, carry):
            ax_copy(r).wait()
            for i in range(nw):
                w_copy(1, nw * (r - r1) + i).wait()
            issue(0, r)
            _a_proj(0, r, ax_v, wtp, qp)
            for i in range(nw):
                _prep_w_block(1, nw * (r - r1) + i, wqkv_v, stage.at[i], wtp)
            return carry

        jax.lax.fori_loop(r1, NR, q_step, 0)

        def k_step(r, carry):
            @pl.when(r < r1)
            def _():
                ax_copy(r).wait()

            w_copy(2, 2 * r).wait()
            w_copy(2, 2 * r + 1).wait()
            issue(1, r)
            _a_proj(1, r, ax_v, wtp, kp)
            for i in range(2):
                _prep_w_block(2, 2 * r + i, wqkv_v, stage.at[i], wtp)
            return carry

        jax.lax.fori_loop(0, NR, k_step, 0)

        def v_step(r, carry):
            for i in range(7):
                f_copy(r, i).wait()
            issue(2, r)
            _a_proj(2, r, ax_v, wtp, vp)
            nq = M // 8 // NR
            nk = C // 8 // NR
            items = (
                [functools.partial(_deinterleave_block, r * nq + i, wq_raw, wq_t, M)
                 for i in range(nq)]
                + [functools.partial(_deinterleave_block, r * nk + i, wuk_raw, wk_t, C)
                   for i in range(nk)]
                + [functools.partial(_deinterleave_block, r * nk + i, wuv_raw, wv_t, C)
                   for i in range(nk)]
                + [functools.partial(_prep_wo_block, 2 * r + i, wo_v, stage.at[i], wop)
                   for i in range(2)]
                + [functools.partial(_repack_rows, r * TA + i * 32, 32, bx_v, bxp)
                   for i in range(TA // 32)]
                + [functools.partial(_repack_rows, r * TA + i * 64, 64, c_v, cp)
                   for i in range(TA // 64)])
            backs = []
            for idx, f in enumerate(items):
                backs.append(f(backs[idx - PACE] if idx >= PACE else None))
            return carry

        jax.lax.fori_loop(0, NR, v_step, 0)

    pl.run_scoped(
        phase_a,
        pltpu.VMEM((S, DA), bf16), pltpu.VMEM((8, Q0, 128), bf16),
        pltpu.VMEM((DA, 3 * DA), bf16),
        pltpu.VMEM((8, DA, 128), bf16), pltpu.VMEM((4, HA * DP, 128), f32),
        pltpu.VMEM((8, 3 * DA // 2, 128), u32),
        pltpu.VMEM((S, M), bf16), pltpu.VMEM((S, C), bf16),
        pltpu.VMEM((M * H, D), bf16), pltpu.VMEM((C * H, D), bf16),
        pltpu.VMEM((C * H, D), bf16))

    def phase_b(ctx, wob_v):
        wob_copy = pltpu.make_async_copy(wob_h, wob_v, sem_wob)
        wob_copy.start()

        def weights(j):
            return (_pair_weights(wq_t, j, M), _pair_weights(wk_t, j, C),
                    _pair_weights(wv_t, j, C))

        half = S // 4
        nf = S // TP // 2

        def first(e, carry):
            ws = weights(0)
            for r in range(nf):
                p0 = pl.multiple_of(e * half + r * (TP // 2), TP // 2)
                for f in _b_proj_parts(p0, ws, bxp, cp, qb, kb, vb, 0):
                    f()
            return carry

        jax.lax.fori_loop(0, 2, first, 0)

        def body(h, carry):
            e = h % 2
            ws = weights(h // 2 + 1)
            wslot = 2 * ((h // 2 + 1) % 2)
            items = []
            for r in range(nf):
                p0 = pl.multiple_of(e * half + r * (TP // 2), TP // 2)
                items += _b_proj_parts(p0, ws, bxp, cp, qb, kb, vb, wslot)
            fillers = {}
            for j, pos in MAIN_PLACE:
                fillers.setdefault(pos, []).append(items[j])
            _b_head(h, h % 4, qb, kb, vb, ctx, MAIN_ORDER, MAIN_LAGS, fillers)
            return carry

        jax.lax.fori_loop(0, H - 2, body, 0)

        for h in range(H - 2, H):
            _b_head(h, h % 4, qb, kb, vb, ctx, TAIL_ORDER, TAIL_LAGS, {})

        wob_copy.wait()

        def out_copy(r, c0, n, sem):
            sl = (pl.ds(pl.multiple_of(r * TO, TO), TO), slice(c0, c0 + n))
            return pltpu.make_async_copy(out_s.at[sl], out_h.at[sl], sem)

        def obody(r, carry):
            r0 = pl.multiple_of(r * TO, TO)
            p0 = pl.multiple_of(r * (TO // 2), TO // 2)
            oa = _a_attn_chunk(r * TO, TO, qp, kp, vp)
            cb = jnp.concatenate(
                [_unpack(ctx[h, pl.ds(p0, TO // 2), :]) for h in range(H)], axis=1)
            out_s[pl.ds(r0, TO), DA:DA + M] = _dot(cb, wob_v[...]).astype(bf16)
            out_copy(r, DA, M, sem_out).start()
            for n in range(2):
                c0 = n * (DA // 2)
                woa = jnp.concatenate(
                    [_unpack(wop[nb]) for nb in range(4 * n, 4 * n + 4)], axis=1)
                out_s[pl.ds(r0, TO), c0:c0 + DA // 2] = _dot(oa, woa).astype(bf16)
                out_copy(r, c0, DA // 2, sem_oa).start()
            return carry

        jax.lax.fori_loop(0, S // TO, obody, 0)
        for r in range(S // TO):
            out_copy(r, DA, M, sem_out).wait()
            for n in range(2):
                out_copy(r, n * (DA // 2), DA // 2, sem_oa).wait()

    pl.run_scoped(
        phase_b,
        pltpu.VMEM((H, S // 2, D), u32), pltpu.VMEM((H * D, M), bf16))


@jax.jit
def pallas_concat_heads__sliding_local_dilated__compressed_kv_cla__prompt_kernel(
    A_x: jax.Array,
    A_wqkv: jax.Array,
    A_wo: jax.Array,
    B_x: jax.Array,
    B_c_kv: jax.Array,
    B_w_q: jax.Array,
    B_w_uk: jax.Array,
    B_w_uv: jax.Array,
    B_w_o: jax.Array,
):
    any_spec = pl.BlockSpec(memory_space=pl.ANY)
    out = pl.pallas_call(
        _kernel,
        out_shape=jax.ShapeDtypeStruct((S, DA + M), bf16),
        in_specs=[any_spec] * 9,
        out_specs=any_spec,
        scratch_shapes=[
            pltpu.VMEM((4, S // 2, D), u32),
            pltpu.VMEM((4, S // 2, D), u32),
            pltpu.VMEM((4, S // 2, D), u32),
            pltpu.VMEM((8, DA // 2, 128), u32),
            pltpu.VMEM((8, S + PADR, 128), f32),
            pltpu.VMEM((8, S + PADR, 128), f32),
            pltpu.VMEM((8, S + PADR, 128), f32),
            pltpu.VMEM((H // 2 * (M + 1) + 48, D), u32),
            pltpu.VMEM((H // 2 * (C + 1) + 48, D), u32),
            pltpu.VMEM((H // 2 * (C + 1) + 48, D), u32),
            pltpu.VMEM((S // 2, M), u32),
            pltpu.VMEM((S // 2, C), u32),
            pltpu.VMEM((S, DA + M), bf16),
            pltpu.SemaphoreType.DMA((24,)),
            pltpu.SemaphoreType.DMA((4,)),
            pltpu.SemaphoreType.DMA((8,)),
            pltpu.SemaphoreType.DMA((28,)),
            pltpu.SemaphoreType.DMA(()),
            pltpu.SemaphoreType.DMA(()),
            pltpu.SemaphoreType.DMA(()),
        ],
        compiler_params=pltpu.CompilerParams(vmem_limit_bytes=120 * 1024 * 1024),
    )(
        A_x.reshape(S, DA), A_wqkv, A_wo,
        B_x.reshape(S, M), B_c_kv.reshape(S, C),
        B_w_q.reshape(M * H, D), B_w_uk.reshape(C * H, D), B_w_uv.reshape(C * H, D),
        B_w_o.reshape(H * D, M),
    )
    return out.reshape(1, S, DA + M)
```

```python
import functools
import math

import jax
import jax.numpy as jnp
import jax.experimental.pallas as pl
import jax.experimental.pallas.tpu as pltpu

bf16 = jnp.bfloat16
f32 = jnp.float32
u32 = jnp.uint32

S = 2048
DA = 1024
HA = 32
DH = 32
WIN = 8
DIL = 2
M = 1024
C = 512
H = 32
D = 128
LOG2E = math.log2(math.e)
NEG = -1e30
PADR = 16
DP = HA + 1
TA = 512
Q0 = 1024
TQ = 256
TP = 256
TO = 256
PACE = 16
P_ROLLS = 3
NM = 4
A_PACE = 3
A_ROLLS = 5
NT = (((1,), (1,)), ((), ()))


def _unpack(x):
    return pltpu.bitcast(x, bf16)


def _pack(x):
    return pltpu.bitcast(x, u32)


def _dot(a, b):
    return jnp.dot(a, b, preferred_element_type=f32)


def _dot_nt(a, b):
    return jax.lax.dot_general(a, b, NT, preferred_element_type=f32)


def _zero_after(dep, rolls=P_ROLLS):
    for _ in range(rolls):
        dep = pltpu.roll(dep, 1, 1)
    return (dep >> 16) >> 16


def _or_tiled(x, z):
    row = jnp.concatenate([z] * (x.shape[1] // 128), axis=1)
    return x | jnp.concatenate([row] * (x.shape[0] // 8), axis=0)


def _prep_w_block(t, rb, wqkv_v, stage, wtp):
    r0 = pl.multiple_of(rb * 128, 128)
    for cb in range(8):
        c0 = t * DA + cb * 128
        tile = wqkv_v[pl.ds(r0, 128), c0:c0 + 128].astype(f32).T
        for hl in range(4):
            stage[pl.ds(4 * cb + hl, DH, stride=DP), :] = tile[hl * DH:(hl + 1) * DH, :]
    for d in range(DH):
        rows = stage[pl.ds(d * DP, HA), :]
        o0 = (t * DA + d * HA) // 2
        wtp[rb, o0:o0 + HA // 2, :] = _pack(rows.astype(bf16))


def _prep_wo_block(nb, wo_v, stage, wop, dep=None):
    z = None if dep is None else _zero_after(dep)
    for h in range(HA):
        rows = wo_v[nb, h * DH:(h + 1) * DH, :].astype(f32)
        if z is not None:
            rows = pltpu.bitcast(_or_tiled(pltpu.bitcast(rows, u32), z), f32)
        stage[pl.ds(h, DH, stride=DP), :] = rows
    for d in range(DH):
        rows = stage[pl.ds(d * DP, HA), :]
        wop[nb, d * (HA // 2):(d + 1) * (HA // 2), :] = _pack(rows.astype(bf16))
    return wop[nb, DA // 2 - 8:DA // 2, :]


NB = 512


def _a_proj(t, r, ax_v, wtp, dst):
    r0 = pl.multiple_of(r * TA, TA)
    x = ax_v[pl.ds(r0, TA), :]
    for n in range(DA // NB):
        f0 = (t * DA + n * NB) // 2
        w = jnp.concatenate(
            [_unpack(wtp[rb, f0:f0 + NB // 2, :]) for rb in range(8)], axis=1)
        y = _dot_nt(x, w)
        if t == 0:
            y = y * ((DH ** -0.5) * LOG2E)
        for cc in range(NB // 128):
            dst[n * (NB // 128) + cc, pl.ds(r0 + PADR, TA), :] = (
                y[:, cc * 128:(cc + 1) * 128])


def _a_attn_rows(row0, qp, kp, vp, masked, dep):
    G = 8
    q = [qp[c, pl.ds(row0 + PADR, G), :] for c in range(8)]
    if dep is not None:
        z = _zero_after(pltpu.bitcast(dep, u32), A_ROLLS)
        q = [pltpu.bitcast(pltpu.bitcast(x, u32) | z, f32) for x in q]
    if masked:
        pos = row0 + jax.lax.broadcasted_iota(jnp.int32, (G, 128), 0)
    logits = []
    for w in range(WIN):
        z = None
        for c in range(8):
            p = q[c] * kp[c, pl.ds(row0 + PADR - DIL * w, G), :]
            z = p if z is None else z + p
        z = z + pltpu.roll(z, 64, 1)
        z = z + pltpu.roll(z, 32, 1)
        if masked and w > 0:
            z = jnp.where(pos >= DIL * w, z, NEG)
        logits.append(z)
    m = logits[0]
    for w in range(1, WIN):
        m = jnp.maximum(m, logits[w])
    es = [jnp.exp2(z - m) for z in logits]
    l = es[0]
    for w in range(1, WIN):
        l = l + es[w]
    inv = 1.0 / l
    attn = [e * inv for e in es]
    outs = []
    for c in range(8):
        acc = None
        for w in range(WIN):
            v = vp[c, pl.ds(row0 + PADR - DIL * w, G), :]
            acc = attn[w] * v if acc is None else acc + attn[w] * v
        outs.append(acc)
    return outs


def _a_attn_chunk(row0, n, qp, kp, vp):
    units = []
    for g in range(n // 8):
        dep = units[g - A_PACE][7] if g >= A_PACE else None
        units.append(_a_attn_rows(row0 + g * 8, qp, kp, vp, g < 2, dep))
    return jnp.concatenate(
        [jnp.concatenate(u, axis=1) for u in units], axis=0).astype(bf16)


def _deinterleave_block(m0, raw, dst, rows, dep=None):
    pitch = rows + 1
    base = pl.multiple_of(m0, NM)
    blk = _pack(raw[pl.ds(pl.multiple_of(base * H, NM * H), NM * H), :])
    if dep is not None:
        blk = _or_tiled(blk, _zero_after(dep))
    for mm in range(NM):
        dst[pl.ds(base + mm, H // 2, stride=pitch), :] = (
            blk[mm * (H // 2):(mm + 1) * (H // 2), :])
    back = dst[pl.ds(base + (H // 2 - 1) * pitch, NM), :]
    return jnp.concatenate([back] * (8 // NM), axis=0)


def _repack_rows(row0, n, src, dst, dep=None):
    val = _pack(src[pl.ds(pl.multiple_of(row0, n), n), :])
    if dep is not None:
        val = _or_tiled(val, _zero_after(dep))
    dst[pl.ds(pl.multiple_of(row0 // 2, n // 2), n // 2), :] = val
    last = pl.multiple_of((row0 + n) // 2 - 8, 8)
    return dst[pl.ds(last, 8), val.shape[1] - 128:val.shape[1]]


def _pair_weights(wt, j, rows):
    w = wt[pl.ds(j * (rows + 1), rows), :]
    lo = pltpu.bitcast(w << 16, f32).astype(bf16)
    hi = pltpu.bitcast(w & jnp.uint32(0xFFFF0000), f32).astype(bf16)
    return jnp.concatenate([lo, hi], axis=1)


def _b_proj_parts(p0, ws, bxp, cp, qb, kb, vb, slot0):
    wq, wk, wv = ws
    rows = pl.ds(p0, TP // 2)

    def put(dst, y):
        for e in range(2):
            dst[slot0 + e, rows, :] = _pack(y[:, e * D:(e + 1) * D].astype(bf16))

    return [
        lambda: put(qb, _dot(_unpack(bxp[rows, :]), wq) * ((D ** -0.5) * LOG2E)),
        lambda: put(kb, _dot(_unpack(cp[rows, :]), wk)),
        lambda: put(vb, _dot(_unpack(cp[rows, :]), wv)),
    ]


HQ = TQ // 2


def _b_qk(i, qa, ka):
    k0 = i * TQ
    n = k0 + HQ
    q = qa[k0:k0 + TQ]
    s = _dot_nt(q, ka[0:n])
    s2 = _dot_nt(q[HQ:], ka[n:n + HQ])
    row = jax.lax.broadcasted_iota(jnp.int32, (HQ, 128), 0)
    col = jax.lax.broadcasted_iota(jnp.int32, (HQ, 128), 1)
    tri = col <= row
    nb = n // 128
    top = [s[:HQ, j * 128:(j + 1) * 128] for j in range(nb)]
    top[-1] = jnp.where(tri, top[-1], NEG)
    bot = [s[HQ:, j * 128:(j + 1) * 128] for j in range(nb)]
    bot.append(jnp.where(tri, s2, NEG))
    mps = []
    for blocks in (top, bot):
        mp = blocks[0]
        for c in blocks[1:]:
            mp = jnp.maximum(mp, c)
        mps.append(mp)
    return (top, bot), mps


def _b_softmax(blocks, mps, prev):
    ps, lps = [], []
    for half in range(2):
        mp = mps[half]
        if prev is not None:
            mp = jnp.maximum(mp, jnp.minimum(prev[half], NEG))
        m = jnp.max(mp, axis=1, keepdims=True)
        lp = None
        pl_ = []
        for jj, c in enumerate(blocks[half]):
            p = jnp.exp2(c - m)
            lp = p if lp is None else lp + p
            if jj == len(blocks[half]) - 1:
                p = p + jnp.minimum(lp, 0.0)
            pl_.append(p.astype(bf16))
        ps.append(pl_)
        lps.append(lp)
    return ps, lps


def _b_pv(i, ps, lps, va, ctx, h):
    k0 = i * TQ
    n = k0 + HQ
    nb = n // 128
    ls = [jnp.sum(lp, axis=1, keepdims=True) for lp in lps]
    pc = jnp.concatenate(
        [jnp.concatenate(ps[0], axis=1), jnp.concatenate(ps[1][:nb], axis=1)], axis=0)
    o = _dot(pc, va[0:n])
    o2 = _dot(ps[1][nb], va[n:n + HQ])
    o_top = o[:HQ] * (1.0 / ls[0])
    o_bot = (o[HQ:] + o2) * (1.0 / ls[1])
    ctx[h, k0 // 2:(k0 + HQ) // 2, :] = _pack(o_top.astype(bf16))
    ctx[h, (k0 + HQ) // 2:(k0 + TQ) // 2, :] = _pack(o_bot.astype(bf16))
    return (o_top, o_bot)


def _b_head(h, slot, qb, kb, vb, ctx, order, lags, fillers):
    qa, ka, va = _unpack(qb[slot]), _unpack(kb[slot]), _unpack(vb[slot])
    cur = _b_qk(order[0], qa, ka)
    outs = []
    for t, i in enumerate(order):
        nxt = _b_qk(order[t + 1], qa, ka) if t + 1 < len(order) else None
        for f in fillers.get(('a', t), ()):
            f()
        prev = outs[-lags[t]] if 0 < lags[t] <= len(outs) else None
        ps, lps = _b_softmax(cur[0], cur[1], prev)
        for f in fillers.get(('m', t), ()):
            f()
        outs.append(_b_pv(i, ps, lps, va, ctx, h))
        for f in fillers.get(('p', t), ()):
            f()
        cur = nxt


MAIN_ORDER = (1, 7, 3, 4, 6, 2, 5, 0)
MAIN_LAGS = (1, 1, 1, 1, 1, 0, 1, 1)
MAIN_PLACE = (
    (6, ('a', 6)), (0, ('m', 4)), (1, ('p', 0)), (4, ('p', 0)), (11, ('m', 7)),
    (3, ('m', 4)), (10, ('p', 3)), (7, ('m', 6)), (9, ('m', 4)), (2, ('a', 4)),
    (8, ('p', 6)), (5, ('m', 1)))
TAIL_ORDER = (1, 7, 3, 4, 2, 5, 6, 0)
TAIL_LAGS = (1, 1, 1, 1, 1, 1, 0, 2)


def _kernel(ax_h, wqkv_h, wo_h, bx_h, c_h, wq_h, wuk_h, wuv_h, wob_h, out_h,
            qb, kb, vb, wop, qp, kp, vp,
            wq_t, wk_t, wv_t, bxp, cp, out_s,
            sem_w, sem_ax, sem_x0, sem_f, sem_wob, sem_out, sem_oa):
    NR = S // TA

    def rows(ref, r, n):
        return ref.at[pl.ds(pl.multiple_of(r * n, n), n), :]

    def phase_a(ax_v, x0, wqkv_v, wo_v, stage, wtp, bx_v, c_v,
                wq_raw, wuk_raw, wuv_raw):
        def w_copy(t, rb):
            r0 = pl.multiple_of(rb * 128, 128)
            sl = (pl.ds(r0, 128), slice(t * DA, (t + 1) * DA))
            return pltpu.make_async_copy(wqkv_h.at[sl], wqkv_v.at[sl],
                                         sem_w.at[8 * t + rb])

        def ax_copy(r):
            return pltpu.make_async_copy(rows(ax_h, r, TA), rows(ax_v, r, TA),
                                         sem_ax.at[r])

        def x0_copy(rb):
            c0 = pl.multiple_of(rb * 128, 128)
            return pltpu.make_async_copy(ax_h.at[0:Q0, pl.ds(c0, 128)], x0.at[rb],
                                         sem_x0.at[rb])

        def f_copy(r, i):
            sem = sem_f.at[7 * r + i]
            if i < 3:
                src, dst, n = ((wq_h, wq_raw, M), (wuk_h, wuk_raw, C),
                               (wuv_h, wuv_raw, C))[i]
                n = n * H // NR
                return pltpu.make_async_copy(rows(src, r, n), rows(dst, r, n), sem)
            if i < 5:
                src, dst = ((bx_h, bx_v), (c_h, c_v))[i - 3]
                return pltpu.make_async_copy(rows(src, r, TA), rows(dst, r, TA), sem)
            nb = 2 * r + (i - 5)
            c0 = pl.multiple_of(nb * 128, 128)
            return pltpu.make_async_copy(wo_h.at[:, pl.ds(c0, 128)], wo_v.at[nb], sem)

        W = lambda t, rb: (lambda: w_copy(t, rb))
        X = lambda r: (lambda: ax_copy(r))
        F = lambda r, i: (lambda: f_copy(r, i))
        sched = {
            2: [X(3), W(1, 4), W(1, 5), W(1, 6), W(1, 7), F(0, 2), F(0, 4)],
            3: [W(2, 0), W(2, 1), X(0), X(1), F(0, 3)],
            4: [W(2, 2), W(2, 3), F(0, 5), F(0, 6), F(1, 0), F(1, 4)],
            5: [W(2, 4), W(2, 5), F(1, 1), F(1, 2), F(1, 3)],
            6: [W(2, 6), W(2, 7), F(1, 5), F(1, 6), F(2, 0), F(2, 4)],
            7: [F(2, 1), F(2, 2), F(2, 3), F(2, 5), F(2, 6)],
            8: [F(3, 0), F(3, 1)],
            9: [F(3, 2), F(3, 3), F(3, 4), F(3, 5), F(3, 6)],
        }

        def issue_at(table, idx, keys):
            for k in keys:
                items = table.get(k, [])
                if items:
                    @pl.when(idx == k)
                    def _():
                        for mk in items:
                            mk().start()

        def issue(t, r):
            issue_at({k - NR * t: v for k, v in sched.items()}, r, range(NR))

        w_copy(0, 0).start()
        x0_copy(0).start()
        w_copy(0, 1).start()
        x0_copy(1).start()
        w_copy(0, 2).start()
        for ref in (kp, vp):
            ref[:, 0:PADR, :] = jnp.zeros((8, PADR, 128), f32)
        qp[:, PADR:PADR + Q0, :] = jnp.zeros((8, Q0, 128), f32)
        w_copy(0, 0).wait()
        _prep_w_block(0, 0, wqkv_v, stage.at[0], wtp)
        early = {k: ([lambda k=k: x0_copy(k + 2)] if k + 2 < 8 else [])
                 + ([W(0, k + 3)] if k + 3 < 8 else []) for k in range(8)}
        early[2].append(X(2))
        early[4] += [W(1, 0), W(1, 1)]
        early[5] += [W(1, 2), W(1, 3)]
        early[6].append(F(0, 0))
        early[7].append(F(0, 1))

        def q0_step(rb, carry):
            x0_copy(rb).wait()

            @pl.when(rb < 7)
            def _():
                w_copy(0, rb + 1).wait()

            issue_at(early, rb, range(8))
            y = _dot_nt(x0[rb], _unpack(wtp[rb, 0:DA // 2, :]))
            y = y * ((DH ** -0.5) * LOG2E)
            for c in range(8):
                qp[c, PADR:PADR + Q0, :] += y[:, c * 128:(c + 1) * 128]
            _prep_w_block(0, jnp.minimum(rb + 1, 7), wqkv_v, stage.at[1], wtp)
            return carry

        jax.lax.fori_loop(0, 8, q0_step, 0)

        r1 = Q0 // TA
        nw = 8 // (NR - r1)

        def q_step(r, carry):
            ax_copy(r).wait()
            for i in range(nw):
                w_copy(1, nw * (r - r1) + i).wait()
            issue(0, r)
            _a_proj(0, r, ax_v, wtp, qp)
            for i in range(nw):
                _prep_w_block(1, nw * (r - r1) + i, wqkv_v, stage.at[i], wtp)
            return carry

        jax.lax.fori_loop(r1, NR, q_step, 0)

        def k_step(r, carry):
            @pl.when(r < r1)
            def _():
                ax_copy(r).wait()

            w_copy(2, 2 * r).wait()
            w_copy(2, 2 * r + 1).wait()
            issue(1, r)
            _a_proj(1, r, ax_v, wtp, kp)
            for i in range(2):
                _prep_w_block(2, 2 * r + i, wqkv_v, stage.at[i], wtp)
            return carry

        jax.lax.fori_loop(0, NR, k_step, 0)

        def v_step(r, carry):
            for i in range(7):
                f_copy(r, i).wait()
            issue(2, r)
            _a_proj(2, r, ax_v, wtp, vp)
            mq = M // NR
            mk = C // NR
            items = (
                [functools.partial(_deinterleave_block, r * mq + i, wq_raw, wq_t, M)
                 for i in range(0, mq, NM)]
                + [functools.partial(_deinterleave_block, r * mk + i, wuk_raw, wk_t, C)
                   for i in range(0, mk, NM)]
                + [functools.partial(_deinterleave_block, r * mk + i, wuv_raw, wv_t, C)
                   for i in range(0, mk, NM)]
                + [functools.partial(_prep_wo_block, 2 * r + i, wo_v, stage.at[i], wop)
                   for i in range(2)]
                + [functools.partial(_repack_rows, r * TA + i, 16, bx_v, bxp)
                   for i in range(0, TA, 16)]
                + [functools.partial(_repack_rows, r * TA + i, 32, c_v, cp)
                   for i in range(0, TA, 32)])
            backs = []
            for idx, f in enumerate(items):
                backs.append(f(backs[idx - PACE] if idx >= PACE else None))
            return carry

        jax.lax.fori_loop(0, NR, v_step, 0)

    pl.run_scoped(
        phase_a,
        pltpu.VMEM((S, DA), bf16), pltpu.VMEM((8, Q0, 128), bf16),
        pltpu.VMEM((DA, 3 * DA), bf16),
        pltpu.VMEM((8, DA, 128), bf16), pltpu.VMEM((4, HA * DP, 128), f32),
        pltpu.VMEM((8, 3 * DA // 2, 128), u32),
        pltpu.VMEM((S, M), bf16), pltpu.VMEM((S, C), bf16),
        pltpu.VMEM((M * H, D), bf16), pltpu.VMEM((C * H, D), bf16),
        pltpu.VMEM((C * H, D), bf16))

    def phase_b(ctx, wob_v):
        wob_copy = pltpu.make_async_copy(wob_h, wob_v, sem_wob)
        wob_copy.start()

        def weights(j):
            return (_pair_weights(wq_t, j, M), _pair_weights(wk_t, j, C),
                    _pair_weights(wv_t, j, C))

        half = S // 4
        nf = S // TP // 2

        def first(e, carry):
            ws = weights(0)
            for r in range(nf):
                p0 = pl.multiple_of(e * half + r * (TP // 2), TP // 2)
                for f in _b_proj_parts(p0, ws, bxp, cp, qb, kb, vb, 0):
                    f()
            return carry

        jax.lax.fori_loop(0, 2, first, 0)

        def body(h, carry):
            e = h % 2
            ws = weights(h // 2 + 1)
            wslot = 2 * ((h // 2 + 1) % 2)
            items = []
            for r in range(nf):
                p0 = pl.multiple_of(e * half + r * (TP // 2), TP // 2)
                items += _b_proj_parts(p0, ws, bxp, cp, qb, kb, vb, wslot)
            fillers = {}
            for j, pos in MAIN_PLACE:
                fillers.setdefault(pos, []).append(items[j])
            _b_head(h, h % 4, qb, kb, vb, ctx, MAIN_ORDER, MAIN_LAGS, fillers)
            return carry

        jax.lax.fori_loop(0, H - 2, body, 0)

        for h in range(H - 2, H):
            _b_head(h, h % 4, qb, kb, vb, ctx, TAIL_ORDER, TAIL_LAGS, {})

        wob_copy.wait()

        def out_copy(r, c0, n, sem):
            sl = (pl.ds(pl.multiple_of(r * TO, TO), TO), slice(c0, c0 + n))
            return pltpu.make_async_copy(out_s.at[sl], out_h.at[sl], sem)

        def obody(r, carry):
            r0 = pl.multiple_of(r * TO, TO)
            p0 = pl.multiple_of(r * (TO // 2), TO // 2)
            oa = _a_attn_chunk(r * TO, TO, qp, kp, vp)
            cb = jnp.concatenate(
                [_unpack(ctx[h, pl.ds(p0, TO // 2), :]) for h in range(H)], axis=1)
            out_s[pl.ds(r0, TO), DA:DA + M] = _dot(cb, wob_v[...]).astype(bf16)
            out_copy(r, DA, M, sem_out).start()
            for n in range(2):
                c0 = n * (DA // 2)
                woa = jnp.concatenate(
                    [_unpack(wop[nb]) for nb in range(4 * n, 4 * n + 4)], axis=1)
                out_s[pl.ds(r0, TO), c0:c0 + DA // 2] = _dot(oa, woa).astype(bf16)
                out_copy(r, c0, DA // 2, sem_oa).start()
            return carry

        jax.lax.fori_loop(0, S // TO, obody, 0)
        for r in range(S // TO):
            out_copy(r, DA, M, sem_out).wait()
            for n in range(2):
                out_copy(r, n * (DA // 2), DA // 2, sem_oa).wait()

    pl.run_scoped(
        phase_b,
        pltpu.VMEM((H, S // 2, D), u32), pltpu.VMEM((H * D, M), bf16))


@jax.jit
def pallas_concat_heads__sliding_local_dilated__compressed_kv_cla__prompt_kernel(
    A_x: jax.Array,
    A_wqkv: jax.Array,
    A_wo: jax.Array,
    B_x: jax.Array,
    B_c_kv: jax.Array,
    B_w_q: jax.Array,
    B_w_uk: jax.Array,
    B_w_uv: jax.Array,
    B_w_o: jax.Array,
):
    any_spec = pl.BlockSpec(memory_space=pl.ANY)
    out = pl.pallas_call(
        _kernel,
        out_shape=jax.ShapeDtypeStruct((S, DA + M), bf16),
        in_specs=[any_spec] * 9,
        out_specs=any_spec,
        scratch_shapes=[
            pltpu.VMEM((4, S // 2, D), u32),
            pltpu.VMEM((4, S // 2, D), u32),
            pltpu.VMEM((4, S // 2, D), u32),
            pltpu.VMEM((8, DA // 2, 128), u32),
            pltpu.VMEM((8, S + PADR, 128), f32),
            pltpu.VMEM((8, S + PADR, 128), f32),
            pltpu.VMEM((8, S + PADR, 128), f32),
            pltpu.VMEM((H // 2 * (M + 1) + 48, D), u32),
            pltpu.VMEM((H // 2 * (C + 1) + 48, D), u32),
            pltpu.VMEM((H // 2 * (C + 1) + 48, D), u32),
            pltpu.VMEM((S // 2, M), u32),
            pltpu.VMEM((S // 2, C), u32),
            pltpu.VMEM((S, DA + M), bf16),
            pltpu.SemaphoreType.DMA((24,)),
            pltpu.SemaphoreType.DMA((4,)),
            pltpu.SemaphoreType.DMA((8,)),
            pltpu.SemaphoreType.DMA((28,)),
            pltpu.SemaphoreType.DMA(()),
            pltpu.SemaphoreType.DMA(()),
            pltpu.SemaphoreType.DMA(()),
        ],
        compiler_params=pltpu.CompilerParams(vmem_limit_bytes=120 * 1024 * 1024),
    )(
        A_x.reshape(S, DA), A_wqkv, A_wo,
        B_x.reshape(S, M), B_c_kv.reshape(S, C),
        B_w_q.reshape(M * H, D), B_w_uk.reshape(C * H, D), B_w_uv.reshape(C * H, D),
        B_w_o.reshape(H * D, M),
    )
    return out.reshape(1, S, DA + M)
```
